```python
import jax
import jax.numpy as jnp

def _softmax(x, axis=-1):
    return jax.nn.softmax(x, axis=axis)
def _gelu(x):
    return jax.nn.gelu(x, approximate=True)
def _silu(x):
    return jax.nn.silu(x)
def _sigmoid(x):
    return jax.nn.sigmoid(x)
def _layernorm(x, axis=-1, eps=1e-5):
    m = jnp.mean(x, axis=axis, keepdims=True)
    v = jnp.var(x, axis=axis, keepdims=True)
    return (x - m) / jnp.sqrt(v + eps)
def _scatter_add(tgt, idx, src, axis=0):
    return tgt.at[idx].add(src)
def _segment_sum(src, seg, n):
    return jax.ops.segment_sum(src, seg, n)
class _Rng:
    def __init__(self, key):
        self._k = key
    def _next(self):
        self._k, sub = jax.random.split(self._k)
        return sub
    def normal(self, shape):
        return jax.random.normal(self._next(), shape, dtype=jnp.bfloat16)
    def randint(self, lo, hi, shape):
        return jax.random.randint(self._next(), shape, lo, hi, dtype=jnp.int32)
    def uniform(self, shape, lo=0.0, hi=1.0):
        return jax.random.uniform(self._next(), shape, jnp.bfloat16, lo, hi)
    def permutation(self, n):
        return jax.random.permutation(self._next(), n)


kernel_name = 'interleave_layers__sliding_local_dilated__ssm_conv_s4__prompt'

def setup_inputs():
    _rng = _Rng(jax.random.key(int.from_bytes(__import__("os").urandom(4), "little")))
    _w = (lambda a: (lambda t: t.astype(jnp.bfloat16) if jnp.issubdtype(t.dtype, jnp.floating) else t)(jnp.asarray(a)))
    def _A_setup():
        B, S, D = 1, 2048, 512
        return {
            "x": _w((lambda *s: _rng.normal(s) * 0.05)(B, S, D)),
            "wqkv": _w((lambda *s: _rng.normal(s) * 0.05)(D, 3 * D)),
            "wo": _w((lambda *s: _rng.normal(s) * 0.05)(D, D)),
        }
    _A_in = _A_setup()

    def _B_setup():
        B, L, D, N = 1, 2048, 512, 128
        A_re = -jnp.exp((lambda *s: _rng.normal(s) * 0.05)(D, N))
        A_im = jnp.pi * (lambda *s: _rng.normal(s) * 0.05)(D, N)
        B_re = (lambda *s: _rng.normal(s) * 0.05)(D, N)
        B_im = (lambda *s: _rng.normal(s) * 0.05)(D, N)
        C_re = (lambda *s: _rng.normal(s) * 0.05)(D, N)
        C_im = (lambda *s: _rng.normal(s) * 0.05)(D, N)
        log_dt = (lambda *s: _rng.normal(s) * 0.05)(D) * 0.5 - 4.0
        Dskip = (lambda *s: _rng.normal(s) * 0.05)(D)
        return {
            "u": _w((lambda *s: _rng.normal(s) * 0.05)(B, L, D)),
            "A_re": _w(A_re),
            "A_im": _w(A_im),
            "B_re": _w(B_re),
            "B_im": _w(B_im),
            "C_re": _w(C_re),
            "C_im": _w(C_im),
            "log_dt": _w(log_dt),
            "Dskip": _w(Dskip),
        }
    _B_in = _B_setup()

    return {
        "A_x": _A_in["x"],
        "A_wqkv": _A_in["wqkv"],
        "A_wo": _A_in["wo"],
        "B_u": _B_in["u"],
        "B_A_re": _B_in["A_re"],
        "B_A_im": _B_in["A_im"],
        "B_B_re": _B_in["B_re"],
        "B_B_im": _B_in["B_im"],
        "B_C_re": _B_in["C_re"],
        "B_C_im": _B_in["C_im"],
        "B_log_dt": _B_in["log_dt"],
        "B_Dskip": _B_in["Dskip"],
    }

def reference(A_x, A_wqkv, A_wo, B_u, B_A_re, B_A_im, B_B_re, B_B_im, B_C_re, B_C_im, B_log_dt, B_Dskip):
    def _A_ref(x, wqkv, wo):
        B, S, D = x.shape
        H = 32; Dh = D // H
        W, dil = 8, 2
        qkv = (lambda x, *d: x.transpose(*d))((x @ wqkv).reshape(B, S, 3, H, Dh), 2, 0, 3, 1, 4)
        q, k, v = qkv[0], qkv[1], qkv[2]
        scale = Dh ** -0.5
        pos = jnp.arange(S)
        off = jnp.arange(W) * dil
        idx = pos[:, None] - off[None, :]
        mask = idx >= 0
        idx_c = jnp.where(mask, idx, 0).reshape(-1)
        kg = k[:, :, idx_c, :].reshape(B, H, S, W, Dh)
        vg = v[:, :, idx_c, :].reshape(B, H, S, W, Dh)
        logits = jnp.einsum("bhsd,bhswd->bhsw", q, kg) * scale
        logits = jnp.where(mask[None, None, :, :], logits, -1e9)
        attn = _softmax(logits, axis=-1)
        o = jnp.einsum("bhsw,bhswd->bhsd", attn, vg)
        return (lambda x, *d: x.transpose(*d))(o, 0, 2, 1, 3).reshape(B, S, D) @ wo

    def _B_ref(u, A_re, A_im, B_re, B_im, C_re, C_im, log_dt, Dskip):
        Bsz, L, D = u.shape
        dt = jnp.exp(log_dt)[:, None]
        A = A_re + 1j * A_im
        Bc = B_re + 1j * B_im
        Cc = C_re + 1j * C_im
        logdA = dt * A
        dB = dt * Bc
        l = (lambda x, dt: x.astype(dt))(jnp.arange(L), A_re.dtype)
        P = jnp.exp(logdA[:, :, None] * l[None, None, :])
        K = jnp.einsum("dn,dnl,dn->dl", Cc, P, dB).real
        L2 = 2 * L
        Kp = jnp.pad(K, ((0, 0), (0, L)))
        up = (lambda x, *d: x.transpose(*d))(u, 0, 2, 1)
        up = jnp.pad(up, ((0, 0), (0, 0), (0, L)))
        Kf = (lambda x, axes=(-2,-1): jnp.fft.rfft2(x.astype(jnp.float32), axes=axes))(Kp[:, None, :], axes=(-2, -1))
        Uf = (lambda x, axes=(-2,-1): jnp.fft.rfft2(x.astype(jnp.float32), axes=axes))(up[:, :, None, :], axes=(-2, -1))
        Yf = Uf * Kf[None, :, :, :]
        y = (lambda x, s, axes=(-2,-1): jnp.fft.irfft2(x, s=s, axes=axes).astype(jnp.bfloat16))(Yf, (1, L2), axes=(-2, -1))[:, :, 0, :L]
        y = (lambda x, *d: x.transpose(*d))(y, 0, 2, 1) + u * Dskip[None, None, :]
        return y

    x = A_x
    x = x + _A_ref(_layernorm(x, axis=-1), A_wqkv, A_wo)
    x = x + _B_ref(_layernorm(x, axis=-1), B_A_re, B_A_im, B_B_re, B_B_im, B_C_re, B_C_im, B_log_dt, B_Dskip)
    x = x + _A_ref(_layernorm(x, axis=-1), A_wqkv, A_wo)
    x = x + _B_ref(_layernorm(x, axis=-1), B_A_re, B_A_im, B_B_re, B_B_im, B_C_re, B_C_im, B_log_dt, B_Dskip)
    return x
```

```python
import math

import jax
import jax.numpy as jnp
import ml_dtypes
import numpy as np
import jax.experimental.pallas as pl
import jax.experimental.pallas.tpu as pltpu

S, D, H, DH, WIN = 2048, 512, 32, 16, 8
NJ, NA = 16, 128
EPS = 1e-5
F32, BF16, U32, I32 = jnp.float32, jnp.bfloat16, jnp.uint32, jnp.int32
NT = (((1,), (1,)), ((), ()))


def _dft_consts():
    a = np.arange(NA)[None, :, None]
    j = np.arange(NJ)[:, None, None]
    k = np.arange(NA)[None, None, :]
    th = np.pi * (((NJ * a + j) * (2 * k + 1)) % (4 * S)) / (2 * S)
    f = np.concatenate([np.cos(th), -np.sin(th)], axis=-1)
    lane = np.arange(NA)
    ln = (lane - 7) % NA
    fk = f[:, 16 * (ln % 8) + ln // 8, :]
    perm = np.zeros((NA, NA), np.float32)
    perm[lane, (lane % 8) * DH + lane // 8] = 1.0
    pm = np.stack([perm * DH ** -0.5, perm, np.eye(NA, dtype=np.float32)])
    bf = ml_dtypes.bfloat16
    return f.astype(bf), fk.astype(bf), pm.astype(bf)


_F, _FK, _PM = _dft_consts()


def _round_l(l):
    return int(np.float32(l).astype(ml_dtypes.bfloat16).astype(np.float32))


_R = [[_round_l(256 * a1 + j) - 256 * a1 for j in range(NJ)] for a1 in range(8)]
assert all(_round_l(256 * a1 + 16 * b + j) == 256 * a1 + 16 * b + _R[a1][j]
           for a1 in range(8) for b in range(16) for j in range(NJ))
_ENTRIES = [(a1, r) for a1 in range(8) for r in sorted(set(_R[a1]))]


def _cmul(x, y):
    return x[0] * y[0] - x[1] * y[1], x[0] * y[1] + x[1] * y[0]


def _bfly4(x, inv):
    (ar, ai), (br, bi), (cr, ci), (dr, di) = x
    sr, si, tr, ti = ar + cr, ai + ci, ar - cr, ai - ci
    ur, ui, vr, vi = br + dr, bi + di, br - dr, bi - di
    y1, y3 = (tr + vi, ti - vr), (tr - vi, ti + vr)
    if inv:
        y1, y3 = y3, y1
    return [(sr + ur, si + ui), y1, (sr - ur, si - ui), y3]


def _twiddle(x, e):
    e %= 16
    xr, xi = x
    if e == 0:
        return x
    if e == 4:
        return xi, -xr
    if e == 12:
        return -xi, xr
    c, s = math.cos(math.pi * e / 8), -math.sin(math.pi * e / 8)
    if e % 2 == 0:
        if c * s > 0:
            return (xr - xi) * c, (xr + xi) * c
        return (xr + xi) * c, (xi - xr) * c
    return xr * c - xi * s, xr * s + xi * c


def _fft_first(x):
    a = [_bfly4([x[4 * j1 + j0] for j1 in range(4)], False) for j0 in range(4)]
    return [[_twiddle(a[j0][m0], j0 * m0) for j0 in range(4)] for m0 in range(4)]


def _layernorm_t(x):
    m = jnp.sum(x, axis=0, keepdims=True) * (1.0 / D)
    c = x - m
    v = jnp.sum(c * c, axis=0, keepdims=True) * (1.0 / D)
    return c * jax.lax.rsqrt(v + EPS)


def _flip8(x, sub):
    r = [pltpu.roll(x, k, 0) for k in (7, 5, 3, 1)]
    s4 = sub & 3
    return jnp.where(s4 == 3, r[0], jnp.where(s4 == 2, r[1], jnp.where(s4 == 1, r[2], r[3])))


def _kernel(x_hbm, wqkv_hbm, wo_hbm, f_hbm, fk_hbm, pm_ref,
            are_ref, aim_ref, bre_ref, bim_ref, cre_ref, cim_ref, ldt_ref, dsk_ref,
            out_hbm,
            xs, wqkv, wo, fm, fk, par, dtc, dsc, wt, wot, xr, xn, qs, ke, ve, os_, zs, kf,
            sem_in, sem_out):
    xu, xs = xs, xs.bitcast(BF16)
    cp_fk = pltpu.make_async_copy(fk_hbm, fk, sem_in.at[0])
    cp_x = [pltpu.make_async_copy(x_hbm.at[:, pl.ds(128 * c, 128)], xs.at[c], sem_in.at[1 + c])
            for c in range(4)]
    cp_wqkv = pltpu.make_async_copy(wqkv_hbm, wqkv, sem_in.at[5])
    cp_wo = pltpu.make_async_copy(wo_hbm, wo, sem_in.at[6])
    cp_f = pltpu.make_async_copy(f_hbm, fm, sem_in.at[7])
    for c in (cp_fk, *cp_x, cp_wqkv, cp_wo, cp_f):
        c.start()

    for i, r in enumerate((are_ref, aim_ref, bre_ref, bim_ref, cre_ref, cim_ref)):
        par[i] = r[...].astype(F32)
    dt_row = jnp.exp(ldt_ref[...].astype(F32)).astype(BF16).astype(F32)
    dtc[...] = jnp.broadcast_to(dt_row, (128, D)).T
    dsc[...] = jnp.broadcast_to(dsk_ref[...].astype(F32), (128, D)).T

    def kgen8(rows):
        sub = jax.lax.broadcasted_iota(I32, (8, 128), 0)
        slot = (jax.lax.broadcasted_iota(I32, (8, 128), 1) + 1) & 7
        dt = dtc[rows]
        zr, zi = dt * par[0, rows], dt * par[1, rows]
        mag = jnp.exp(zr)
        lam = {1: (mag * jnp.cos(zi), mag * jnp.sin(zi))}
        for p in (2, 4, 8):
            lam[p] = _cmul(lam[p // 2], lam[p // 2])
        mag = jnp.exp(zr * 16.0)
        beta = (mag * jnp.cos(zi * 16.0), mag * jnp.sin(zi * 16.0))
        br = (_flip8(beta[0], sub), _flip8(beta[1], sub))
        rt = [(jnp.ones((8, 128), F32), jnp.zeros((8, 128), F32)), br]
        for b in range(2, 16):
            rt.append(_cmul(rt[b // 2], rt[b - b // 2]))
        g = beta
        for _ in range(4):
            g = _cmul(g, g)
        c0 = _cmul((par[4, rows], par[5, rows]), (dt * par[2, rows], dt * par[3, rows]))
        lt = {(0, 0): c0}
        prev = None
        for a1, r in _ENTRIES:
            if r == 0 and a1 > 0:
                lt[a1, 0] = _cmul(lt[a1 - 1, 0], g)
            elif r > 0:
                lt[a1, r] = _cmul(lt[prev], lam[r - prev[1]])
            prev = (a1, r)
        ls = [lt[e] for e in _ENTRIES]
        ls.append(ls[-1])
        lhs = jnp.concatenate([jnp.concatenate([v[0] for v in ls], axis=0),
                               jnp.concatenate([-v[1] for v in ls], axis=0)], axis=1)
        rhs = jnp.concatenate([jnp.concatenate([v[0] for v in rt], axis=0),
                               jnp.concatenate([v[1] for v in rt], axis=0)], axis=1)
        out = jax.lax.dot_general(lhs.astype(BF16), rhs.astype(BF16), NT,
                                  preferred_element_type=F32)
        piece = {e: pltpu.roll(out[8 * i:8 * i + 8], e[0], 1, stride=1, stride_axis=0)
                 for i, e in enumerate(_ENTRIES)}
        memo = {}

        def merged(a1, j):
            if a1 == 7:
                return piece[7, _R[7][j]]
            key = (a1,) + tuple(_R[a][j] for a in range(a1, 8))
            if key not in memo:
                memo[key] = jnp.where(slot == a1, piece[a1, _R[a1][j]], merged(a1 + 1, j))
            return memo[key]

        return [merged(0, j) for j in range(NJ)]

    @pl.loop(0, D // 16)
    def _(g):
        r0 = pl.multiple_of(g * 16, 16)
        lo = kgen8(pl.ds(r0, 8))
        hi = kgen8(pl.ds(r0 + 8, 8))
        for j in range(NJ):
            xn[j, pl.ds(r0, 16)] = jnp.concatenate([lo[j], hi[j]], axis=0).astype(BF16)

    cp_fk.wait()

    @pl.loop(0, NJ)
    def _(j):
        zs[j] = jnp.dot(xn[j], fk[j], preferred_element_type=F32)

    @pl.loop(0, D // 8)
    def _(g):
        rows = pl.ds(pl.multiple_of(g * 8, 8), 8)
        a = _fft_first([(zs[j, rows, :128], zs[j, rows, 128:]) for j in range(NJ)])
        dsk = dsc[rows]
        for m0 in range(4):
            for m1, (yr, yi) in enumerate(_bfly4(a[m0], False)):
                kf[4 * m0 + m1, rows, :128] = (yr + dsk) * (1.0 / S)
                kf[4 * m0 + m1, rows, 128:] = yi * (1.0 / S)

    cp_wqkv.wait()
    for b in range(12):
        wt[128 * b:128 * b + 128] = jax.lax.dot_general(
            pm_ref[0 if b < 4 else 1], wqkv[:, 128 * b:128 * b + 128], NT,
            preferred_element_type=F32).astype(BF16)
    cp_wo.wait()
    for b in range(4):
        wp = jnp.dot(pm_ref[1], wo[128 * b:128 * b + 128], preferred_element_type=F32)
        wot[:, 128 * b:128 * b + 128] = wp.T.astype(BF16)

    for c in cp_x:
        c.wait()

    @pl.loop(0, NJ // 2)
    def _(j2):
        for c in range(4):
            v = xu[c, pl.ds(j2, NA, stride=NJ // 2), :].T
            xr[2 * j2, 128 * c:128 * c + 128] = pltpu.bitcast(v << 16, F32)
            xr[2 * j2 + 1, 128 * c:128 * c + 128] = pltpu.bitcast(v & np.uint32(0xFFFF0000), F32)

    cp_f.wait()

    @pl.loop(0, 2)
    def _(layer):
        @pl.loop(0, NJ)
        def _(j):
            p, jj = j & 1, j >> 1
            u = _layernorm_t(xr[j]).astype(BF16)
            qkv = jnp.dot(wt[...], u, preferred_element_type=F32)
            qs[j] = qkv[:D]
            k, v = qkv[D:2 * D], qkv[2 * D:]
            ke[p, 8 + jj] = k
            ve[p, 8 + jj] = v
            ke[p, jj] = pltpu.roll(k, 1, 1)
            ve[p, jj] = pltpu.roll(v, 1, 1)

        @pl.loop(0, NJ)
        def _(j):
            p, jj = j & 1, j >> 1
            lane = jax.lax.broadcasted_iota(I32, (8, 128), 1)
            for hg in range(4):
                rows = [pl.ds(128 * hg + 8 * d, 8) for d in range(DH)]
                q = [qs[j, r] for r in rows]
                s = []
                for w in range(WIN):
                    acc = q[0] * ke[p, 8 + jj - w, rows[0]]
                    for d in range(1, DH):
                        acc = acc + q[d] * ke[p, 8 + jj - w, rows[d]]
                    if w:
                        acc = jnp.where(lane * 8 + jj >= w, acc, -1e9)
                    s.append(acc)
                m = s[0]
                for w in range(1, WIN):
                    m = jnp.maximum(m, s[w])
                e = [jnp.exp(a - m) for a in s]
                tot = e[0]
                for w in range(1, WIN):
                    tot = tot + e[w]
                inv = 1.0 / tot
                e = [a * inv for a in e]
                for d in range(0, DH, 2):
                    o = []
                    for r in rows[d:d + 2]:
                        acc = e[0] * ve[p, 8 + jj, r]
                        for w in range(1, WIN):
                            acc = acc + e[w] * ve[p, 8 + jj - w, r]
                        o.append(acc)
                    os_[pl.ds(128 * hg + 8 * d, 16)] = jnp.concatenate(o, axis=0).astype(BF16)
            x = xr[j] + jnp.dot(wot[...], os_[...], preferred_element_type=F32)
            xr[j] = x
            u = _layernorm_t(x).astype(BF16)
            zs[j] = jnp.dot(u, fm[j], preferred_element_type=F32)

        @pl.loop(0, D // 8)
        def _(g):
            rows = pl.ds(pl.multiple_of(g * 8, 8), 8)
            a = _fft_first([(zs[j, rows, :128], zs[j, rows, 128:]) for j in range(NJ)])
            b = []
            for m0 in range(4):
                y = [_cmul(v, (kf[4 * m0 + m1, rows, :128], kf[4 * m0 + m1, rows, 128:]))
                     for m1, v in enumerate(_bfly4(a[m0], False))]
                b.append([_twiddle(v, -j0 * m0) for j0, v in enumerate(_bfly4(y, True))])
            for j0 in range(4):
                for j1, (yr, yi) in enumerate(_bfly4([b[m0][j0] for m0 in range(4)], True)):
                    zs[4 * j1 + j0, rows, :128] = yr
                    zs[4 * j1 + j0, rows, 128:] = yi

        @pl.loop(0, NJ)
        def _(j):
            xr[j] = xr[j] + jax.lax.dot_general(zs[j].astype(BF16), fm[j], NT,
                                                preferred_element_type=F32)

    @pl.loop(0, NJ // 2)
    def _(j2):
        for c in range(4):
            lo = xr[2 * j2, 128 * c:128 * c + 128].astype(BF16).astype(F32)
            hi = xr[2 * j2 + 1, 128 * c:128 * c + 128].astype(BF16).astype(F32)
            v = (pltpu.bitcast(lo, U32) >> 16) | pltpu.bitcast(hi, U32)
            xu[c, pl.ds(j2, NA, stride=NJ // 2), :] = v.T

    cp_o = [pltpu.make_async_copy(xs.at[c], out_hbm.at[:, pl.ds(128 * c, 128)], sem_out.at[c])
            for c in range(4)]
    for c in cp_o:
        c.start()
    for c in cp_o:
        c.wait()


@jax.jit
def pallas_interleave_layers__sliding_local_dilated__ssm_conv_s4__prompt_kernel(
    A_x: jax.Array,
    A_wqkv: jax.Array,
    A_wo: jax.Array,
    B_u: jax.Array,
    B_A_re: jax.Array,
    B_A_im: jax.Array,
    B_B_re: jax.Array,
    B_B_im: jax.Array,
    B_C_re: jax.Array,
    B_C_im: jax.Array,
    B_log_dt: jax.Array,
    B_Dskip: jax.Array,
):
    del B_u
    hbm = pl.BlockSpec(memory_space=pl.ANY)
    vmem = pl.BlockSpec(memory_space=pltpu.VMEM)
    out = pl.pallas_call(
        _kernel,
        in_specs=[hbm] * 5 + [vmem] * 9,
        out_specs=hbm,
        out_shape=jax.ShapeDtypeStruct((S, D), BF16),
        scratch_shapes=[
            pltpu.VMEM((4, S // 2, 128), U32),
            pltpu.VMEM((D, 3 * D), BF16),
            pltpu.VMEM((D, D), BF16),
            pltpu.VMEM((NJ, NA, 256), BF16),
            pltpu.VMEM((NJ, NA, 256), BF16),
            pltpu.VMEM((6, D, 128), F32),
            pltpu.VMEM((D, 128), F32),
            pltpu.VMEM((D, 128), F32),
            pltpu.VMEM((3 * D, D), BF16),
            pltpu.VMEM((D, D), BF16),
            pltpu.VMEM((NJ, D, NA), F32),
            pltpu.VMEM((NJ, D, NA), BF16),
            pltpu.VMEM((NJ, D, NA), F32),
            pltpu.VMEM((2, NJ, D, NA), F32),
            pltpu.VMEM((2, NJ, D, NA), F32),
            pltpu.VMEM((D, NA), BF16),
            pltpu.VMEM((NJ, D, 256), F32),
            pltpu.VMEM((NJ, D, 256), F32),
            pltpu.SemaphoreType.DMA((8,)),
            pltpu.SemaphoreType.DMA((4,)),
        ],
        compiler_params=pltpu.CompilerParams(vmem_limit_bytes=100 << 20),
    )(A_x.reshape(S, D), A_wqkv, A_wo, _F, _FK, _PM,
      B_A_re, B_A_im, B_B_re, B_B_im, B_C_re, B_C_im,
      B_log_dt.reshape(1, D), B_Dskip.reshape(1, D))
    return out.reshape(1, S, D)
```

```python
import math

import jax
import jax.numpy as jnp
import ml_dtypes
import numpy as np
import jax.experimental.pallas as pl
import jax.experimental.pallas.tpu as pltpu

S, D, H, DH, WIN = 2048, 512, 32, 16, 8
NJ, NA = 16, 128
EPS = 1e-5
F32, BF16, U32, I32 = jnp.float32, jnp.bfloat16, jnp.uint32, jnp.int32
NP = 4
LG = 4
K0, K1 = 12, 26
NT = (((1,), (1,)), ((), ()))


def _dft_consts():
    a = np.arange(NA)[None, :, None]
    j = np.arange(NJ)[:, None, None]
    k = np.arange(NA)[None, None, :]
    th = np.pi * (((NJ * a + j) * (2 * k + 1)) % (4 * S)) / (2 * S)
    f = np.concatenate([np.cos(th), -np.sin(th)], axis=-1)
    lane = np.arange(NA)
    ln = (lane - 3) % NA
    fk = f[:, 32 * (ln % 4) + ln // 4, :]
    perm = np.zeros((NA, NA), np.float32)
    perm[lane, (lane % 8) * DH + lane // 8] = 1.0
    il = 16 * (lane // 16) + 8 * (lane % 2) + (lane % 16) // 2
    pm = np.stack([perm * DH ** -0.5, perm, perm[il]])
    bf = ml_dtypes.bfloat16
    return f.astype(bf), fk.astype(bf), pm.astype(bf)


_F, _FK, _PM = _dft_consts()


def _round_l(l):
    return int(np.float32(l).astype(ml_dtypes.bfloat16).astype(np.float32))


_R = [[_round_l(256 * q + j) - 256 * q for j in range(NJ)] for q in range(8)]
assert all(_round_l(256 * q + 16 * b + j) == 256 * q + 16 * b + _R[q][j]
           for q in range(8) for b in range(16) for j in range(NJ))
assert _R[2] == _R[3] and _R[4] == _R[5] == _R[6] == _R[7]
_PAIRS = ([((0, r), (0, r + 8)) for r in range(8)]
          + [((1, 0), (1, 4)), ((1, 8), (1, 12)), ((0, 16), (1, 16))]
          + [((2, r), (3, r)) for r in (0, 8, 16)])


def _cmul(x, y):
    return x[0] * y[0] - x[1] * y[1], x[0] * y[1] + x[1] * y[0]


def _csq(x):
    return x[0] * x[0] - x[1] * x[1], (x[0] + x[0]) * x[1]


def _bfly4(x, inv):
    (ar, ai), (br, bi), (cr, ci), (dr, di) = x
    sr, si, tr, ti = ar + cr, ai + ci, ar - cr, ai - ci
    ur, ui, vr, vi = br + dr, bi + di, br - dr, bi - di
    y1, y3 = (tr + vi, ti - vr), (tr - vi, ti + vr)
    if inv:
        y1, y3 = y3, y1
    return [(sr + ur, si + ui), y1, (sr - ur, si - ui), y3]


def _twiddle(x, e):
    e %= 16
    xr, xi = x
    if e == 0:
        return x
    if e == 4:
        return xi, -xr
    if e == 12:
        return -xi, xr
    c, s = math.cos(math.pi * e / 8), -math.sin(math.pi * e / 8)
    if e % 2 == 0:
        if c * s > 0:
            return (xr - xi) * c, (xr + xi) * c
        return (xr + xi) * c, (xi - xr) * c
    return xr * c - xi * s, xr * s + xi * c


def _half4(p, q, h):
    (pr, pi), (qr, qi) = p, q
    if h:
        return (pr + qi, pi - qr), (pr - qi, pi + qr)
    return (pr + qr, pi + qi), (pr - qr, pi - qi)


def _pk(x):
    return pltpu.bitcast(x.astype(BF16), U32)


def _pk2(a, b):
    return pltpu.pack_elementwise([a, b], packed_dtype=BF16).astype(U32)


def _bf(x):
    return pltpu.bitcast(x, BF16)


def _dot(a, b, dims=(((1,), (0,)), ((), ()))):
    return jax.lax.dot_general(a, b, dims, preferred_element_type=F32)


def _merge(*streams):
    keyed = []
    for n, st in enumerate(streams):
        tot, acc = sum(c for c, _ in st), 0
        for t in st:
            keyed.append(((acc + 0.5 * t[0]) / tot, n, len(keyed), t))
            acc += t[0]
    return [k[-1] for k in sorted(keyed, key=lambda k: k[:3])]


def _flip8(x, sub):
    r = [pltpu.roll(x, k, 0) for k in (7, 5, 3, 1)]
    s4 = sub & 3
    return jnp.where(s4 == 3, r[0], jnp.where(s4 == 2, r[1], jnp.where(s4 == 1, r[2], r[3])))


def _kernel(x_hbm, wqkv_hbm, wo_hbm, f_hbm, fk_hbm, pm_ref,
            are_ref, aim_ref, bre_ref, bim_ref, cre_ref, cim_ref, ldt_ref, dsk_ref,
            out_hbm,
            xu, wqkv, wo, fm, fk, dtc, dsc, wk, kt, wt, wot, xn, xl, os_, xr, qs, ke, ve, kf, zs, zero,
            sem_in, sem_out, sem_b):
    xb = xu.bitcast(BF16)
    cp_x = [pltpu.make_async_copy(x_hbm.at[:, pl.ds(128 * c, 128)], xb.at[c], sem_in.at[c])
            for c in range(4)]
    cp_wqkv = pltpu.make_async_copy(wqkv_hbm, wqkv, sem_in.at[4])
    cp_wo = pltpu.make_async_copy(wo_hbm, wo, sem_in.at[5])
    cp_fk = pltpu.make_async_copy(fk_hbm, fk.bitcast(BF16), sem_in.at[6])
    cp_f = pltpu.make_async_copy(f_hbm, fm.bitcast(BF16), sem_in.at[7])
    cp_o = [pltpu.make_async_copy(xb.at[c], out_hbm.at[:, pl.ds(128 * c, 128)], sem_out.at[c])
            for c in range(4)]
    for c in (cp_wqkv, *cp_x, cp_fk, cp_wo, cp_f):
        c.start()

    for ref in (dtc, dsc, wk, kt, wt, wot, xn, xl, os_, xr, qs, ke, ve, kf, zs):
        ref[(0,) * (len(ref.shape) - 2) + (pl.ds(1, 8), pl.ds(0, 128))] = jnp.zeros((8, 128), ref.dtype)

    zero[pl.ds(1, 16)] = jnp.zeros((16, 128), U32)
    marks, used = [], []

    def mark(x, *_):
        marks.extend(x[r:r + 8, :128] for r in range(0, x.shape[0], 32))

    def pace(vals):
        if len(marks) < LG:
            return vals
        i = len(marks) - LG
        if used and used[-1] == i:
            i += 2
        used.append(i)
        t = pltpu.bitcast(marks[i], U32) & zero[8:16]
        return [pltpu.bitcast(pltpu.bitcast(v, U32) | t, F32) for v in vals]

    def barrier():
        pl.semaphore_signal(sem_b, 1)
        pl.semaphore_wait(sem_b, 1)
        marks[:], used[:] = [], []

    def iota(axis):
        return jax.lax.broadcasted_iota(I32, (8, 128), axis)

    dt_row = jnp.exp(ldt_ref[...].astype(F32).reshape(1, D)).astype(BF16).astype(F32)
    dtc[...] = jnp.broadcast_to(dt_row, (128, D)).T
    dsc[...] = jnp.broadcast_to(dsk_ref[...].astype(F32).reshape(1, D), (128, D)).T

    def k_tables(g):
        st = {}

        def par(ref):
            return ref[16 * (g // 2):16 * (g // 2) + 16].astype(F32)[8 * (g % 2):8 * (g % 2) + 8]

        def mix(u, v):
            lo = iota(0) < 4
            rv = [pltpu.roll(c, 4, 0) for c in v]
            return (tuple(jnp.where(lo, a, b) for a, b in zip(u, rv)),
                    tuple(jnp.where(lo, b, a) for a, b in zip(u, rv)))

        def put(name, t, two):
            kreg.setdefault((name, g, t), []).append(jnp.concatenate(
                [jnp.concatenate([two[0][c], two[1][c]], axis=0).astype(BF16) for c in range(2)],
                axis=1))

        def base():
            dt = dtc[8 * g:8 * g + 8]
            zr, zi = dt * par(are_ref), dt * par(aim_ref)
            mag = jnp.exp(zr)
            st[1] = (mag * jnp.cos(zi), mag * jnp.sin(zi))
            st[0] = _cmul((par(cre_ref), par(cim_ref)), (dt * par(bre_ref), dt * par(bim_ref)))

        def left():
            lam = {1: st[1]}
            for p in range(1, 10):
                lam[2 ** p] = _csq(lam[2 ** (p - 1)])
            st[16] = lam[16]
            e = {(0, 0): st[0]}
            for a1 in (1, 2, 3):
                e[a1, 0] = _cmul(e[a1 - 1, 0], lam[512])
            for a1, r in ((0, 8), (1, 4), (0, 16), (1, 16)):
                e[a1, r] = _cmul(e[a1, 0], lam[r])
            d1, d8 = mix(lam[1], lam[1]), mix(lam[8], lam[8])
            prev, done = None, []
            for i, (u, v) in enumerate(_PAIRS):
                if u in e:
                    cur = mix(e[u], e[v])
                else:
                    m = d1 if i < 8 else d8
                    cur = (_cmul(prev[0], m[0]), _cmul(prev[1], m[1]))
                prev = cur
                done.append(cur)
                if i % 2:
                    for t in range(2):
                        put("l", t, (done[i - 1][t], done[i][t]))

        def right(t):
            lo = iota(0) < 4
            if t == 0:
                f = (_flip8(st[16][0], iota(0)), -_flip8(st[16][1], iota(0)))
                st["d"] = mix(f, f)[::-1]
            d = st["d"][t]
            d2 = _csq(d)
            one = (1.0, 0.0)
            cur = tuple(jnp.where(lo, a, b) for a, b in (zip(one, d), zip(d, d2))[t])
            for v in range(0, 16, 2):
                if v:
                    cur = _cmul(cur, d2)
                nxt = _cmul(cur, d2)
                if t and v == 14:
                    nxt = tuple(jnp.where(lo, a, b) for a, b in zip(nxt, one))
                put("r", t, (cur, nxt))
                cur = nxt

        return [(45, base), (70, left), (35, lambda: right(0)), (30, lambda: right(1))]

    kreg = {}

    def k_matmul(g):
        def mm():
            kreg[g] = [_dot(jnp.concatenate(kreg.pop(("l", g, t)), axis=0),
                            jnp.concatenate(kreg.pop(("r", g, t)), axis=0), NT) for t in range(2)]

        def post():
            o0, o1 = kreg.pop(g)
            lo = iota(0) < 4
            ln = (iota(1) + (NA - 3)) & (NA - 1)
            piece = {}
            for i, (u, v) in enumerate(_PAIRS):
                a, b = o0[8 * i:8 * i + 8], o1[8 * i:8 * i + 8]
                for e, x in ((u, jnp.where(lo, a, b)), (v, pltpu.roll(jnp.where(lo, b, a), 4, 0))):
                    piece[e] = pltpu.roll(x, e[0], 1, stride=1, stride_axis=0)
            memo, res = {}, []
            for j in range(NJ):
                r2, r4, r8 = _R[1][j], _R[2][j], _R[4][j]
                if r8 not in memo:
                    memo[r8] = jnp.where((ln & 3) == 2, piece[2, r8], piece[3, r8])
                if (r4, r8) not in memo:
                    memo[r4, r8] = jnp.where((ln & 3) == 1, piece[1, r4], memo[r8])
                x = piece[0, j] if r2 == j else jnp.where(ln < 64, piece[0, j], piece[0, r2])
                res.append(jnp.where((ln & 3) == 0, x, memo[r4, r8]))
            if g % 2 == 0:
                kreg["even"] = res
            else:
                for j, ev in enumerate(kreg.pop("even")):
                    kt[j, 4 * g - 4:4 * g + 4] = _pk(jnp.concatenate([ev, res[j]], axis=0))

        return [(5, mm)], [(30, post)]

    def k_fft(g):
        def run(h):
            rows = pl.ds(8 * g, 8)
            dsk = dsc[rows]
            for i, xs_ in enumerate(spectrum(rows, h)):
                for m1, (yr, yi) in enumerate(xs_):
                    kf[0, 4 * (h + 2 * i) + m1, rows] = (yr + dsk) * (1.0 / S)
                    kf[1, 4 * (h + 2 * i) + m1, rows] = yi * (1.0 / S)
        return [(20 + 6 * h, lambda h=h: run(h)) for h in range(2)]

    def w_qkv(b):
        def run():
            cols = pl.ds(128 * b, 128)
            for r in range(0, D, 16):
                w = wqkv[r:r + 16, cols].astype(F32)
                wk[r // 2:r // 2 + 8, cols] = _pk2(w[:8], w[8:])
            wt[64 * b:64 * b + 64] = _pk(_dot(pm_ref[0 if b < 4 else 1], _bf(wk[:, cols]), NT))
        return [(128, run)]

    def w_out(b):
        def run():
            wot[:, 128 * b:128 * b + 128] = _pk(_dot(pm_ref[2], wo[128 * b:128 * b + 128]).T)
        return [(128, run)]

    def x_in(j2):
        def run(c):
            v = xu[c, pl.ds(j2, NA, stride=NJ // 2), :].T
            xr[2 * j2, 128 * c:128 * c + 128] = pltpu.bitcast(v << 16, F32)
            xr[2 * j2 + 1, 128 * c:128 * c + 128] = pltpu.bitcast(v & np.uint32(0xFFFF0000), F32)
        return [(40, lambda c=c: run(c)) for c in range(4)]

    def x_out(c, j2):
        def run():
            v = _pk2(xr[2 * j2, 128 * c:128 * c + 128], xr[2 * j2 + 1, 128 * c:128 * c + 128])
            xu[c, pl.ds(j2, NA, stride=NJ // 2), :] = v.T
            if j2 == NJ // 2 - 1:
                cp_o[c].start()
        return [(25, run)]

    def tree(xs_):
        acc = list(xs_[:4])
        for i, x in enumerate(xs_[4:]):
            acc[i % 4] = acc[i % 4] + x
        return jnp.broadcast_to(
            jnp.sum((acc[0] + acc[1]) + (acc[2] + acc[3]), axis=0, keepdims=True), (8, 128))

    def ln(j, lhs=False):
        st = {}

        def mean():
            v = [xr[j, r:r + 8] for r in range(0, D, 8)]
            st["m"] = tree((v[:4] if lhs else pace(v[:4])) + v[4:]) * (1.0 / D)

        def var():
            c = [xr[j, r:r + 8] - st["m"] for r in range(0, D, 8)]
            st["s"] = jax.lax.rsqrt(tree([v * v for v in c]) * (1.0 / D) + EPS)

        def norm():
            for r in range(0, D, 16):
                u = [(xr[j, r + h:r + h + 8] - st["m"]) * st["s"] for h in (0, 8)]
                if lhs:
                    xl[j, r // 2:r // 2 + 8] = _pk(jnp.concatenate(u, axis=0))
                else:
                    xn[j, r // 2:r // 2 + 8] = _pk2(*u)

        return [(18, mean), (50, var), (40, norm)]

    def kv(j):
        p, jj = j & 1, j >> 1

        def run(dst, b):
            k = _dot(_bf(wt[64 * b:64 * b + 64]), _bf(xn[j]))
            mark(k)
            r = pl.ds(128 * (b % 4), 128)
            dst[p, 7 + jj, r] = k
            if jj:
                dst[p, jj - 1, r] = pltpu.roll(k, 1, 1)

        return [(128, lambda b=b: run(ke if b < 8 else ve, b)) for b in range(4, 12)]

    def qproj(j):
        def run(b):
            q = _dot(_bf(wt[64 * b:64 * b + 64]), _bf(xn[j]))
            mark(q)
            qs[j, 128 * b:128 * b + 128] = q
        return [(128, lambda b=b: run(b)) for b in range(4)]

    def core(j):
        p, jj = j & 1, j >> 1
        st = {}

        def probs(hg):
            s = [None] * WIN
            for d in range(DH):
                r = pl.ds(128 * hg + 8 * d, 8)
                q = qs[j, r]
                for w in range(WIN):
                    t = q * ke[p, 7 + jj - w, r]
                    s[w] = t if d == 0 else s[w] + t
            for w in range(jj + 1, WIN):
                s[w] = jnp.where(iota(1) >= 1, s[w], -1e9)
            m = s[0]
            for w in range(1, WIN):
                m = jnp.maximum(m, s[w])
            e = [jnp.exp(a - m) for a in s]
            tot = e[0]
            for w in range(1, WIN):
                tot = tot + e[w]
            inv = 1.0 / tot
            st[hg] = [a * inv for a in e]

        def apply(hg):
            e = st.pop(hg)
            for d in range(0, DH, 2):
                o = []
                for r in (pl.ds(128 * hg + 8 * d, 8), pl.ds(128 * hg + 8 * d + 8, 8)):
                    acc = e[0] * ve[p, 7 + jj, r]
                    for w in range(1, WIN):
                        acc = acc + e[w] * ve[p, 7 + jj - w, r]
                    o.append(acc)
                os_[j, pl.ds(64 * hg + 4 * d, 8)] = _pk2(*o)

        return [t for hg in range(4)
                for t in ((75, lambda hg=hg: probs(hg)), (62, lambda hg=hg: apply(hg)))]

    def wout(j):
        def run(b):
            r = pl.ds(128 * b, 128)
            y = _dot(_bf(wot[64 * b:64 * b + 64]), _bf(os_[j]))
            mark(y)
            xr[j, r] = xr[j, r] + y
        return [(128, lambda b=b: run(b)) for b in range(4)]

    def dft(src, mat, c0, n):
        def run(j):
            a, b = (_dot(_bf(src[i, c0 // 2:(c0 + n) // 2]), _bf(mat[i])) for i in (j, j + 8))
            for i, z in ((j, a + b), (j + 8, a - b)):
                zs[0, i, c0:c0 + n] = z[:, :128]
                zs[1, i, c0:c0 + n] = z[:, 128:]
            mark(z)
        return [(n, lambda j=j: run(j)) for j in range(NJ // 2)]

    def spectrum(rows, h):
        z = [(zs[0, 8 * h + j, rows], zs[1, 8 * h + j, rows]) for j in range(8)]
        pz = pace([c for v in z[:NP] for c in v])
        z[:NP] = list(zip(pz[::2], pz[1::2]))
        a = [_half4(z[j0], z[j0 + 4], h) for j0 in range(4)]
        return [_bfly4([_twiddle(a[j0][i], j0 * (h + 2 * i)) for j0 in range(4)], False)
                for i in range(2)]

    def fft(c0, n):
        def run(r0, h):
            rows = pl.ds(r0, 8)
            b = []
            for i, xs_ in enumerate(spectrum(rows, h)):
                m0 = h + 2 * i
                y = [_cmul(v, (kf[0, 4 * m0 + m1, rows], kf[1, 4 * m0 + m1, rows]))
                     for m1, v in enumerate(xs_)]
                b.append([_twiddle(v, -j0 * m0) for j0, v in enumerate(_bfly4(y, True))])
            for j0 in range(4):
                (ar, ai), (br, bi) = b[0][j0], b[1][j0]
                lo = (ar + br, ai + bi)
                hi = (bi - ai, ar - br) if h else (ar - br, ai - bi)
                for c in range(2):
                    zs[c, 8 * h + j0, rows] = lo[c]
                    zs[c, 8 * h + j0 + 4, rows] = hi[c]
        return [(40 + 12 * h, lambda r0=r0, h=h: run(r0, h))
                for r0 in range(c0, c0 + n, 8) for h in range(2)]

    def inv(c0, n, js):
        def run(j):
            rows = pl.ds(c0, n)
            a, b = (jnp.concatenate([zs[0, i, rows], zs[1, i, rows]], axis=1) for i in (j, j + 8))
            ys = [_dot(z.astype(BF16), _bf(fm[i]), NT) for i, z in ((j, a + b), (j + 8, a - b))]
            for i, y in zip((j, j + 8), ys):
                xr[i, rows] = xr[i, rows] + y
            mark(*ys)
        return [(n, lambda j=j: run(j)) for j in js]

    def cat(lists):
        return [t for l in lists for t in l]

    k_steps = []
    for g in range(-1, 64):
        mm, post = k_matmul(g) if g >= 0 else ([], [])
        tab = k_tables(g + 1) if g + 1 < 64 else []
        k_steps.append(mm + tab[:2] + post + tab[2:])
    k_tail = cat(dft(kt, fk, c, 128) for c in range(0, D, 128))

    order = [2 * (i // 2) + 8 * (i % 2) + p for p in range(2) for i in range(8)]
    G = 128

    def attention(pre):
        steps = [pre[0] + pre[1] + ln(order[0])]
        for i in range(8):
            steps.append(_merge(kv(order[i]) + pre[i + 2], ln(order[i + 1])))
        steps.append(qproj(order[0]))
        for i in range(NJ + 2):
            m, v = [], []
            if i < 6:
                m += pre[i + 10]
            m += _merge(kv(order[8 + i]) if i < 8 else [], qproj(order[i + 1]) if i + 1 < NJ else [],
                        wout(order[i - 1]) if 1 <= i <= NJ else [])
            if i < 7:
                v += ln(order[8 + i + 1])
            if i < NJ:
                v += core(order[i])
            if i >= 2:
                v += ln(order[i - 2], True)
            steps.append(_merge(m, v))
        return steps

    def ssm(tail):
        prog = dft(xl, fm, 0, G) + [(0, barrier)]
        for g in range(4):
            m = dft(xl, fm, G * (g + 1), G) if g < 3 else []
            m = _merge(m, inv(G * (g - 1), G, range(NJ // 2)) if g else [])
            prog += _merge(m, fft(G * g, G), tail(g - 2) if g >= 2 else []) + [(0, barrier)]
        return prog

    def wait(*cps):
        def run():
            for c in cps:
                c.wait()
            marks[:], used[:] = [], []
        return [(0, run)]

    a1 = attention([x_in(j // 2) if j % 2 == 0 else [] for j in order])
    prog = cat(k_steps[:K0]) + wait(cp_wqkv, cp_fk)
    prog += _merge(cat(k_steps[K0:K1]), cat(w_qkv(b) for b in range(12))) + wait(*cp_x, cp_wo, cp_f)
    prog += _merge(cat(k_steps[K1:65]), cat(a1[:9]) + cat(w_out(b) for b in range(4)))
    prog += _merge(k_tail, cat(a1[9:11])) + [(0, barrier)]
    prog += _merge(cat(k_fft(g) for g in range(64)), cat(a1[11:18])) + cat(a1[18:])
    prog += ssm(lambda c: [])
    prog += cat(attention([inv(3 * G, G, [j]) if j < 8 else [] for j in order]))
    prog += ssm(lambda c: cat(x_out(c, j2) for j2 in range(8)))
    prog += inv(3 * G, G, range(NJ // 2)) + cat(x_out(c, j2) for c in (2, 3) for j2 in (0, 4, 1, 5, 2, 6, 3, 7))
    for _, fn in prog:
        fn()
    for c in cp_o:
        c.wait()


@jax.jit
def pallas_interleave_layers__sliding_local_dilated__ssm_conv_s4__prompt_kernel(
    A_x: jax.Array,
    A_wqkv: jax.Array,
    A_wo: jax.Array,
    B_u: jax.Array,
    B_A_re: jax.Array,
    B_A_im: jax.Array,
    B_B_re: jax.Array,
    B_B_im: jax.Array,
    B_C_re: jax.Array,
    B_C_im: jax.Array,
    B_log_dt: jax.Array,
    B_Dskip: jax.Array,
):
    del B_u
    hbm = pl.BlockSpec(memory_space=pl.ANY)
    vmem = pl.BlockSpec(memory_space=pltpu.VMEM)
    out = pl.pallas_call(
        _kernel,
        in_specs=[hbm] * 5 + [vmem] * 9,
        out_specs=hbm,
        out_shape=jax.ShapeDtypeStruct((S, D), BF16),
        scratch_shapes=[
            pltpu.VMEM((4, S // 2, 128), U32),
            pltpu.VMEM((D, 3 * D), BF16),
            pltpu.VMEM((D, D), BF16),
            pltpu.VMEM((NJ, NA // 2, 256), U32),
            pltpu.VMEM((NJ, NA // 2, 256), U32),
            pltpu.VMEM((D, 128), F32),
            pltpu.VMEM((D, 128), F32),
            pltpu.VMEM((D // 2, 3 * D), U32),
            pltpu.VMEM((NJ, D // 2, NA), U32),
            pltpu.VMEM((3 * D // 2, D), U32),
            pltpu.VMEM((D // 2, D), U32),
            pltpu.VMEM((NJ, D // 2, NA), U32),
            pltpu.VMEM((NJ, D // 2, NA), U32),
            pltpu.VMEM((NJ, D // 2, NA), U32),
            pltpu.VMEM((NJ, D, NA), F32),
            pltpu.VMEM((NJ, D, NA), F32),
            pltpu.VMEM((2, NJ - 1, D, NA), F32),
            pltpu.VMEM((2, NJ - 1, D, NA), F32),
            pltpu.VMEM((2, NJ, D, NA), F32),
            pltpu.VMEM((2, NJ, D, NA), F32),
            pltpu.VMEM((24, NA), U32),
            pltpu.SemaphoreType.DMA((8,)),
            pltpu.SemaphoreType.DMA((4,)),
            pltpu.SemaphoreType.REGULAR,
        ],
        compiler_params=pltpu.CompilerParams(vmem_limit_bytes=100 << 20),
    )(A_x.reshape(S, D), A_wqkv, A_wo, _F, _FK, _PM,
      B_A_re, B_A_im, B_B_re, B_B_im, B_C_re, B_C_im,
      B_log_dt, B_Dskip)
    return out.reshape(1, S, D)
```

```python
import math

import jax
import jax.numpy as jnp
import ml_dtypes
import numpy as np
import jax.experimental.pallas as pl
import jax.experimental.pallas.tpu as pltpu

S, D, H, DH, WIN = 2048, 512, 32, 16, 8
NJ, NA = 16, 128
EPS = 1e-5
F32, BF16, U32, I32 = jnp.float32, jnp.bfloat16, jnp.uint32, jnp.int32
NP = 4
LG = 24
P0, K0 = 64, 36
NT = (((1,), (1,)), ((), ()))


def _dft_consts():
    a = np.arange(NA)[None, :, None]
    j = np.arange(NJ)[:, None, None]
    k = np.arange(NA)[None, None, :]
    th = np.pi * (((NJ * a + j) * (2 * k + 1)) % (4 * S)) / (2 * S)
    f = np.concatenate([np.cos(th), -np.sin(th)], axis=-1)
    lane = np.arange(NA)
    ln = (lane - 3) % NA
    fk = f[:, 32 * (ln % 4) + ln // 4, :]
    perm = np.zeros((NA, NA), np.float32)
    perm[lane, (lane % 8) * DH + lane // 8] = 1.0
    il = 16 * (lane // 16) + 8 * (lane % 2) + (lane % 16) // 2
    pm = np.stack([perm * DH ** -0.5, perm, perm[il]])
    bf = ml_dtypes.bfloat16
    return f.astype(bf), fk.astype(bf), pm.astype(bf)


_F, _FK, _PM = _dft_consts()


def _round_l(l):
    return int(np.float32(l).astype(ml_dtypes.bfloat16).astype(np.float32))


_R = [[_round_l(256 * q + j) - 256 * q for j in range(NJ)] for q in range(8)]
assert all(_round_l(256 * q + 16 * b + j) == 256 * q + 16 * b + _R[q][j]
           for q in range(8) for b in range(16) for j in range(NJ))
assert _R[2] == _R[3] and _R[4] == _R[5] == _R[6] == _R[7]
_PAIRS = ([((0, r), (0, r + 8)) for r in range(8)]
          + [((1, 0), (1, 4)), ((1, 8), (1, 12)), ((0, 16), (1, 16))]
          + [((2, r), (3, r)) for r in (0, 8, 16)])


def _cmul(x, y):
    return x[0] * y[0] - x[1] * y[1], x[0] * y[1] + x[1] * y[0]


def _csq(x):
    return x[0] * x[0] - x[1] * x[1], (x[0] + x[0]) * x[1]


def _bfly4(x, inv):
    (ar, ai), (br, bi), (cr, ci), (dr, di) = x
    sr, si, tr, ti = ar + cr, ai + ci, ar - cr, ai - ci
    ur, ui, vr, vi = br + dr, bi + di, br - dr, bi - di
    y1, y3 = (tr + vi, ti - vr), (tr - vi, ti + vr)
    if inv:
        y1, y3 = y3, y1
    return [(sr + ur, si + ui), y1, (sr - ur, si - ui), y3]


def _twiddle(x, e):
    e %= 16
    xr, xi = x
    if e == 0:
        return x
    if e == 4:
        return xi, -xr
    if e == 12:
        return -xi, xr
    c, s = math.cos(math.pi * e / 8), -math.sin(math.pi * e / 8)
    if e % 2 == 0:
        if c * s > 0:
            return (xr - xi) * c, (xr + xi) * c
        return (xr + xi) * c, (xi - xr) * c
    return xr * c - xi * s, xr * s + xi * c


def _half4(p, q, h):
    (pr, pi), (qr, qi) = p, q
    if h:
        return (pr + qi, pi - qr), (pr - qi, pi + qr)
    return (pr + qr, pi + qi), (pr - qr, pi - qi)


def _pk(x):
    return pltpu.bitcast(x.astype(BF16), U32)


def _pk2(a, b):
    return pltpu.pack_elementwise([a, b], packed_dtype=BF16).astype(U32)


def _bf(x):
    return pltpu.bitcast(x, BF16)


def _dot(a, b, dims=(((1,), (0,)), ((), ()))):
    return jax.lax.dot_general(a, b, dims, preferred_element_type=F32)


def _merge(*streams):
    keyed = []
    for n, st in enumerate(streams):
        tot, acc = sum(c for c, _ in st), 0
        for t in st:
            keyed.append(((acc + 0.5 * t[0]) / tot, n, len(keyed), t))
            acc += t[0]
    return [k[-1] for k in sorted(keyed, key=lambda k: k[:3])]


def _flip8(x, sub):
    r = [pltpu.roll(x, k, 0) for k in (7, 5, 3, 1)]
    s4 = sub & 3
    return jnp.where(s4 == 3, r[0], jnp.where(s4 == 2, r[1], jnp.where(s4 == 1, r[2], r[3])))


def _kernel(x_hbm, wqkv_hbm, wo_hbm, f_hbm, fk_hbm,
            are_hbm, aim_hbm, bre_hbm, bim_hbm, cre_hbm, cim_hbm, pm_ref, ldt_ref, dsk_ref,
            out_hbm,
            par_ref, xu, wqkv, wo, fm, fk, dtc, dsc, wk, kt, wt, wot, xn, xl, os_, xr, qs, ke, ve, kf, zs, zero,
            sem_in, sem_out, sem_p, sem_b):
    xb = xu.bitcast(BF16)
    cp_x = [pltpu.make_async_copy(x_hbm.at[:, pl.ds(128 * c, 128)], xb.at[c], sem_in.at[c])
            for c in range(4)]
    cp_wqkv = pltpu.make_async_copy(wqkv_hbm, wqkv, sem_in.at[4])
    cp_wo = pltpu.make_async_copy(wo_hbm, wo, sem_in.at[5])
    cp_fk = pltpu.make_async_copy(fk_hbm, fk.bitcast(BF16), sem_in.at[6])
    cp_f = pltpu.make_async_copy(f_hbm, fm.bitcast(BF16), sem_in.at[7])
    cp_o = [pltpu.make_async_copy(xb.at[c], out_hbm.at[:, pl.ds(128 * c, 128)], sem_out.at[c])
            for c in range(4)]
    cp_p = [[pltpu.make_async_copy(r.at[rows], par_ref.at[i, rows], sem_p.at[6 * h + i])
             for i, r in enumerate((are_hbm, aim_hbm, bre_hbm, bim_hbm, cre_hbm, cim_hbm))]
            for h, rows in enumerate((pl.ds(0, P0), pl.ds(P0, D - P0)))]
    for c in cp_p[0] + cp_p[1]:
        c.start()

    for ref in (dtc, dsc, wk, kt, wt, wot, xn, xl, os_, xr, qs, ke, ve, kf, zs):
        ref[(0,) * (len(ref.shape) - 2) + (pl.ds(1, 8), pl.ds(0, 128))] = jnp.zeros((8, 128), ref.dtype)

    zero[pl.ds(1, 16)] = jnp.zeros((16, 128), U32)
    marks, used, rate = [], [], [1.0]

    def mark(x, *_):
        marks.extend(x[r:r + 8, :128] for r in range(0, x.shape[0], 16) for _ in range(x.shape[1] // 128))

    def pace(vals, cost):
        if not marks:
            return vals
        i = min(max(used + [0, len(marks) - LG]), len(marks) - 1)
        used[:] = [i + cost * rate[0] / 16]
        t = pltpu.bitcast(marks[int(i)], U32) & zero[8:16]
        return [pltpu.bitcast(pltpu.bitcast(v, U32) | t, F32) for v in vals]

    def overlap(m, *vs):
        r = sum(c for c, _ in m) / max(1, sum(c for v in vs for c, _ in v))
        return [(1, lambda: rate.__setitem__(0, r))] + _merge(m, *vs)

    def barrier():
        pl.semaphore_signal(sem_b, 1)
        pl.semaphore_wait(sem_b, 1)
        marks[:], used[:] = [], []

    def iota(axis):
        return jax.lax.broadcasted_iota(I32, (8, 128), axis)

    dt_row = jnp.exp(ldt_ref[...].astype(F32).reshape(1, D)).astype(BF16).astype(F32)
    dtc[...] = jnp.broadcast_to(dt_row, (128, D)).T

    def d_skip():
        dsc[...] = jnp.broadcast_to(dsk_ref[...].astype(F32).reshape(1, D), (128, D)).T

    def k_tables(g):
        st = {}

        def par(i):
            return par_ref[i, 16 * (g // 2):16 * (g // 2) + 16].astype(F32)[8 * (g % 2):8 * (g % 2) + 8]

        def mix(u, v):
            lo = iota(0) < 4
            rv = [pltpu.roll(c, 4, 0) for c in v]
            return (tuple(jnp.where(lo, a, b) for a, b in zip(u, rv)),
                    tuple(jnp.where(lo, b, a) for a, b in zip(u, rv)))

        def put(name, t, two):
            kreg.setdefault((name, g, t), []).append(jnp.concatenate(
                [jnp.concatenate([two[0][c], two[1][c]], axis=0) for c in range(2)], axis=1))

        def base():
            dt, = pace([dtc[8 * g:8 * g + 8]], 45)
            zr, zi = dt * par(0), dt * par(1)
            mag = jnp.exp(zr)
            st[1] = (mag * jnp.cos(zi), mag * jnp.sin(zi))
            st[0] = _cmul((par(4), par(5)), (dt * par(2), dt * par(3)))

        def left():
            lam = {1: tuple(pace(st[1], 70))}
            for p in range(1, 10):
                lam[2 ** p] = _csq(lam[2 ** (p - 1)])
            st[16] = lam[16]
            e = {(0, 0): st[0]}
            for a1 in (1, 2, 3):
                e[a1, 0] = _cmul(e[a1 - 1, 0], lam[512])
            for a1, r in ((0, 8), (1, 4), (0, 16), (1, 16)):
                e[a1, r] = _cmul(e[a1, 0], lam[r])
            d1, d8 = mix(lam[1], lam[1]), mix(lam[8], lam[8])
            prev, done = None, []
            for i, (u, v) in enumerate(_PAIRS):
                if u in e:
                    cur = mix(e[u], e[v])
                else:
                    m = d1 if i < 8 else d8
                    cur = (_cmul(prev[0], m[0]), _cmul(prev[1], m[1]))
                prev = cur
                done.append(cur)
                if i % 2:
                    for t in range(2):
                        put("l", t, (done[i - 1][t], done[i][t]))

        def right(t):
            lo = iota(0) < 4
            if t == 0:
                f = (_flip8(st[16][0], iota(0)), -_flip8(st[16][1], iota(0)))
                st["d"] = mix(f, f)[::-1]
            d = st["d"][t]
            d2 = _csq(d)
            one = (1.0, 0.0)
            cur = tuple(jnp.where(lo, a, b) for a, b in (zip(one, d), zip(d, d2))[t])
            for v in range(0, 16, 2):
                if v:
                    cur = _cmul(cur, d2)
                nxt = _cmul(cur, d2)
                if t and v == 14:
                    nxt = tuple(jnp.where(lo, a, b) for a, b in zip(nxt, one))
                put("r", t, (cur, nxt))
                cur = nxt

        return [(45, base), (70, left), (35, lambda: right(0)), (30, lambda: right(1))]

    kreg = {}

    def k_matmul(g):
        def mm():
            kreg[g] = [_dot(*(jnp.concatenate(kreg.pop((n, g, t)), axis=0).astype(BF16)
                              for n in "lr"), NT) for t in range(2)]

        def post():
            o0, o1 = kreg.pop(g)
            mark(o0)
            lo = iota(0) < 4
            ln = (iota(1) + (NA - 3)) & (NA - 1)
            piece = {}
            for i, (u, v) in enumerate(_PAIRS):
                a, b = o0[8 * i:8 * i + 8], o1[8 * i:8 * i + 8]
                for e, x in ((u, jnp.where(lo, a, b)), (v, pltpu.roll(jnp.where(lo, b, a), 4, 0))):
                    piece[e] = pltpu.roll(x, e[0], 1, stride=1, stride_axis=0)
            memo, res = {}, []
            for j in range(NJ):
                r2, r4, r8 = _R[1][j], _R[2][j], _R[4][j]
                if r8 not in memo:
                    memo[r8] = jnp.where((ln & 3) == 2, piece[2, r8], piece[3, r8])
                if (r4, r8) not in memo:
                    memo[r4, r8] = jnp.where((ln & 3) == 1, piece[1, r4], memo[r8])
                x = piece[0, j] if r2 == j else jnp.where(ln < 64, piece[0, j], piece[0, r2])
                res.append(jnp.where((ln & 3) == 0, x, memo[r4, r8]))
            if g % 2 == 0:
                kreg["even"] = res
            else:
                for j, ev in enumerate(kreg.pop("even")):
                    kt[j, 4 * g - 4:4 * g + 4] = _pk(jnp.concatenate([ev, res[j]], axis=0))

        return [(5, mm)], [(30, post)]

    def k_fft(g):
        def run(h):
            rows = pl.ds(8 * g, 8)
            dsk = dsc[rows]
            for i, xs_ in enumerate(spectrum(rows, h)):
                for m1, (yr, yi) in enumerate(xs_):
                    kf[0, 4 * (h + 2 * i) + m1, rows] = (yr + dsk) * (1.0 / S)
                    kf[1, 4 * (h + 2 * i) + m1, rows] = yi * (1.0 / S)
        return [(20 + 6 * h, lambda h=h: run(h)) for h in range(2)]

    def w_qkv(b):
        def run():
            cols = pl.ds(128 * b, 128)
            for r in range(0, D, 16):
                w = wqkv[r:r + 16, cols].astype(F32)
                wk[r // 2:r // 2 + 8, cols] = _pk2(w[:8], w[8:])
            w = _dot(pm_ref[0 if b < 4 else 1], _bf(wk[:, cols]), NT)
            mark(w)
            wt[64 * b:64 * b + 64] = _pk(w)
        return [(128, run)]

    def w_out(b):
        def run():
            wot[:, 128 * b:128 * b + 128] = _pk(_dot(pm_ref[2], wo[128 * b:128 * b + 128]).T)
        return [(128, run)]

    def x_in(j2):
        def run(c):
            v = xu[c, pl.ds(j2, NA, stride=NJ // 2), :].T
            xr[2 * j2, 128 * c:128 * c + 128] = pltpu.bitcast(v << 16, F32)
            xr[2 * j2 + 1, 128 * c:128 * c + 128] = pltpu.bitcast(v & np.uint32(0xFFFF0000), F32)
        return [(40, lambda c=c: run(c)) for c in range(4)]

    def x_out(c, j2):
        def run():
            v = _pk2(xr[2 * j2, 128 * c:128 * c + 128], xr[2 * j2 + 1, 128 * c:128 * c + 128])
            xu[c, pl.ds(j2, NA, stride=NJ // 2), :] = v.T
            if j2 == NJ // 2 - 1:
                cp_o[c].start()
        return [(25, run)]

    def tree(acc, xs_):
        acc = list(acc)
        for i, x in enumerate(xs_):
            acc[i % 4] = acc[i % 4] + x
        return acc

    def total(acc):
        return jnp.broadcast_to(
            jnp.sum((acc[0] + acc[1]) + (acc[2] + acc[3]), axis=0, keepdims=True), (8, 128))

    def ln(j, lhs=False):
        st = {}

        def mean():
            v = [xr[j, r:r + 8] for r in range(0, D, 8)]
            st["m"] = total(tree(pace(v[:4], 18), v[4:])) * (1.0 / D)

        def var(r0):
            m, = pace([st["m"]], 25)
            c = [xr[j, r:r + 8] - m for r in range(r0, r0 + D // 2, 8)]
            c = [v * v for v in c]
            if r0:
                st["s"] = jax.lax.rsqrt(total(tree(st["v"], c)) * (1.0 / D) + EPS)
            else:
                st["v"] = tree(c[:4], c[4:])

        def norm():
            for r in range(0, D, 16):
                if r % 128 == 0:
                    m, s_ = pace([st["m"], st["s"]], 10)
                u = [(xr[j, r + h:r + h + 8] - m) * s_ for h in (0, 8)]
                if lhs:
                    xl[j, r // 2:r // 2 + 8] = _pk(jnp.concatenate(u, axis=0))
                else:
                    xn[j, r // 2:r // 2 + 8] = _pk2(*u)

        return [(18, mean), (25, lambda: var(0)), (25, lambda: var(D // 2)), (40, norm)]

    def kv(j):
        p, jj = j & 1, j >> 1

        def run(dst, b):
            k = _dot(_bf(wt[64 * b:64 * b + 64]), _bf(xn[j]))
            mark(k)
            r = pl.ds(128 * (b % 4), 128)
            dst[p, 7 + jj, r] = k
            if jj:
                dst[p, jj - 1, r] = pltpu.roll(k, 1, 1)

        return [(128, lambda b=b: run(ke if b < 8 else ve, b)) for b in range(4, 12)]

    def qproj(j):
        def run(b):
            q = _dot(_bf(wt[64 * b:64 * b + 64]), _bf(xn[j]))
            mark(q)
            qs[j, 128 * b:128 * b + 128] = q
        return [(128, lambda b=b: run(b)) for b in range(4)]

    def core(j):
        p, jj = j & 1, j >> 1
        st = {}

        def probs(hg, d0):
            s = st.pop(hg) if d0 else [None] * WIN
            rows = [pl.ds(128 * hg + 8 * d, 8) for d in range(d0, d0 + DH // 2)]
            qv = [qs[j, r] for r in rows]
            for r, q in zip(rows, pace(qv[:4], 16) + pace(qv[4:], 29 if d0 else 17)):
                for w in range(WIN):
                    t = q * ke[p, 7 + jj - w, r]
                    s[w] = t if s[w] is None else s[w] + t
            if not d0:
                st[hg] = s
                return
            for w in range(jj + 1, WIN):
                s[w] = jnp.where(iota(1) >= 1, s[w], -1e9)
            m = s[0]
            for w in range(1, WIN):
                m = jnp.maximum(m, s[w])
            e = [jnp.exp(a - m) for a in s]
            tot = e[0]
            for w in range(1, WIN):
                tot = tot + e[w]
            inv = 1.0 / tot
            st[hg] = [a * inv for a in e]

        def apply(hg, d0):
            e = pace(st.pop(hg) if d0 else st[hg], 32)
            for d in range(d0, d0 + DH // 2, 2):
                o = []
                for r in (pl.ds(128 * hg + 8 * d, 8), pl.ds(128 * hg + 8 * d + 8, 8)):
                    acc = e[0] * ve[p, 7 + jj, r]
                    for w in range(1, WIN):
                        acc = acc + e[w] * ve[p, 7 + jj - w, r]
                    o.append(acc)
                os_[j, pl.ds(64 * hg + 4 * d, 8)] = _pk2(*o)

        return [(c, lambda f=f, hg=hg, d0=d0: f(hg, d0)) for hg in range(4)
                for c, f, d0 in ((33, probs, 0), (45, probs, 8), (32, apply, 0), (32, apply, 8))]

    def wout(j):
        def run(b):
            r = pl.ds(128 * b, 128)
            y = _dot(_bf(wot[64 * b:64 * b + 64]), _bf(os_[j]))
            mark(y)
            xr[j, r] = xr[j, r] + y
        return [(128, lambda b=b: run(b)) for b in range(4)]

    def dft(src, mat, c0, n):
        def run(j):
            a, b = (_dot(_bf(src[i, c0 // 2:(c0 + n) // 2]), _bf(mat[i])) for i in (j, j + 8))
            for i, z in ((j, a + b), (j + 8, a - b)):
                zs[0, i, c0:c0 + n] = z[:, :128]
                zs[1, i, c0:c0 + n] = z[:, 128:]
            mark(z)
        return [(n, lambda j=j: run(j)) for j in range(NJ // 2)]

    def spectrum(rows, h, src=False):
        z = [(zs[0, 8 * h + j, rows], zs[1, 8 * h + j, rows]) for j in range(8)]
        pz = pace([c for v in z[:NP] for c in v], 40 + 12 * h if src else 20 + 6 * h)
        z[:NP] = list(zip(pz[::2], pz[1::2]))
        a = [_half4(z[j0], z[j0 + 4], h) for j0 in range(4)]
        return [_bfly4([_twiddle(a[j0][i], j0 * (h + 2 * i)) for j0 in range(4)], False)
                for i in range(2)]

    def fft(c0, n):
        def run(r0, h):
            rows = pl.ds(r0, 8)
            b = []
            for i, xs_ in enumerate(spectrum(rows, h, True)):
                m0 = h + 2 * i
                y = [_cmul(v, (kf[0, 4 * m0 + m1, rows], kf[1, 4 * m0 + m1, rows]))
                     for m1, v in enumerate(xs_)]
                b.append([_twiddle(v, -j0 * m0) for j0, v in enumerate(_bfly4(y, True))])
            for j0 in range(4):
                (ar, ai), (br, bi) = b[0][j0], b[1][j0]
                lo = (ar + br, ai + bi)
                hi = (bi - ai, ar - br) if h else (ar - br, ai - bi)
                for c in range(2):
                    zs[c, 8 * h + j0, rows] = lo[c]
                    zs[c, 8 * h + j0 + 4, rows] = hi[c]
        return [(40 + 12 * h, lambda r0=r0, h=h: run(r0, h))
                for r0 in range(c0, c0 + n, 8) for h in range(2)]

    def inv(c0, n, js):
        def run(j):
            rows = pl.ds(c0, n)
            a, b = (jnp.concatenate([zs[0, i, rows], zs[1, i, rows]], axis=1) for i in (j, j + 8))
            ys = [_dot(z.astype(BF16), _bf(fm[i]), NT) for i, z in ((j, a + b), (j + 8, a - b))]
            for i, y in zip((j, j + 8), ys):
                xr[i, rows] = xr[i, rows] + y
            mark(*ys)
        return [(n, lambda j=j: run(j)) for j in js]

    def cat(lists):
        return [t for l in lists for t in l]

    k_steps, tab = [], [k_tables(g) for g in range(64)] + [[], [], []]
    for g in range(-2, 64):
        mm, post = k_matmul(g) if g >= 0 else ([], [])
        k_steps.append(mm + tab[g + 1][1:2] + tab[g + 2][:1] + post + tab[g + 1][2:])

    order = [2 * (i // 2) + 8 * (i % 2) + p for p in range(2) for i in range(8)]
    G = 128

    f0, f1 = dft(xl, fm, 0, G), dft(xl, fm, G, G)
    fill = {14: f0[0:1], 15: f0[2:7:2], 16: [f0[1], f0[3], f1[0]], 17: [f0[5], f1[2], f1[4]]}

    def attention(pre):
        steps = [pre[0] + pre[1] + ln(order[0])]
        for i in range(8):
            steps.append(overlap(kv(order[i]) + pre[i + 2], ln(order[i + 1])))
        steps.append(qproj(order[0]))
        for i in range(NJ + 2):
            wo_, ln2 = ([order[n] for n in (2 * k - 1, 2 * k) if 0 <= n < NJ] for k in (i - 8, i - 9))
            m = pre[i + 10] if i < 6 else []
            m = m + _merge(kv(order[8 + i]) if i < 8 else [],
                           qproj(order[i + 1]) if i + 1 < NJ else [], cat(wout(j) for j in wo_))
            m = _merge(m, fill.get(i, []))
            v = (ln(order[8 + i + 1]) if i < 7 else []) + cat(ln(j, True) for j in ln2)
            steps.append(overlap(m, core(order[i]) if i < NJ else [], v))
        return steps + [f0[7:]]

    def ssm(tail):
        prog = [(0, barrier)]
        for g in range(4):
            m = dft(xl, fm, G * (g + 1), G) if g < 3 else []
            if g == 0:
                m = [f1[i] for i in (1, 3, 5, 6, 7)] + dft(xl, fm, 2 * G, G)[:3]
            elif g == 1:
                m = m[3:] + dft(xl, fm, 3 * G, G)[:1]
            elif g == 2:
                m = m[1:]
            m = _merge(m, inv(G * (g - 1), G, range(NJ // 2)) if g else [])
            prog += overlap(m, fft(G * g, G), tail(g - 2) if g >= 2 else []) + [(0, barrier)]
        return prog

    def wait(*cps):
        def run():
            for c in cps:
                c.wait()
            marks[:], used[:] = [], []
        return [(0, run)]

    def start(*cps):
        return [(0, lambda: [c.start() for c in cps])]

    kd = [dft(kt, fk, c, 128) for c in range(0, D, 128)]
    a1 = attention([[]] * NJ)
    head = wait(*cp_p[0]) + cat(k_steps[:P0 // 8]) + wait(*cp_p[1]) + start(cp_wqkv, *cp_x)
    head += cat(k_steps[P0 // 8:K0]) + wait(cp_wqkv) + start(cp_fk, cp_wo, cp_f)
    head += _merge(cat(k_steps[K0:]), cat(w_qkv(b) for b in range(12)))
    head += wait(*cp_x, cp_fk, cp_wo, cp_f) + [(1, d_skip)]
    head += _merge(cat(kd), cat(x_in(j2) for j2 in range(8)) + a1[0])
    head += [(0, barrier)]
    head += _merge(cat(a1[1:11]), cat(k_fft(g) for g in range(64)))
    prog = head + cat(w_out(b) for b in range(4))
    prog += cat(a1[11:]) + ssm(lambda c: [])
    a2 = attention([inv(3 * G, G, [j]) if j < 8 else [] for j in order])
    prog += cat(a2)
    prog += ssm(lambda c: cat(x_out(c, j2) for j2 in range(8)))
    last = inv(3 * G, G, range(NJ // 2))
    prog += _merge(last[:3], cat(x_out(2, j2) for j2 in range(8))) + last[3:]
    prog += cat(x_out(3, j2) for j2 in (0, 4, 1, 5, 2, 6, 3, 7))
    for _, fn in prog:
        fn()
    for c in cp_o:
        c.wait()


@jax.jit
def pallas_interleave_layers__sliding_local_dilated__ssm_conv_s4__prompt_kernel(
    A_x: jax.Array,
    A_wqkv: jax.Array,
    A_wo: jax.Array,
    B_u: jax.Array,
    B_A_re: jax.Array,
    B_A_im: jax.Array,
    B_B_re: jax.Array,
    B_B_im: jax.Array,
    B_C_re: jax.Array,
    B_C_im: jax.Array,
    B_log_dt: jax.Array,
    B_Dskip: jax.Array,
):
    del B_u
    hbm = pl.BlockSpec(memory_space=pl.ANY)
    vmem = pl.BlockSpec(memory_space=pltpu.VMEM)
    out = pl.pallas_call(
        _kernel,
        in_specs=[hbm] * 11 + [vmem] * 3,
        out_specs=hbm,
        out_shape=jax.ShapeDtypeStruct((S, D), BF16),
        scratch_shapes=[
            pltpu.VMEM((6, D, 128), BF16),
            pltpu.VMEM((4, S // 2, 128), U32),
            pltpu.VMEM((D, 3 * D), BF16),
            pltpu.VMEM((D, D), BF16),
            pltpu.VMEM((NJ, NA // 2, 256), U32),
            pltpu.VMEM((NJ, NA // 2, 256), U32),
            pltpu.VMEM((D, 128), F32),
            pltpu.VMEM((D, 128), F32),
            pltpu.VMEM((D // 2, 3 * D), U32),
            pltpu.VMEM((NJ, D // 2, NA), U32),
            pltpu.VMEM((3 * D // 2, D), U32),
            pltpu.VMEM((D // 2, D), U32),
            pltpu.VMEM((NJ, D // 2, NA), U32),
            pltpu.VMEM((NJ, D // 2, NA), U32),
            pltpu.VMEM((NJ, D // 2, NA), U32),
            pltpu.VMEM((NJ, D, NA), F32),
            pltpu.VMEM((NJ, D, NA), F32),
            pltpu.VMEM((2, NJ - 1, D, NA), F32),
            pltpu.VMEM((2, NJ - 1, D, NA), F32),
            pltpu.VMEM((2, NJ, D, NA), F32),
            pltpu.VMEM((2, NJ, D, NA), F32),
            pltpu.VMEM((24, NA), U32),
            pltpu.SemaphoreType.DMA((8,)),
            pltpu.SemaphoreType.DMA((4,)),
            pltpu.SemaphoreType.DMA((12,)),
            pltpu.SemaphoreType.REGULAR,
        ],
        compiler_params=pltpu.CompilerParams(vmem_limit_bytes=100 << 20),
    )(A_x.reshape(S, D), A_wqkv, A_wo, _F, _FK,
      B_A_re, B_A_im, B_B_re, B_B_im, B_C_re, B_C_im,
      _PM, B_log_dt, B_Dskip)
    return out.reshape(1, S, D)
```

```python
import math

import jax
import jax.numpy as jnp
import ml_dtypes
import numpy as np
import jax.experimental.pallas as pl
import jax.experimental.pallas.tpu as pltpu

S, D, H, DH, WIN = 2048, 512, 32, 16, 8
NJ, NA = 16, 128
EPS = 1e-5
F32, BF16, U32, I32 = jnp.float32, jnp.bfloat16, jnp.uint32, jnp.int32
NP = 4
LG, G = 24, 64
SL = 0.5
LATE = ((7, 2), (6, 3), (7, 3))
P0 = 64
NT = (((1,), (1,)), ((), ()))


def _dft_consts():
    a = np.arange(NA)[None, :, None]
    j = np.arange(NJ)[:, None, None]
    k = np.arange(NA)[None, None, :]
    th = np.pi * (((NJ * a + j) * (2 * k + 1)) % (4 * S)) / (2 * S)
    f = np.concatenate([np.cos(th), -np.sin(th)], axis=-1)
    lane = np.arange(NA)
    ln = (lane - 3) % NA
    fk = f[:, 32 * (ln % 4) + ln // 4, :]
    perm = np.zeros((NA, NA), np.float32)
    perm[lane, (lane % 8) * DH + lane // 8] = 1.0
    il = 16 * (lane // 16) + 8 * (lane % 2) + (lane % 16) // 2
    pm = np.stack([perm * DH ** -0.5, perm, perm[il]])
    bf = ml_dtypes.bfloat16
    return f.astype(bf), fk.astype(bf), pm.astype(bf)


_F, _FK, _PM = _dft_consts()


def _round_l(l):
    return int(np.float32(l).astype(ml_dtypes.bfloat16).astype(np.float32))


_R = [[_round_l(256 * q + j) - 256 * q for j in range(NJ)] for q in range(8)]
assert all(_round_l(256 * q + 16 * b + j) == 256 * q + 16 * b + _R[q][j]
           for q in range(8) for b in range(16) for j in range(NJ))
assert _R[2] == _R[3] and _R[4] == _R[5] == _R[6] == _R[7]
_PAIRS = ([((0, r), (0, r + 8)) for r in range(8)]
          + [((1, 0), (1, 4)), ((1, 8), (1, 12)), ((0, 16), (1, 16))]
          + [((2, r), (3, r)) for r in (0, 8, 16)])


def _cmul(x, y):
    return x[0] * y[0] - x[1] * y[1], x[0] * y[1] + x[1] * y[0]


def _csq(x):
    return x[0] * x[0] - x[1] * x[1], (x[0] + x[0]) * x[1]


def _bfly4(x, inv):
    (ar, ai), (br, bi), (cr, ci), (dr, di) = x
    sr, si, tr, ti = ar + cr, ai + ci, ar - cr, ai - ci
    ur, ui, vr, vi = br + dr, bi + di, br - dr, bi - di
    y1, y3 = (tr + vi, ti - vr), (tr - vi, ti + vr)
    if inv:
        y1, y3 = y3, y1
    return [(sr + ur, si + ui), y1, (sr - ur, si - ui), y3]


def _twiddle(x, e):
    e %= 16
    xr, xi = x
    if e == 0:
        return x
    if e == 4:
        return xi, -xr
    if e == 12:
        return -xi, xr
    c, s = math.cos(math.pi * e / 8), -math.sin(math.pi * e / 8)
    if e % 2 == 0:
        if c * s > 0:
            return (xr - xi) * c, (xr + xi) * c
        return (xr + xi) * c, (xi - xr) * c
    return xr * c - xi * s, xr * s + xi * c


def _half4(p, q, h):
    (pr, pi), (qr, qi) = p, q
    if h:
        return (pr + qi, pi - qr), (pr - qi, pi + qr)
    return (pr + qr, pi + qi), (pr - qr, pi - qi)


def _pk(x):
    return pltpu.bitcast(x.astype(BF16), U32)


def _pk2(a, b):
    return pltpu.pack_elementwise([a, b], packed_dtype=BF16).astype(U32)


def _bf(x):
    return pltpu.bitcast(x, BF16)


def _dot(a, b, dims=(((1,), (0,)), ((), ()))):
    return jax.lax.dot_general(a, b, dims, preferred_element_type=F32)


def _merge(*streams):
    keyed = []
    for n, st in enumerate(streams):
        tot, acc = sum(c for c, _ in st) or 1, 0
        for t in st:
            keyed.append(((acc + 0.5 * t[0]) / tot, n, len(keyed), t))
            acc += t[0]
    return [k[-1] for k in sorted(keyed, key=lambda k: k[:3])]


def _flip8(x, sub):
    r = [pltpu.roll(x, k, 0) for k in (7, 5, 3, 1)]
    s4 = sub & 3
    return jnp.where(s4 == 3, r[0], jnp.where(s4 == 2, r[1], jnp.where(s4 == 1, r[2], r[3])))


def _kernel(x_hbm, wqkv_hbm, wo_hbm, f_hbm, fk_hbm,
            are_hbm, aim_hbm, bre_hbm, bim_hbm, cre_hbm, cim_hbm, pm_ref, ldt_ref, dsk_ref,
            out_hbm,
            par_ref, xu, wqkv, wo, fm, fk, dtc, dsc, wk, kt, wt, wot, xn, xl, os_, xr, qs, ke, ve, kf, zs, zero,
            sem_in, sem_out, sem_p, sem_b):
    xb = xu.bitcast(BF16)
    cp_x = [pltpu.make_async_copy(x_hbm.at[:, pl.ds(128 * c, 128)], xb.at[c], sem_in.at[c])
            for c in range(4)]
    cp_wqkv = pltpu.make_async_copy(wqkv_hbm, wqkv, sem_in.at[4])
    cp_wo = pltpu.make_async_copy(wo_hbm, wo, sem_in.at[5])
    cp_fk = pltpu.make_async_copy(fk_hbm, fk.bitcast(BF16), sem_in.at[6])
    cp_f = pltpu.make_async_copy(f_hbm, fm.bitcast(BF16), sem_in.at[7])
    cp_o = [pltpu.make_async_copy(xb.at[c], out_hbm.at[:, pl.ds(128 * c, 128)], sem_out.at[c])
            for c in range(4)]
    cp_p = [[pltpu.make_async_copy(r.at[rows], par_ref.at[i, rows], sem_p.at[6 * h + i])
             for i, r in enumerate((are_hbm, aim_hbm, bre_hbm, bim_hbm, cre_hbm, cim_hbm))]
            for h, rows in enumerate((pl.ds(0, P0), pl.ds(P0, D - P0)))]
    for c in cp_p[0] + cp_p[1]:
        c.start()

    for ref in (dtc, dsc, wk, kt, wt, wot, xn, xl, os_, xr, qs, ke, ve, kf, zs):
        ref[(0,) * (len(ref.shape) - 2) + (pl.ds(1, 8), pl.ds(0, 128))] = jnp.zeros((8, 128), ref.dtype)

    zero[pl.ds(1, 16)] = jnp.zeros((16, 128), U32)
    marks, used, rate = [], [], [1.0]

    def mark(x):
        marks.extend(x[r:r + 8, :128] for r in range(0, x.shape[0], 16) for _ in range(x.shape[1] // 128))

    def pace(vals, cost):
        if not marks:
            return list(vals)
        i = min(max(used + [0, len(marks) - LG]), len(marks) - 1)
        used[:] = [i + cost * rate[0] / 16]
        t = pltpu.bitcast(marks[int(i)], U32) & zero[8:16]
        return [pltpu.bitcast(pltpu.bitcast(v, U32) | t, F32) for v in vals]

    def overlap(m, *vs):
        r = sum(c for c, _ in m) / max(1, sum(c for v in vs for c, _ in v))
        return [(1, lambda: rate.__setitem__(0, r))] + _merge(m, *vs)

    def barrier():
        pl.semaphore_signal(sem_b, 1)
        pl.semaphore_wait(sem_b, 1)
        marks[:], used[:] = [], []

    def iota(axis):
        return jax.lax.broadcasted_iota(I32, (8, 128), axis)

    dt_row = jnp.exp(ldt_ref[...].astype(F32).reshape(1, D)).astype(BF16).astype(F32)
    dtc[...] = jnp.broadcast_to(dt_row, (128, D)).T

    def d_skip():
        dsc[...] = jnp.broadcast_to(dsk_ref[...].astype(F32).reshape(1, D), (128, D)).T

    def k_tables(g):
        st = {}

        def par(i):
            return par_ref[i, 16 * (g // 2):16 * (g // 2) + 16].astype(F32)[8 * (g % 2):8 * (g % 2) + 8]

        def mix(u, v):
            lo = iota(0) < 4
            rv = [pltpu.roll(c, 4, 0) for c in v]
            return (tuple(jnp.where(lo, a, b) for a, b in zip(u, rv)),
                    tuple(jnp.where(lo, b, a) for a, b in zip(u, rv)))

        def put(name, t, two):
            kreg.setdefault((name, g, t), []).append(jnp.concatenate(
                [jnp.concatenate([two[0][c], two[1][c]], axis=0) for c in range(2)], axis=1))

        def base():
            dt, = pace([dtc[8 * g:8 * g + 8]], 100)
            zr, zi = dt * par(0), dt * par(1)
            mag = jnp.exp(zr)
            st[1] = (mag * jnp.cos(zi), mag * jnp.sin(zi))
            st[0] = _cmul((par(4), par(5)), (dt * par(2), dt * par(3)))

        def left():
            lam = {1: st[1]}
            for p in range(1, 10):
                lam[2 ** p] = _csq(lam[2 ** (p - 1)])
            st[16] = lam[16]
            e = {(0, 0): st[0]}
            for a1 in (1, 2, 3):
                e[a1, 0] = _cmul(e[a1 - 1, 0], lam[512])
            for a1, r in ((0, 8), (1, 4), (0, 16), (1, 16)):
                e[a1, r] = _cmul(e[a1, 0], lam[r])
            d1, d8 = mix(lam[1], lam[1]), mix(lam[8], lam[8])
            prev, done = None, []
            for i, (u, v) in enumerate(_PAIRS):
                if u in e:
                    cur = mix(e[u], e[v])
                else:
                    m = d1 if i < 8 else d8
                    cur = (_cmul(prev[0], m[0]), _cmul(prev[1], m[1]))
                prev = cur
                done.append(cur)
                if i % 2:
                    for t in range(2):
                        put("l", t, (done[i - 1][t], done[i][t]))

        def right(t):
            lo = iota(0) < 4
            if t == 0:
                f = (_flip8(st[16][0], iota(0)), -_flip8(st[16][1], iota(0)))
                st["d"] = mix(f, f)[::-1]
            d = st["d"][t]
            d2 = _csq(d)
            one = (1.0, 0.0)
            cur = tuple(jnp.where(lo, a, b) for a, b in (zip(one, d), zip(d, d2))[t])
            for v in range(0, 16, 2):
                if v:
                    cur = _cmul(cur, d2)
                nxt = _cmul(cur, d2)
                if t and v == 14:
                    nxt = tuple(jnp.where(lo, a, b) for a, b in zip(nxt, one))
                put("r", t, (cur, nxt))
                cur = nxt

        return [(45, base), (70, left), (35, lambda: right(0)), (30, lambda: right(1))]

    kreg = {}

    def k_matmul(g):
        def mm():
            kreg[g] = [_dot(*(jnp.concatenate(kreg.pop((n, g, t)), axis=0).astype(BF16)
                              for n in "lr"), NT) for t in range(2)]

        def post():
            o0, o1 = kreg.pop(g)
            mark(o0); mark(o1)
            lo = iota(0) < 4
            ln = (iota(1) + (NA - 3)) & (NA - 1)
            piece = {}
            for i, (u, v) in enumerate(_PAIRS):
                a, b = o0[8 * i:8 * i + 8], o1[8 * i:8 * i + 8]
                for e, x in ((u, jnp.where(lo, a, b)), (v, pltpu.roll(jnp.where(lo, b, a), 4, 0))):
                    piece[e] = pltpu.roll(x, e[0], 1, stride=1, stride_axis=0)
            memo, res = {}, []
            for j in range(NJ):
                r2, r4, r8 = _R[1][j], _R[2][j], _R[4][j]
                if r8 not in memo:
                    memo[r8] = jnp.where((ln & 3) == 2, piece[2, r8], piece[3, r8])
                if (r4, r8) not in memo:
                    memo[r4, r8] = jnp.where((ln & 3) == 1, piece[1, r4], memo[r8])
                x = piece[0, j] if r2 == j else jnp.where(ln < 64, piece[0, j], piece[0, r2])
                res.append(jnp.where((ln & 3) == 0, x, memo[r4, r8]))
            if g % 2 == 0:
                kreg["even"] = res
            else:
                for j, ev in enumerate(kreg.pop("even")):
                    kt[j, 4 * g - 4:4 * g + 4] = _pk(jnp.concatenate([ev, res[j]], axis=0))

        return [(5, mm)], [(30, post)]

    def k_fft(g):
        def run(h):
            rows = pl.ds(8 * g, 8)
            dsk = dsc[rows]
            for i, xs_ in enumerate(spectrum(rows, h, 20 + 6 * h)):
                for m1, (yr, yi) in enumerate(xs_):
                    kf[0, 4 * (h + 2 * i) + m1, rows] = (yr + dsk) * (1.0 / S)
                    kf[1, 4 * (h + 2 * i) + m1, rows] = yi * (1.0 / S)
        return [(20 + 6 * h, lambda h=h: run(h)) for h in range(2)]

    def w_qkv(b):
        def run():
            cols = pl.ds(128 * b, 128)
            for r in range(0, D, 16):
                w = wqkv[r:r + 16, cols].astype(F32)
                wk[r // 2:r // 2 + 8, cols] = _pk2(w[:8], w[8:])
            w = _dot(pm_ref[0 if b < 4 else 1], _bf(wk[:, cols]), NT)
            mark(w)
            wt[64 * b:64 * b + 64] = _pk(w)
        return [(128, run)]

    def w_out(b):
        def run():
            wot[:, 128 * b:128 * b + 128] = _pk(_dot(pm_ref[2], wo[128 * b:128 * b + 128]).T)
        return [(128, run)]

    def x_in(j2):
        def run(c):
            v = xu[c, pl.ds(j2, NA, stride=NJ // 2), :].T
            xr[2 * j2, 128 * c:128 * c + 128] = pltpu.bitcast(v << 16, F32)
            xr[2 * j2 + 1, 128 * c:128 * c + 128] = pltpu.bitcast(v & np.uint32(0xFFFF0000), F32)
        return [(40, lambda c=c: run(c)) for c in range(4)]

    def x_out(c, j2):
        def run():
            v = _pk2(xr[2 * j2, 128 * c:128 * c + 128], xr[2 * j2 + 1, 128 * c:128 * c + 128])
            xu[c, pl.ds(j2, NA, stride=NJ // 2), :] = v.T
            if j2 == NJ // 2 - 1:
                cp_o[c].start()
        return [(25, run)]

    def tree(acc, xs_):
        acc = list(acc)
        for i, x in enumerate(xs_):
            acc[i % 4] = acc[i % 4] + x
        return acc

    def total(acc):
        return jnp.broadcast_to(
            jnp.sum((acc[0] + acc[1]) + (acc[2] + acc[3]), axis=0, keepdims=True), (8, 128))

    def ln(j, lhs=False):
        st = {}

        def mean():
            v = [xr[j, r:r + 8] for r in range(0, D, 8)]
            st["m"] = total(tree(pace(v[:4], 18), v[4:])) * (1.0 / D)

        def var(r0):
            m, = pace([st["m"]], 25)
            c = [xr[j, r:r + 8] - m for r in range(r0, r0 + D // 2, 8)]
            c = [v * v for v in c]
            if r0:
                st["s"] = jax.lax.rsqrt(total(tree(st["v"], c)) * (1.0 / D) + EPS)
            else:
                st["v"] = tree(c[:4], c[4:])

        def norm():
            for r in range(0, D, 16):
                if r % 128 == 0:
                    m, s_ = pace([st["m"], st["s"]], 10)
                u = [(xr[j, r + h:r + h + 8] - m) * s_ for h in (0, 8)]
                if lhs:
                    xl[j, r // 2:r // 2 + 8] = _pk(jnp.concatenate(u, axis=0))
                else:
                    xn[j, r // 2:r // 2 + 8] = _pk2(*u)

        return [(18, mean), (25, lambda: var(0)), (25, lambda: var(D // 2)), (40, norm)]

    def kv(j):
        p, jj = j & 1, j >> 1

        def run(dst, b):
            k = _dot(_bf(wt[64 * b:64 * b + 64]), _bf(xn[j]))
            mark(k)
            r = pl.ds(128 * (b % 4), 128)
            dst[p, 7 + jj, r] = k
            if jj:
                dst[p, jj - 1, r] = pltpu.roll(k, 1, 1)

        return [(128, lambda b=b: run(ke if b < 8 else ve, b)) for b in range(4, 12)]

    def qproj(j):
        def run(b):
            q = _dot(_bf(wt[64 * b:64 * b + 64]), _bf(xn[j]))
            mark(q)
            qs[j, 128 * b:128 * b + 128] = q
        return [(128, lambda b=b: run(b)) for b in range(4)]

    def core(j):
        p, jj = j & 1, j >> 1
        st = {}

        def probs(hg, d0):
            s = st.pop(hg) if d0 else [None] * WIN
            rows = [pl.ds(128 * hg + 8 * d, 8) for d in range(d0, d0 + DH // 2)]
            qv = [qs[j, r] for r in rows]
            for r, q in zip(rows, pace(qv[:4], 16) + pace(qv[4:], 29 if d0 else 17)):
                for w in range(WIN):
                    t = q * ke[p, 7 + jj - w, r]
                    s[w] = t if s[w] is None else s[w] + t
            if not d0:
                st[hg] = s
                return
            for w in range(jj + 1, WIN):
                s[w] = jnp.where(iota(1) >= 1, s[w], -1e9)
            m = s[0]
            for w in range(1, WIN):
                m = jnp.maximum(m, s[w])
            e = [jnp.exp(a - m) for a in s]
            tot = e[0]
            for w in range(1, WIN):
                tot = tot + e[w]
            inv = 1.0 / tot
            st[hg] = [a * inv for a in e]

        def apply(hg, d0):
            e = pace(st.pop(hg) if d0 else st[hg], 32)
            for d in range(d0, d0 + DH // 2, 2):
                o = []
                for r in (pl.ds(128 * hg + 8 * d, 8), pl.ds(128 * hg + 8 * d + 8, 8)):
                    acc = e[0] * ve[p, 7 + jj, r]
                    for w in range(1, WIN):
                        acc = acc + e[w] * ve[p, 7 + jj - w, r]
                    o.append(acc)
                os_[j, pl.ds(64 * hg + 4 * d, 8)] = _pk2(*o)

        return [(c, lambda f=f, hg=hg, d0=d0: f(hg, d0)) for hg in range(4)
                for c, f, d0 in ((33, probs, 0), (45, probs, 8), (32, apply, 0), (32, apply, 8))]

    def wout(j):
        def run(b):
            r = pl.ds(128 * b, 128)
            y = _dot(_bf(wot[64 * b:64 * b + 64]), _bf(os_[j]))
            mark(y)
            xr[j, r] = xr[j, r] + y
        return [(128, lambda b=b: run(b)) for b in range(4)]

    def dft(src, mat, c0, n, more=False):
        def run(j):
            rows = pl.ds(c0, n)
            a, b = (_dot(_bf(src[i, c0 // 2:(c0 + n) // 2]), _bf(mat[i])) for i in (j, j + 8))
            for h, z in enumerate((a + b, a - b)):
                i = 8 * h + j
                res = {i: (z[:, :128], z[:, 128:])}
                if more and 4 <= j < 7:
                    res[i - 4], res[i] = second((zs[0, i - 4, rows], zs[1, i - 4, rows]), res[i], j - 4, h)
                for k, v in res.items():
                    zs[0, k, rows], zs[1, k, rows] = v
            mark(z)
        return [(n, lambda j=j: run(j)) for j in range(NJ // 2)]

    def second(p, q, j0, h):
        return [_twiddle(v, j0 * (h + 2 * i)) for i, v in enumerate(_half4(p, q, h))]

    def spectrum(rows, h, cost, done=0):
        z = [(zs[0, 8 * h + j, rows], zs[1, 8 * h + j, rows]) for j in range(8)]
        paced = (0, 3, 4) if done else (0, 1, 2, 3)
        pz = pace([c for i in paced for c in z[i]], cost)
        for n, i in enumerate(paced):
            z[i] = tuple(pz[2 * n:2 * n + 2])
        a = [(z[j0], z[j0 + 4]) if j0 < done else second(z[j0], z[j0 + 4], j0, h) for j0 in range(4)]
        return [_bfly4([a[j0][i] for j0 in range(4)], False) for i in range(2)]

    def fft(c0, n):
        def run(r0, h):
            rows = pl.ds(r0, 8)
            b = []
            for i, xs_ in enumerate(spectrum(rows, h, 40 + 6 * h, 3)):
                m0 = h + 2 * i
                y = [_cmul(v, (kf[0, 4 * m0 + m1, rows], kf[1, 4 * m0 + m1, rows]))
                     for m1, v in enumerate(xs_)]
                b.append([_twiddle(v, -j0 * m0) for j0, v in enumerate(_bfly4(y, True))])
            for j0 in range(4):
                (ar, ai), (br, bi) = b[0][j0], b[1][j0]
                lo = (ar + br, ai + bi)
                hi = (bi - ai, ar - br) if h else (ar - br, ai - bi)
                for c in range(2):
                    zs[c, 8 * h + j0, rows] = lo[c]
                    zs[c, 8 * h + j0 + 4, rows] = hi[c]
        return [(40 + 6 * h, lambda r0=r0, h=h: run(r0, h))
                for r0 in range(c0, c0 + n, 8) for h in range(2)]

    def inv(c0, n, js):
        def run(j):
            rows = pl.ds(c0, n)
            a, b = (jnp.concatenate([zs[0, i, rows], zs[1, i, rows]], axis=1) for i in (j, j + 8))
            ys = [_dot(z.astype(BF16), _bf(fm[i]), NT) for i, z in ((j, a + b), (j + 8, a - b))]
            for i, y in zip((j, j + 8), ys):
                xr[i, rows] = xr[i, rows] + y
            mark(ys[0])
        return [(n, lambda j=j: run(j)) for j in js]

    def cat(lists):
        return [t for l in lists for t in l]

    k_steps, tab = [], [k_tables(g) for g in range(64)] + [[], [], []]
    for g in range(-2, 64):
        mm, post = k_matmul(g) if g >= 0 else ([], [])
        k_steps.append(mm + tab[g + 1][1:2] + tab[g + 2][:1] + post + tab[g + 1][2:])

    order = [j0 + d for j0 in (0, 2, 1, 3) for d in (0, 8, 4, 12)]

    def lane_dft(n):
        return [dft(xl, fm, c, 128, True)[order[2 * n]] for c in range(0, D, 128)]

    def attention(pre, extra):
        steps = [pre[0] + pre[1] + ln(order[0])]
        for i in range(8):
            steps.append(overlap(kv(order[i]) + pre[i + 2], ln(order[i + 1]), extra[i]))
        steps.append(qproj(order[0]))
        for i in range(NJ + 4):
            wo_, ln2 = ([order[n] for n in (2 * k - 1, 2 * k) if 0 <= n < NJ] for k in (i - 8, i - 9))
            m = pre[i + 10] if i < 6 else []
            m = m + _merge(kv(order[8 + i]) if i < 8 else [],
                           qproj(order[i + 1]) if i + 1 < NJ else [], cat(wout(j) for j in wo_))
            if i >= 12:
                m = _merge(m, [t for c, t in enumerate(lane_dft(i - 12)) if (i - 12, c) not in LATE])
            v = (ln(order[8 + i + 1]) if i < 7 else []) + cat(ln(j, True) for j in ln2)
            c = core(order[i]) if i < NJ else []
            if i >= NJ - 1:
                c, v = (t + [(SL * sum(x for x, _ in t), lambda: None)] for t in (c, v))
            steps.append(overlap(m, c, v))
        return steps

    def ssm(last):
        prog = [(0, barrier)]
        for c in range(0, D, G):
            out = cat(x_out(c // 128 - 1, j2) for j2 in range(8)) if last and c > 128 and c % 128 else []
            prog += overlap(inv(c - G, G, range(NJ // 2)) if c else [lane_dft(n)[b] for n, b in LATE],
                            fft(c, G), out)
            if out and c > 256:
                prog += [(0, barrier)]
        return prog

    def wait(*cps):
        def run():
            for c in cps:
                c.wait()
            marks[:], used[:] = [], []
        return [(0, run)]

    def start(*cps):
        return [(0, lambda: [c.start() for c in cps])]

    kd = [dft(kt, fk, c, 128) for c in range(0, D, 128)]
    a1 = attention([[]] * NJ, [cat(k_fft(g) for g in range(8 * i, 8 * i + 8)) for i in range(8)])
    head = wait(*cp_p[0]) + cat(k_steps[:P0 // 8]) + wait(*cp_p[1]) + start(cp_wqkv, *cp_x, cp_fk, cp_wo, cp_f)
    head += cat(k_steps[P0 // 8:]) + wait(cp_wqkv, *cp_x, cp_fk, cp_wo, cp_f) + [(1, d_skip)]
    head += _merge(_merge(cat(kd), cat(w_qkv(b) for b in range(12))),
                   x_in(0) + a1[0] + cat(x_in(j2) for j2 in range(1, 8)))
    head += [(0, barrier)]
    prog = head + cat(a1[1:11]) + cat(w_out(b) for b in range(4))
    prog += cat(a1[11:]) + ssm(False)
    a2 = attention([inv(D - G, G, [j]) if j < 8 else [] for j in order], [[]] * 8)
    prog += cat(a2)
    prog += ssm(True)
    prog += inv(D - G, G, range(NJ // 2))
    prog += cat(x_out(3, j2) for j2 in (0, 4, 1, 5, 2, 6, 3, 7))
    for _, fn in prog:
        fn()
    for c in cp_o:
        c.wait()


@jax.jit
def pallas_interleave_layers__sliding_local_dilated__ssm_conv_s4__prompt_kernel(
    A_x: jax.Array,
    A_wqkv: jax.Array,
    A_wo: jax.Array,
    B_u: jax.Array,
    B_A_re: jax.Array,
    B_A_im: jax.Array,
    B_B_re: jax.Array,
    B_B_im: jax.Array,
    B_C_re: jax.Array,
    B_C_im: jax.Array,
    B_log_dt: jax.Array,
    B_Dskip: jax.Array,
):
    del B_u
    hbm = pl.BlockSpec(memory_space=pl.ANY)
    vmem = pl.BlockSpec(memory_space=pltpu.VMEM)
    out = pl.pallas_call(
        _kernel,
        in_specs=[hbm] * 11 + [vmem] * 3,
        out_specs=hbm,
        out_shape=jax.ShapeDtypeStruct((S, D), BF16),
        scratch_shapes=[
            pltpu.VMEM((6, D, 128), BF16),
            pltpu.VMEM((4, S // 2, 128), U32),
            pltpu.VMEM((D, 3 * D), BF16),
            pltpu.VMEM((D, D), BF16),
            pltpu.VMEM((NJ, NA // 2, 256), U32),
            pltpu.VMEM((NJ, NA // 2, 256), U32),
            pltpu.VMEM((D, 128), F32),
            pltpu.VMEM((D, 128), F32),
            pltpu.VMEM((D // 2, 3 * D), U32),
            pltpu.VMEM((NJ, D // 2, NA), U32),
            pltpu.VMEM((3 * D // 2, D), U32),
            pltpu.VMEM((D // 2, D), U32),
            pltpu.VMEM((NJ, D // 2, NA), U32),
            pltpu.VMEM((NJ, D // 2, NA), U32),
            pltpu.VMEM((NJ, D // 2, NA), U32),
            pltpu.VMEM((NJ, D, NA), F32),
            pltpu.VMEM((NJ, D, NA), F32),
            pltpu.VMEM((2, NJ - 1, D, NA), F32),
            pltpu.VMEM((2, NJ - 1, D, NA), F32),
            pltpu.VMEM((2, NJ, D, NA), F32),
            pltpu.VMEM((2, NJ, D, NA), F32),
            pltpu.VMEM((24, NA), U32),
            pltpu.SemaphoreType.DMA((8,)),
            pltpu.SemaphoreType.DMA((4,)),
            pltpu.SemaphoreType.DMA((12,)),
            pltpu.SemaphoreType.REGULAR,
        ],
        compiler_params=pltpu.CompilerParams(vmem_limit_bytes=100 << 20),
    )(A_x.reshape(S, D), A_wqkv, A_wo, _F, _FK,
      B_A_re, B_A_im, B_B_re, B_B_im, B_C_re, B_C_im,
      _PM, B_log_dt, B_Dskip)
    return out.reshape(1, S, D)
```

```python
import math

import jax
import jax.numpy as jnp
import ml_dtypes
import numpy as np
import jax.experimental.pallas as pl
import jax.experimental.pallas.tpu as pltpu

S, D, H, DH, WIN = 2048, 512, 32, 16, 8
NJ, NA = 16, 128
EPS = 1e-5
F32, BF16, U32, I32 = jnp.float32, jnp.bfloat16, jnp.uint32, jnp.int32
NP = 4
LG, G = 24, 64
LATE = ((7, 2), (6, 3), (7, 3))
P0 = 80
NT = (((1,), (1,)), ((), ()))


def _dft_consts():
    a = np.arange(NA)[None, :, None]
    j = np.arange(NJ)[:, None, None]
    k = np.arange(NA)[None, None, :]
    th = np.pi * (((NJ * a + j) * (2 * k + 1)) % (4 * S)) / (2 * S)
    f = np.concatenate([np.cos(th), -np.sin(th)], axis=-1)
    lane = np.arange(NA)
    ln = (lane - 3) % NA
    fk = f[:, 32 * (ln % 4) + ln // 4, :]
    perm = np.zeros((NA, NA), np.float32)
    perm[lane, (lane % 8) * DH + lane // 8] = 1.0
    il = 16 * (lane // 16) + 8 * (lane % 2) + (lane % 16) // 2
    pm = np.stack([perm * DH ** -0.5, perm, perm[il]])
    bf = ml_dtypes.bfloat16
    return f.astype(bf), fk.astype(bf), pm.astype(bf)


_F, _FK, _PM = _dft_consts()


def _round_l(l):
    return int(np.float32(l).astype(ml_dtypes.bfloat16).astype(np.float32))


_R = [[_round_l(256 * q + j) - 256 * q for j in range(NJ)] for q in range(8)]
assert all(_round_l(256 * q + 16 * b + j) == 256 * q + 16 * b + _R[q][j]
           for q in range(8) for b in range(16) for j in range(NJ))
assert _R[2] == _R[3] and _R[4] == _R[5] == _R[6] == _R[7]
_PAIRS = ([((0, r), (0, r + 8)) for r in range(8)]
          + [((1, 0), (1, 4)), ((1, 8), (1, 12)), ((0, 16), (1, 16))]
          + [((2, r), (3, r)) for r in (0, 8, 16)])


def _cmul(x, y):
    return x[0] * y[0] - x[1] * y[1], x[0] * y[1] + x[1] * y[0]


def _csq(x):
    return x[0] * x[0] - x[1] * x[1], (x[0] + x[0]) * x[1]


def _bfly4(x, inv):
    (ar, ai), (br, bi), (cr, ci), (dr, di) = x
    sr, si, tr, ti = ar + cr, ai + ci, ar - cr, ai - ci
    ur, ui, vr, vi = br + dr, bi + di, br - dr, bi - di
    y1, y3 = (tr + vi, ti - vr), (tr - vi, ti + vr)
    if inv:
        y1, y3 = y3, y1
    return [(sr + ur, si + ui), y1, (sr - ur, si - ui), y3]


def _twiddle(x, e):
    e %= 16
    xr, xi = x
    if e == 0:
        return x
    if e == 4:
        return xi, -xr
    if e == 12:
        return -xi, xr
    c, s = math.cos(math.pi * e / 8), -math.sin(math.pi * e / 8)
    if e % 2 == 0:
        if c * s > 0:
            return (xr - xi) * c, (xr + xi) * c
        return (xr + xi) * c, (xi - xr) * c
    return xr * c - xi * s, xr * s + xi * c


def _half4(p, q, h):
    (pr, pi), (qr, qi) = p, q
    if h:
        return (pr + qi, pi - qr), (pr - qi, pi + qr)
    return (pr + qr, pi + qi), (pr - qr, pi - qi)


def _pk(x):
    return pltpu.bitcast(x.astype(BF16), U32)


def _pk2(a, b):
    return pltpu.pack_elementwise([a, b], packed_dtype=BF16).astype(U32)


def _bf(x):
    return pltpu.bitcast(x, BF16)


def _dot(a, b, dims=(((1,), (0,)), ((), ()))):
    return jax.lax.dot_general(a, b, dims, preferred_element_type=F32)


def _merge(*streams):
    keyed = []
    for n, st in enumerate(streams):
        tot, acc = sum(c for c, _ in st) or 1, 0
        for t in st:
            keyed.append(((acc + 0.5 * t[0]) / tot, n, len(keyed), t))
            acc += t[0]
    return [k[-1] for k in sorted(keyed, key=lambda k: k[:3])]


def _flip8(x, sub):
    r = [pltpu.roll(x, k, 0) for k in (7, 5, 3, 1)]
    s4 = sub & 3
    return jnp.where(s4 == 3, r[0], jnp.where(s4 == 2, r[1], jnp.where(s4 == 1, r[2], r[3])))


def _kernel(x_hbm, wqkv_hbm, wo_hbm, f_hbm, fk_hbm,
            are_hbm, aim_hbm, bre_hbm, bim_hbm, cre_hbm, cim_hbm, pm_hbm, ldt_hbm, dsk_hbm,
            out_hbm,
            pm_ref, ldt_ref, dsk_ref, par_ref, xu, wqkv, wo, fm, fk, dtc, dsc, wk, kt, wt, wot, xn, xl, os_, xr, qs, ke, ve, kf, zs, zero,
            sem_in, sem_out, sem_p, sem_b):
    xb = xu.bitcast(BF16)
    cp_x = [pltpu.make_async_copy(x_hbm.at[:, pl.ds(128 * c, 128)], xb.at[c], sem_in.at[c])
            for c in range(4)]
    cp_wqkv = pltpu.make_async_copy(wqkv_hbm, wqkv, sem_in.at[4])
    cp_wo = pltpu.make_async_copy(wo_hbm, wo, sem_in.at[5])
    cp_fk = pltpu.make_async_copy(fk_hbm, fk.bitcast(BF16), sem_in.at[6])
    cp_f = pltpu.make_async_copy(f_hbm, fm.bitcast(BF16), sem_in.at[7])
    cp_o = [pltpu.make_async_copy(xb.at[c], out_hbm.at[:, pl.ds(128 * c, 128)], sem_out.at[c])
            for c in range(4)]
    cp_p = [[pltpu.make_async_copy(r.at[rows], par_ref.at[i, rows], sem_p.at[6 * h + i])
             for i, r in enumerate((are_hbm, aim_hbm, bre_hbm, bim_hbm, cre_hbm, cim_hbm))]
            for h, rows in enumerate((pl.ds(0, P0), pl.ds(P0, D - P0)))]
    cp_s = [pltpu.make_async_copy(a, b, sem_p.at[12 + i])
            for i, (a, b) in enumerate(((ldt_hbm, ldt_ref), (dsk_hbm, dsk_ref), (pm_hbm, pm_ref)))]
    cp_p = [cp_s[:1] + cp_p[0], cp_p[1] + cp_s[1:]]
    for c in cp_p[0] + cp_p[1]:
        c.start()

    for ref in (dtc, dsc, wk, kt, wt, wot, xn, xl, os_, xr, qs, ke, ve, kf, zs):
        ref[(0,) * (len(ref.shape) - 2) + (pl.ds(1, 8), pl.ds(0, 128))] = jnp.zeros((8, 128), ref.dtype)

    zero[pl.ds(1, 16)] = jnp.zeros((16, 128), U32)
    marks, used, rate = [], [], [1.0]

    def mark(x):
        marks.extend(x[r:r + 8, :128] for r in range(0, x.shape[0], 16) for _ in range(x.shape[1] // 128))

    def pace(vals, cost):
        if not marks:
            return list(vals)
        i = min(max(used + [0, len(marks) - LG]), len(marks) - 1)
        used[:] = [i + cost * rate[0] / 16]
        t = pltpu.bitcast(marks[int(i)], U32) & zero[8:16]
        return [pltpu.bitcast(pltpu.bitcast(v, U32) | t, F32) for v in vals]

    def overlap(m, *vs):
        r = sum(c for c, _ in m) / max(1, sum(c for v in vs for c, _ in v))
        return [(1, lambda: rate.__setitem__(0, r))] + _merge(m, *vs)

    def barrier():
        pl.semaphore_signal(sem_b, 1)
        pl.semaphore_wait(sem_b, 1)
        marks[:], used[:] = [], []

    def iota(axis):
        return jax.lax.broadcasted_iota(I32, (8, 128), axis)

    def step_size():
        dt_row = jnp.exp(ldt_ref[...].astype(F32).reshape(1, D)).astype(BF16).astype(F32)
        dtc[...] = jnp.broadcast_to(dt_row, (128, D)).T

    def d_skip():
        dsc[...] = jnp.broadcast_to(dsk_ref[...].astype(F32).reshape(1, D), (128, D)).T

    def k_tables(g):
        st = {}

        def par(i):
            return par_ref[i, 16 * (g // 2):16 * (g // 2) + 16].astype(F32)[8 * (g % 2):8 * (g % 2) + 8]

        def mix(u, v):
            lo = iota(0) < 4
            rv = [pltpu.roll(c, 4, 0) for c in v]
            return (tuple(jnp.where(lo, a, b) for a, b in zip(u, rv)),
                    tuple(jnp.where(lo, b, a) for a, b in zip(u, rv)))

        def put(name, t, two):
            kreg.setdefault((name, g, t), []).append(jnp.concatenate(
                [jnp.concatenate([two[0][c], two[1][c]], axis=0) for c in range(2)], axis=1))

        def base():
            dt, = pace([dtc[8 * g:8 * g + 8]], 100)
            zr, zi = dt * par(0), dt * par(1)
            mag = jnp.exp(zr)
            st[1] = (mag * jnp.cos(zi), mag * jnp.sin(zi))
            st[0] = _cmul((par(4), par(5)), (dt * par(2), dt * par(3)))

        def left():
            lam = {1: st[1]}
            for p in range(1, 10):
                lam[2 ** p] = _csq(lam[2 ** (p - 1)])
            st[16] = lam[16]
            e = {(0, 0): st[0]}
            for a1 in (1, 2, 3):
                e[a1, 0] = _cmul(e[a1 - 1, 0], lam[512])
            for a1, r in ((0, 8), (1, 4), (0, 16), (1, 16)):
                e[a1, r] = _cmul(e[a1, 0], lam[r])
            d1, d8 = mix(lam[1], lam[1]), mix(lam[8], lam[8])
            prev, done = None, []
            for i, (u, v) in enumerate(_PAIRS):
                if u in e:
                    cur = mix(e[u], e[v])
                else:
                    m = d1 if i < 8 else d8
                    cur = (_cmul(prev[0], m[0]), _cmul(prev[1], m[1]))
                prev = cur
                done.append(cur)
                if i % 2:
                    for t in range(2):
                        put("l", t, (done[i - 1][t], done[i][t]))

        def right(t):
            lo = iota(0) < 4
            if t == 0:
                f = (_flip8(st[16][0], iota(0)), -_flip8(st[16][1], iota(0)))
                st["d"] = mix(f, f)[::-1]
            d = st["d"][t]
            d2 = _csq(d)
            one = (1.0, 0.0)
            cur = tuple(jnp.where(lo, a, b) for a, b in (zip(one, d), zip(d, d2))[t])
            for v in range(0, 16, 2):
                if v:
                    cur = _cmul(cur, d2)
                nxt = _cmul(cur, d2)
                if t and v == 14:
                    nxt = tuple(jnp.where(lo, a, b) for a, b in zip(nxt, one))
                put("r", t, (cur, nxt))
                cur = nxt

        return [(45, base), (70, left), (35, lambda: right(0)), (30, lambda: right(1))]

    kreg = {}

    def k_matmul(g):
        def mm():
            kreg[g] = [_dot(*(jnp.concatenate(kreg.pop((n, g, t)), axis=0).astype(BF16)
                              for n in "lr"), NT) for t in range(2)]

        def post():
            o0, o1 = kreg.pop(g)
            mark(o0); mark(o1)
            lo = iota(0) < 4
            ln = (iota(1) + (NA - 3)) & (NA - 1)
            piece = {}
            for i, (u, v) in enumerate(_PAIRS):
                a, b = o0[8 * i:8 * i + 8], o1[8 * i:8 * i + 8]
                for e, x in ((u, jnp.where(lo, a, b)), (v, pltpu.roll(jnp.where(lo, b, a), 4, 0))):
                    piece[e] = pltpu.roll(x, e[0], 1, stride=1, stride_axis=0)
            memo, res = {}, []
            for j in range(NJ):
                r2, r4, r8 = _R[1][j], _R[2][j], _R[4][j]
                if r8 not in memo:
                    memo[r8] = jnp.where((ln & 3) == 2, piece[2, r8], piece[3, r8])
                if (r4, r8) not in memo:
                    memo[r4, r8] = jnp.where((ln & 3) == 1, piece[1, r4], memo[r8])
                x = piece[0, j] if r2 == j else jnp.where(ln < 64, piece[0, j], piece[0, r2])
                res.append(jnp.where((ln & 3) == 0, x, memo[r4, r8]))
            if g % 2 == 0:
                kreg["even"] = res
            else:
                for j, ev in enumerate(kreg.pop("even")):
                    kt[j, 4 * g - 4:4 * g + 4] = _pk(jnp.concatenate([ev, res[j]], axis=0))

        return [(5, mm)], [(30, post)]

    def k_fft(g):
        def run(h):
            rows = pl.ds(8 * g, 8)
            dsk = dsc[rows]
            for i, xs_ in enumerate(spectrum(rows, h, 20 + 6 * h)):
                for m1, (yr, yi) in enumerate(xs_):
                    kf[0, 4 * (h + 2 * i) + m1, rows] = (yr + dsk) * (1.0 / S)
                    kf[1, 4 * (h + 2 * i) + m1, rows] = yi * (1.0 / S)
        return [(20 + 6 * h, lambda h=h: run(h)) for h in range(2)]

    def w_qkv(b):
        def run():
            cols = pl.ds(128 * b, 128)
            for r in range(0, D, 16):
                w = wqkv[r:r + 16, cols].astype(F32)
                wk[r // 2:r // 2 + 8, cols] = _pk2(w[:8], w[8:])
            w = _dot(pm_ref[0 if b < 4 else 1], _bf(wk[:, cols]), NT)
            mark(w)
            wt[64 * b:64 * b + 64] = _pk(w)
        return [(128, run)]

    def w_out(b):
        def run():
            wot[:, 128 * b:128 * b + 128] = _pk(_dot(pm_ref[2], wo[128 * b:128 * b + 128]).T)
        return [(128, run)]

    def x_in(j2):
        def run(c):
            v = xu[c, pl.ds(j2, NA, stride=NJ // 2), :].T
            xr[2 * j2, 128 * c:128 * c + 128] = pltpu.bitcast(v << 16, F32)
            xr[2 * j2 + 1, 128 * c:128 * c + 128] = pltpu.bitcast(v & np.uint32(0xFFFF0000), F32)
        return [(40, lambda c=c: run(c)) for c in range(4)]

    def x_out(c, j2):
        def run():
            v = _pk2(xr[2 * j2, 128 * c:128 * c + 128], xr[2 * j2 + 1, 128 * c:128 * c + 128])
            xu[c, pl.ds(j2, NA, stride=NJ // 2), :] = v.T
            if j2 == NJ // 2 - 1:
                cp_o[c].start()
        return [(25, run)]

    def tree(acc, xs_):
        acc = list(acc)
        for i, x in enumerate(xs_):
            acc[i % 4] = acc[i % 4] + x
        return acc

    def total(acc):
        return jnp.broadcast_to(
            jnp.sum((acc[0] + acc[1]) + (acc[2] + acc[3]), axis=0, keepdims=True), (8, 128))

    def ln(j, lhs=False):
        st = {}

        def mean():
            v = [xr[j, r:r + 8] for r in range(0, D, 8)]
            st["m"] = total(tree(pace(v[:4], 18), v[4:])) * (1.0 / D)

        def var(r0):
            m, = pace([st["m"]], 25)
            c = [xr[j, r:r + 8] - m for r in range(r0, r0 + D // 2, 8)]
            c = [v * v for v in c]
            if r0:
                st["s"] = jax.lax.rsqrt(total(tree(st["v"], c)) * (1.0 / D) + EPS)
            else:
                st["v"] = tree(c[:4], c[4:])

        def norm():
            for r in range(0, D, 16):
                if r % 128 == 0:
                    m, s_ = pace([st["m"], st["s"]], 10)
                u = [(xr[j, r + h:r + h + 8] - m) * s_ for h in (0, 8)]
                if lhs:
                    xl[j, r // 2:r // 2 + 8] = _pk(jnp.concatenate(u, axis=0))
                else:
                    xn[j, r // 2:r // 2 + 8] = _pk2(*u)

        return [(18, mean), (25, lambda: var(0)), (25, lambda: var(D // 2)), (40, norm)]

    def kv(j):
        p, jj = j & 1, j >> 1

        def run(dst, b):
            k = _dot(_bf(wt[64 * b:64 * b + 64]), _bf(xn[j]))
            mark(k)
            r = pl.ds(128 * (b % 4), 128)
            dst[p, 7 + jj, r] = k
            if jj:
                dst[p, jj - 1, r] = pltpu.roll(k, 1, 1)

        return [(128, lambda b=b: run(ke if b < 8 else ve, b)) for b in range(4, 12)]

    def qproj(j):
        def run(b):
            q = _dot(_bf(wt[64 * b:64 * b + 64]), _bf(xn[j]))
            mark(q)
            qs[j, 128 * b:128 * b + 128] = q
        return [(128, lambda b=b: run(b)) for b in range(4)]

    def core(j):
        p, jj = j & 1, j >> 1
        st = {}

        def probs(hg, d0):
            s = st.pop(hg) if d0 else [None] * WIN
            rows = [pl.ds(128 * hg + 8 * d, 8) for d in range(d0, d0 + DH // 2)]
            qv = [qs[j, r] for r in rows]
            for r, q in zip(rows, pace(qv[:4], 16) + pace(qv[4:], 29 if d0 else 17)):
                for w in range(WIN):
                    t = q * ke[p, 7 + jj - w, r]
                    s[w] = t if s[w] is None else s[w] + t
            if not d0:
                st[hg] = s
                return
            for w in range(jj + 1, WIN):
                s[w] = jnp.where(iota(1) >= 1, s[w], -1e9)
            m = s[0]
            for w in range(1, WIN):
                m = jnp.maximum(m, s[w])
            e = [jnp.exp(a - m) for a in s]
            tot = e[0]
            for w in range(1, WIN):
                tot = tot + e[w]
            inv = 1.0 / tot
            st[hg] = [a * inv for a in e]

        def apply(hg, d0):
            e = pace(st.pop(hg) if d0 else st[hg], 32)
            for d in range(d0, d0 + DH // 2, 2):
                o = []
                for r in (pl.ds(128 * hg + 8 * d, 8), pl.ds(128 * hg + 8 * d + 8, 8)):
                    acc = e[0] * ve[p, 7 + jj, r]
                    for w in range(1, WIN):
                        acc = acc + e[w] * ve[p, 7 + jj - w, r]
                    o.append(acc)
                os_[j, pl.ds(64 * hg + 4 * d, 8)] = _pk2(*o)

        return [(c, lambda f=f, hg=hg, d0=d0: f(hg, d0)) for hg in range(4)
                for c, f, d0 in ((33, probs, 0), (45, probs, 8), (32, apply, 0), (32, apply, 8))]

    def wout(j):
        def run(b):
            r = pl.ds(128 * b, 128)
            y = _dot(_bf(wot[64 * b:64 * b + 64]), _bf(os_[j]))
            mark(y)
            xr[j, r] = xr[j, r] + y
        return [(128, lambda b=b: run(b)) for b in range(4)]

    def dft(src, mat, c0, n, more=False):
        def run(j):
            rows = pl.ds(c0, n)
            a, b = (_dot(_bf(src[i, c0 // 2:(c0 + n) // 2]), _bf(mat[i])) for i in (j, j + 8))
            for h, z in enumerate((a + b, a - b)):
                i = 8 * h + j
                res = {i: (z[:, :128], z[:, 128:])}
                if more and 4 <= j < 7:
                    res[i - 4], res[i] = second((zs[0, i - 4, rows], zs[1, i - 4, rows]), res[i], j - 4, h)
                for k, v in res.items():
                    zs[0, k, rows], zs[1, k, rows] = v
            mark(z)
        return [(n, lambda j=j: run(j)) for j in range(NJ // 2)]

    def second(p, q, j0, h):
        return [_twiddle(v, j0 * (h + 2 * i)) for i, v in enumerate(_half4(p, q, h))]

    def spectrum(rows, h, cost, done=0):
        z = [(zs[0, 8 * h + j, rows], zs[1, 8 * h + j, rows]) for j in range(8)]
        paced = (0, 3, 4) if done else (0, 1, 2, 3)
        pz = pace([c for i in paced for c in z[i]], cost)
        for n, i in enumerate(paced):
            z[i] = tuple(pz[2 * n:2 * n + 2])
        a = [(z[j0], z[j0 + 4]) if j0 < done else second(z[j0], z[j0 + 4], j0, h) for j0 in range(4)]
        return [_bfly4([a[j0][i] for j0 in range(4)], False) for i in range(2)]

    def fft(c0, n):
        def run(r0, h):
            rows = pl.ds(r0, 8)
            b = []
            for i, xs_ in enumerate(spectrum(rows, h, 40 + 6 * h, 3)):
                m0 = h + 2 * i
                y = [_cmul(v, (kf[0, 4 * m0 + m1, rows], kf[1, 4 * m0 + m1, rows]))
                     for m1, v in enumerate(xs_)]
                b.append([_twiddle(v, -j0 * m0) for j0, v in enumerate(_bfly4(y, True))])
            for j0 in range(4):
                (ar, ai), (br, bi) = b[0][j0], b[1][j0]
                lo = (ar + br, ai + bi)
                hi = (bi - ai, ar - br) if h else (ar - br, ai - bi)
                for c in range(2):
                    zs[c, 8 * h + j0, rows] = lo[c]
                    zs[c, 8 * h + j0 + 4, rows] = hi[c]
        return [(40 + 6 * h, lambda r0=r0, h=h: run(r0, h))
                for r0 in range(c0, c0 + n, 8) for h in range(2)]

    def inv(c0, n, js):
        def run(j):
            rows = pl.ds(c0, n)
            a, b = (jnp.concatenate([zs[0, i, rows], zs[1, i, rows]], axis=1) for i in (j, j + 8))
            ys = [_dot(z.astype(BF16), _bf(fm[i]), NT) for i, z in ((j, a + b), (j + 8, a - b))]
            for i, y in zip((j, j + 8), ys):
                xr[i, rows] = xr[i, rows] + y
            mark(ys[0])
        return [(n, lambda j=j: run(j)) for j in js]

    def cat(lists):
        return [t for l in lists for t in l]

    k_steps, tab = [], [k_tables(g) for g in range(64)] + [[], [], []]
    for g in range(-2, 64):
        mm, post = k_matmul(g) if g >= 0 else ([], [])
        k_steps.append(mm + tab[g + 1][1:2] + tab[g + 2][:1] + post + tab[g + 1][2:])

    order = [j0 + d for j0 in (0, 2, 1, 3) for d in (0, 8, 4, 12)]

    def lane_dft(n):
        return [dft(xl, fm, c, 128, True)[order[2 * n]] for c in range(0, D, 128)]

    def attention(pre, extra):
        steps = [pre[0] + pre[1] + ln(order[0])]
        for i in range(8):
            steps.append(overlap(kv(order[i]) + pre[i + 2], ln(order[i + 1]), extra[i]))
        steps.append(qproj(order[0]))
        for i in range(NJ + 4):
            wo_, ln2 = ([order[n] for n in (2 * k - 1, 2 * k) if 0 <= n < NJ] for k in (i - 8, i - 9))
            m = pre[i + 10] if i < 6 else []
            m = m + _merge(kv(order[8 + i]) if i < 8 else [],
                           qproj(order[i + 1]) if i + 1 < NJ else [], cat(wout(j) for j in wo_))
            if i >= 12:
                m = _merge(m, [t for c, t in enumerate(lane_dft(i - 12)) if (i - 12, c) not in LATE])
            v = (ln(order[8 + i + 1]) if i < 7 else []) + cat(ln(j, True) for j in ln2)
            c = core(order[i]) if i < NJ else []
            if i >= NJ - 1:
                c, v = (t + [(0.5 * sum(x for x, _ in t), lambda: None)] for t in (c, v))
            steps.append(overlap(m, c, v))
        return steps

    def ssm(last):
        prog = [(0, barrier)]
        for c in range(0, D, G):
            out = cat(x_out(c // 128 - 1, j2) for j2 in range(8)) if last and c > 128 and c % 128 else []
            prog += overlap(inv(c - G, G, range(NJ // 2)) if c else [lane_dft(n)[b] for n, b in LATE],
                            fft(c, G), out)
            if out and c > 256:
                prog += [(0, barrier)]
        return prog

    def wait(*cps):
        def run():
            for c in cps:
                c.wait()
            marks[:], used[:] = [], []
        return [(0, run)]

    def start(*cps):
        return [(0, lambda: [c.start() for c in cps])]

    kd = [dft(kt, fk, c, 128) for c in range(0, D, 128)]
    a1 = attention([[]] * NJ, [cat(k_fft(g) for g in range(8 * i, 8 * i + 8)) for i in range(8)])
    head = wait(*cp_p[0]) + [(1, step_size)] + cat(k_steps[:P0 // 8]) + wait(*cp_p[1]) + start(cp_wqkv, *cp_x, cp_fk)
    head += cat(k_steps[P0 // 8:]) + wait(cp_wqkv, *cp_x, cp_fk) + start(cp_wo, cp_f) + [(1, d_skip)]
    head += _merge(_merge(cat(kd), cat(w_qkv(b) for b in range(12))),
                   x_in(0) + a1[0] + cat(x_in(j2) for j2 in range(1, 8)))
    head += wait(cp_wo, cp_f)
    prog = head + cat(a1[1:11]) + cat(w_out(b) for b in range(4))
    prog += cat(a1[11:]) + ssm(False)
    a2 = attention([inv(D - G, G, [j]) if j < 8 else [] for j in order], [[]] * 8)
    prog += cat(a2)
    prog += ssm(True)
    prog += inv(D - G, G, range(NJ // 2))
    prog += cat(x_out(3, j2) for j2 in (0, 4, 1, 5, 2, 6, 3, 7))
    for _, fn in prog:
        fn()
    for c in cp_o:
        c.wait()


@jax.jit
def pallas_interleave_layers__sliding_local_dilated__ssm_conv_s4__prompt_kernel(
    A_x: jax.Array,
    A_wqkv: jax.Array,
    A_wo: jax.Array,
    B_u: jax.Array,
    B_A_re: jax.Array,
    B_A_im: jax.Array,
    B_B_re: jax.Array,
    B_B_im: jax.Array,
    B_C_re: jax.Array,
    B_C_im: jax.Array,
    B_log_dt: jax.Array,
    B_Dskip: jax.Array,
):
    del B_u
    hbm = pl.BlockSpec(memory_space=pl.ANY)
    out = pl.pallas_call(
        _kernel,
        in_specs=[hbm] * 14,
        out_specs=hbm,
        out_shape=jax.ShapeDtypeStruct((S, D), BF16),
        scratch_shapes=[
            pltpu.VMEM((3, NA, NA), BF16),
            pltpu.VMEM((D,), BF16),
            pltpu.VMEM((D,), BF16),
            pltpu.VMEM((6, D, 128), BF16),
            pltpu.VMEM((4, S // 2, 128), U32),
            pltpu.VMEM((D, 3 * D), BF16),
            pltpu.VMEM((D, D), BF16),
            pltpu.VMEM((NJ, NA // 2, 256), U32),
            pltpu.VMEM((NJ, NA // 2, 256), U32),
            pltpu.VMEM((D, 128), F32),
            pltpu.VMEM((D, 128), F32),
            pltpu.VMEM((D // 2, 3 * D), U32),
            pltpu.VMEM((NJ, D // 2, NA), U32),
            pltpu.VMEM((3 * D // 2, D), U32),
            pltpu.VMEM((D // 2, D), U32),
            pltpu.VMEM((NJ, D // 2, NA), U32),
            pltpu.VMEM((NJ, D // 2, NA), U32),
            pltpu.VMEM((NJ, D // 2, NA), U32),
            pltpu.VMEM((NJ, D, NA), F32),
            pltpu.VMEM((NJ, D, NA), F32),
            pltpu.VMEM((2, NJ - 1, D, NA), F32),
            pltpu.VMEM((2, NJ - 1, D, NA), F32),
            pltpu.VMEM((2, NJ, D, NA), F32),
            pltpu.VMEM((2, NJ, D, NA), F32),
            pltpu.VMEM((24, NA), U32),
            pltpu.SemaphoreType.DMA((8,)),
            pltpu.SemaphoreType.DMA((4,)),
            pltpu.SemaphoreType.DMA((15,)),
            pltpu.SemaphoreType.REGULAR,
        ],
        compiler_params=pltpu.CompilerParams(vmem_limit_bytes=100 << 20),
    )(A_x.reshape(S, D), A_wqkv, A_wo, _F, _FK,
      B_A_re, B_A_im, B_B_re, B_B_im, B_C_re, B_C_im,
      _PM, B_log_dt, B_Dskip)
    return out.reshape(1, S, D)
```

```python
import math

import jax
import jax.numpy as jnp
import ml_dtypes
import numpy as np
import jax.experimental.pallas as pl
import jax.experimental.pallas.tpu as pltpu

S, D, H, DH, WIN = 2048, 512, 32, 16, 8
NJ, NA = 16, 128
EPS = 1e-5
F32, BF16, U32, I32 = jnp.float32, jnp.bfloat16, jnp.uint32, jnp.int32
LG, G = 24, 64
LATE = ((7, 2), (6, 3), (7, 3))
P0 = 80
NT = (((1,), (1,)), ((), ()))


def _dft_consts():
    a = np.arange(NA)[None, :, None]
    j = np.arange(NJ)[:, None, None]
    k = np.arange(NA)[None, None, :]
    th = np.pi * (((NJ * a + j) * (2 * k + 1)) % (4 * S)) / (2 * S)
    f = np.concatenate([np.cos(th), -np.sin(th)], axis=-1)
    lane = np.arange(NA)
    ln = (lane - 3) % NA
    fk = f[:, 32 * (ln % 4) + ln // 4, :]
    perm = np.zeros((NA, NA), np.float32)
    perm[lane, (lane % 8) * DH + lane // 8] = 1.0
    pm = np.stack([perm * DH ** -0.5, perm])
    bf = ml_dtypes.bfloat16
    return f.astype(bf), fk.astype(bf), pm.astype(bf)


_F, _FK, _PM = _dft_consts()


def _round_l(l):
    return int(np.float32(l).astype(ml_dtypes.bfloat16).astype(np.float32))


_R = [[_round_l(256 * q + j) - 256 * q for j in range(NJ)] for q in range(8)]
assert all(_round_l(256 * q + 16 * b + j) == 256 * q + 16 * b + _R[q][j]
           for q in range(8) for b in range(16) for j in range(NJ))
assert _R[2] == _R[3] and _R[4] == _R[5] == _R[6] == _R[7]
_PAIRS = ([((0, r), (0, r + 8)) for r in range(8)]
          + [((1, 0), (1, 4)), ((1, 8), (1, 12)), ((0, 16), (1, 16))]
          + [((2, r), (3, r)) for r in (0, 8, 16)])


def _cmul(x, y):
    return x[0] * y[0] - x[1] * y[1], x[0] * y[1] + x[1] * y[0]


def _csq(x):
    return x[0] * x[0] - x[1] * x[1], (x[0] + x[0]) * x[1]


def _bfly4(x, inv):
    (ar, ai), (br, bi), (cr, ci), (dr, di) = x
    sr, si, tr, ti = ar + cr, ai + ci, ar - cr, ai - ci
    ur, ui, vr, vi = br + dr, bi + di, br - dr, bi - di
    y1, y3 = (tr + vi, ti - vr), (tr - vi, ti + vr)
    if inv:
        y1, y3 = y3, y1
    return [(sr + ur, si + ui), y1, (sr - ur, si - ui), y3]


def _twiddle(x, e):
    e %= 16
    xr, xi = x
    if e == 0:
        return x
    if e == 4:
        return xi, -xr
    if e == 12:
        return -xi, xr
    c, s = math.cos(math.pi * e / 8), -math.sin(math.pi * e / 8)
    if e % 2 == 0:
        if c * s > 0:
            return (xr - xi) * c, (xr + xi) * c
        return (xr + xi) * c, (xi - xr) * c
    return xr * c - xi * s, xr * s + xi * c


def _half4(p, q, h):
    (pr, pi), (qr, qi) = p, q
    if h:
        return (pr + qi, pi - qr), (pr - qi, pi + qr)
    return (pr + qr, pi + qi), (pr - qr, pi - qi)


def _pk(x):
    return pltpu.bitcast(x.astype(BF16), U32)


def _bf(x):
    return pltpu.bitcast(x, BF16)


def _dot(a, b, dims=(((1,), (0,)), ((), ()))):
    return jax.lax.dot_general(a, b, dims, preferred_element_type=F32)


def _merge(*streams):
    keyed = []
    for n, st in enumerate(streams):
        tot, acc = sum(c for c, _ in st) or 1, 0
        for t in st:
            keyed.append(((acc + 0.5 * t[0]) / tot, n, len(keyed), t))
            acc += t[0]
    return [k[-1] for k in sorted(keyed, key=lambda k: k[:3])]


def _flip8(x, sub):
    r = [pltpu.roll(x, k, 0) for k in (7, 5, 3, 1)]
    s4 = sub & 3
    return jnp.where(s4 == 3, r[0], jnp.where(s4 == 2, r[1], jnp.where(s4 == 1, r[2], r[3])))


def _kernel(x_hbm, wqkv_hbm, wo_hbm, f_hbm, fk_hbm,
            are_hbm, aim_hbm, bre_hbm, bim_hbm, cre_hbm, cim_hbm, pm_hbm, ldt_hbm, dsk_hbm,
            out_hbm,
            pm_ref, ldt_ref, dsk_ref, par_ref, xu, wqkv, wo, fm, fk, dtc, dsc, kt, wt, wot, xn, os_, xr, qs, ke, ve, kf, zs, zero,
            sem_in, sem_out, sem_p, sem_b):
    xb = xu.bitcast(BF16)
    cp_x = [pltpu.make_async_copy(x_hbm.at[:, pl.ds(128 * c, 128)], xb.at[c], sem_in.at[c])
            for c in range(4)]
    cp_wqkv = pltpu.make_async_copy(wqkv_hbm, wqkv, sem_in.at[4])
    cp_wo = pltpu.make_async_copy(wo_hbm, wo, sem_in.at[5])
    cp_fk = pltpu.make_async_copy(fk_hbm, fk.bitcast(BF16), sem_in.at[6])
    cp_f = pltpu.make_async_copy(f_hbm, fm.bitcast(BF16), sem_in.at[7])
    cp_o = [pltpu.make_async_copy(xb.at[c], out_hbm.at[:, pl.ds(128 * c, 128)], sem_out.at[c])
            for c in range(4)]
    cp_p = [[pltpu.make_async_copy(r.at[rows], par_ref.at[i, rows], sem_p.at[6 * h + i])
             for i, r in enumerate((are_hbm, aim_hbm, bre_hbm, bim_hbm, cre_hbm, cim_hbm))]
            for h, rows in enumerate((pl.ds(0, P0), pl.ds(P0, D - P0)))]
    cp_s = [pltpu.make_async_copy(a, b, sem_p.at[12 + i])
            for i, (a, b) in enumerate(((ldt_hbm, ldt_ref), (dsk_hbm, dsk_ref), (pm_hbm, pm_ref)))]
    cp_p = [cp_s[:1] + cp_p[0], cp_p[1] + cp_s[1:]]
    for c in cp_p[0] + cp_p[1]:
        c.start()

    for ref in (dtc, dsc, kt, wt, wot, xn, os_, xr, qs, ke, ve, kf, zs):
        ref[(0,) * (len(ref.shape) - 2) + (pl.ds(1, 8), pl.ds(0, 128))] = jnp.zeros((8, 128), ref.dtype)

    zero[pl.ds(1, 16)] = jnp.zeros((16, 128), U32)
    marks, used, rate = [], [], [1.0]

    def mark(x):
        marks.extend(x[r:r + 8, :128] for r in range(0, x.shape[0], 16) for _ in range(x.shape[1] // 128))

    def pace(vals, cost):
        if not marks:
            return list(vals)
        i = min(max(used + [0, len(marks) - LG]), len(marks) - 1)
        used[:] = [i + cost * rate[0] / 16]
        t = pltpu.bitcast(marks[int(i)], U32) & zero[8:16]
        return [pltpu.bitcast(pltpu.bitcast(v, U32) | t, F32) for v in vals]

    def overlap(m, *vs):
        r = sum(c for c, _ in m) / max(1, sum(c for v in vs for c, _ in v))
        return [(1, lambda: rate.__setitem__(0, r))] + _merge(m, *vs)

    def barrier():
        pl.semaphore_signal(sem_b, 1)
        pl.semaphore_wait(sem_b, 1)
        marks[:], used[:] = [], []

    def iota(axis):
        return jax.lax.broadcasted_iota(I32, (8, 128), axis)

    def step_size():
        dt_row = jnp.exp(ldt_ref[...].astype(F32).reshape(1, D)).astype(BF16).astype(F32)
        dtc[...] = jnp.broadcast_to(dt_row, (128, D)).T

    def d_skip():
        dsc[...] = jnp.broadcast_to(dsk_ref[...].astype(F32).reshape(1, D), (128, D)).T

    def k_tables(g):
        st = {}

        def par(i):
            return par_ref[i, 16 * (g // 2):16 * (g // 2) + 16].astype(F32)[8 * (g % 2):8 * (g % 2) + 8]

        def mix(u, v):
            lo = iota(0) < 4
            rv = [pltpu.roll(c, 4, 0) for c in v]
            return (tuple(jnp.where(lo, a, b) for a, b in zip(u, rv)),
                    tuple(jnp.where(lo, b, a) for a, b in zip(u, rv)))

        def put(name, t, two):
            kreg.setdefault((name, g, t), []).append(jnp.concatenate(
                [jnp.concatenate([two[0][c], two[1][c]], axis=0) for c in range(2)], axis=1))

        def base():
            dt, = pace([dtc[8 * g:8 * g + 8]], 100)
            zr, zi = dt * par(0), dt * par(1)
            mag = jnp.exp(zr)
            st[1] = (mag * jnp.cos(zi), mag * jnp.sin(zi))
            st[0] = _cmul((par(4), par(5)), (dt * par(2), dt * par(3)))

        def left():
            lam = {1: st[1]}
            for p in range(1, 10):
                lam[2 ** p] = _csq(lam[2 ** (p - 1)])
            st[16] = lam[16]
            e = {(0, 0): st[0]}
            for a1 in (1, 2, 3):
                e[a1, 0] = _cmul(e[a1 - 1, 0], lam[512])
            for a1, r in ((0, 8), (1, 4), (0, 16), (1, 16)):
                e[a1, r] = _cmul(e[a1, 0], lam[r])
            d1, d8 = mix(lam[1], lam[1]), mix(lam[8], lam[8])
            prev, done = None, []
            for i, (u, v) in enumerate(_PAIRS):
                if u in e:
                    cur = mix(e[u], e[v])
                else:
                    m = d1 if i < 8 else d8
                    cur = (_cmul(prev[0], m[0]), _cmul(prev[1], m[1]))
                prev = cur
                done.append(cur)
                if i % 2:
                    for t in range(2):
                        put("l", t, (done[i - 1][t], done[i][t]))

        def right(t):
            lo = iota(0) < 4
            if t == 0:
                f = (_flip8(st[16][0], iota(0)), -_flip8(st[16][1], iota(0)))
                st["d"] = mix(f, f)[::-1]
            d = st["d"][t]
            d2 = _csq(d)
            one = (1.0, 0.0)
            cur = tuple(jnp.where(lo, a, b) for a, b in (zip(one, d), zip(d, d2))[t])
            for v in range(0, 16, 2):
                if v:
                    cur = _cmul(cur, d2)
                nxt = _cmul(cur, d2)
                if t and v == 14:
                    nxt = tuple(jnp.where(lo, a, b) for a, b in zip(nxt, one))
                put("r", t, (cur, nxt))
                cur = nxt

        return [(45, base), (70, left), (35, lambda: right(0)), (30, lambda: right(1))]

    kreg = {}

    def k_matmul(g):
        def mm():
            kreg[g] = [_dot(*(jnp.concatenate(kreg.pop((n, g, t)), axis=0).astype(BF16)
                              for n in "lr"), NT) for t in range(2)]

        def post():
            o0, o1 = kreg.pop(g)
            mark(o0); mark(o1)
            lo = iota(0) < 4
            ln = (iota(1) + (NA - 3)) & (NA - 1)
            piece = {}
            for i, (u, v) in enumerate(_PAIRS):
                a, b = o0[8 * i:8 * i + 8], o1[8 * i:8 * i + 8]
                for e, x in ((u, jnp.where(lo, a, b)), (v, pltpu.roll(jnp.where(lo, b, a), 4, 0))):
                    piece[e] = pltpu.roll(x, e[0], 1, stride=1, stride_axis=0)
            memo, res = {}, []
            for j in range(NJ):
                r2, r4, r8 = _R[1][j], _R[2][j], _R[4][j]
                if r8 not in memo:
                    memo[r8] = jnp.where((ln & 3) == 2, piece[2, r8], piece[3, r8])
                if (r4, r8) not in memo:
                    memo[r4, r8] = jnp.where((ln & 3) == 1, piece[1, r4], memo[r8])
                x = piece[0, j] if r2 == j else jnp.where(ln < 64, piece[0, j], piece[0, r2])
                res.append(jnp.where((ln & 3) == 0, x, memo[r4, r8]))
            if g % 2 == 0:
                kreg["even"] = res
            else:
                for j, ev in enumerate(kreg.pop("even")):
                    kt[j, 4 * g - 4:4 * g + 4] = _pk(jnp.concatenate([ev, res[j]], axis=0))

        return [(5, mm)], [(30, post)]

    def k_fft(g):
        def run(h):
            rows = pl.ds(8 * g, 8)
            dsk = dsc[rows]
            for i, xs_ in enumerate(spectrum(rows, h, 20 + 6 * h)):
                for m1, (yr, yi) in enumerate(xs_):
                    kf[0, 4 * (h + 2 * i) + m1, rows] = (yr + dsk) * (1.0 / S)
                    kf[1, 4 * (h + 2 * i) + m1, rows] = yi * (1.0 / S)
        return [(20 + 6 * h, lambda h=h: run(h)) for h in range(2)]

    def w_qkv(b):
        def run():
            cols = pl.ds(128 * b, 128)
            w = _dot(pm_ref[0 if b < 4 else 1], wqkv[:, cols], NT)
            mark(w)
            wt[64 * b:64 * b + 64] = _pk(w)
        return [(128, run)]

    def w_out(b):
        def run():
            wot[:, 128 * b:128 * b + 128] = _pk(_dot(pm_ref[1], wo[128 * b:128 * b + 128]).T)
        return [(128, run)]

    def x_in(j2):
        def run(c):
            v = xu[c, pl.ds(j2, NA, stride=NJ // 2), :].T
            xr[2 * j2, 128 * c:128 * c + 128] = pltpu.bitcast(v << 16, F32)
            xr[2 * j2 + 1, 128 * c:128 * c + 128] = pltpu.bitcast(v & np.uint32(0xFFFF0000), F32)
        return [(40, lambda c=c: run(c)) for c in range(4)]

    def x_out(c, j2):
        def run():
            lo, hi = (pltpu.bitcast(xr[j, 128 * c:128 * c + 128].astype(BF16).astype(F32), U32)
                      for j in (2 * j2, 2 * j2 + 1))
            v = (lo >> 16) | hi
            xu[c, pl.ds(j2, NA, stride=NJ // 2), :] = v.T
            if j2 == NJ // 2 - 1:
                cp_o[c].start()
        return [(25, run)]

    def tree(acc, xs_):
        acc = list(acc)
        for i, x in enumerate(xs_):
            acc[i % 4] = acc[i % 4] + x
        return acc

    def total(acc):
        return jnp.broadcast_to(
            jnp.sum((acc[0] + acc[1]) + (acc[2] + acc[3]), axis=0, keepdims=True), (8, 128))

    def ln(j):
        st = {}

        def mean():
            v = [xr[j, r:r + 8] for r in range(0, D, 8)]
            st["m"] = total(tree(pace(v[:4], 18), v[4:])) * (1.0 / D)

        def var(r0):
            m, = pace([st["m"]], 25)
            c = [xr[j, r:r + 8] - m for r in range(r0, r0 + D // 2, 8)]
            c = [v * v for v in c]
            if r0:
                st["s"] = jax.lax.rsqrt(total(tree(st["v"], c)) * (1.0 / D) + EPS)
            else:
                st["v"] = tree(c[:4], c[4:])

        def norm():
            for r in range(0, D, 16):
                if r % 128 == 0:
                    m, s_ = pace([st["m"], st["s"]], 15)
                u = [(xr[j, r + h:r + h + 8] - m) * s_ for h in (0, 8)]
                xn[j, r // 2:r // 2 + 8] = _pk(jnp.concatenate(u, axis=0))

        return [(18, mean), (25, lambda: var(0)), (25, lambda: var(D // 2)), (60, norm)]

    def kv(j):
        p, jj = j & 1, j >> 1

        def run(dst, b):
            k = _dot(_bf(wt[64 * b:64 * b + 64]), _bf(xn[j]))
            mark(k)
            r = pl.ds(128 * (b % 4), 128)
            dst[p, 7 + jj, r] = k
            if jj:
                dst[p, jj - 1, r] = pltpu.roll(k, 1, 1)

        return [(128, lambda b=b: run(ke if b < 8 else ve, b)) for b in range(4, 12)]

    def qproj(j):
        def run(b):
            q = _dot(_bf(wt[64 * b:64 * b + 64]), _bf(xn[j]))
            mark(q)
            qs[j, 128 * b:128 * b + 128] = q
        return [(128, lambda b=b: run(b)) for b in range(4)]

    def core(j):
        p, jj = j & 1, j >> 1
        st = {}

        def probs(hg, d0):
            s = st.pop(hg) if d0 else [None] * WIN
            rows = [pl.ds(128 * hg + 8 * d, 8) for d in range(d0, d0 + DH // 2)]
            qv = [qs[j, r] for r in rows]
            for r, q in zip(rows, pace(qv[:4], 16) + pace(qv[4:], 29 if d0 else 17)):
                for w in range(WIN):
                    t = q * ke[p, 7 + jj - w, r]
                    s[w] = t if s[w] is None else s[w] + t
            if not d0:
                st[hg] = s
                return
            for w in range(jj + 1, WIN):
                s[w] = jnp.where(iota(1) >= 1, s[w], -1e9)
            m = s[0]
            for w in range(1, WIN):
                m = jnp.maximum(m, s[w])
            e = [jnp.exp(a - m) for a in s]
            tot = e[0]
            for w in range(1, WIN):
                tot = tot + e[w]
            inv = 1.0 / tot
            st[hg] = [a * inv for a in e]

        def apply(hg, d0):
            e = pace(st.pop(hg) if d0 else st[hg], 37)
            for d in range(d0, d0 + DH // 2, 2):
                o = []
                for r in (pl.ds(128 * hg + 8 * d, 8), pl.ds(128 * hg + 8 * d + 8, 8)):
                    acc = e[0] * ve[p, 7 + jj, r]
                    for w in range(1, WIN):
                        acc = acc + e[w] * ve[p, 7 + jj - w, r]
                    o.append(acc)
                os_[j, pl.ds(64 * hg + 4 * d, 8)] = _pk(jnp.concatenate(o, axis=0))

        return [(c, lambda f=f, hg=hg, d0=d0: f(hg, d0)) for hg in range(4)
                for c, f, d0 in ((33, probs, 0), (45, probs, 8), (37, apply, 0), (37, apply, 8))]

    def wout(j):
        def run(b):
            r = pl.ds(128 * b, 128)
            y = _dot(_bf(wot[64 * b:64 * b + 64]), _bf(os_[j]))
            mark(y)
            xr[j, r] = xr[j, r] + y
        return [(128, lambda b=b: run(b)) for b in range(4)]

    def dft(src, mat, c0, n, more=False):
        def run(j):
            rows = pl.ds(c0, n)
            a, b = (_dot(_bf(src[i, c0 // 2:(c0 + n) // 2]), _bf(mat[i])) for i in (j, j + 8))
            for h, z in enumerate((a + b, a - b)):
                i = 8 * h + j
                res = {i: (z[:, :128], z[:, 128:])}
                if more and 4 <= j < 7:
                    res[i - 4], res[i] = second((zs[0, i - 4, rows], zs[1, i - 4, rows]), res[i], j - 4, h)
                for k, v in res.items():
                    zs[0, k, rows], zs[1, k, rows] = v
            mark(z)
        return [(n, lambda j=j: run(j)) for j in range(NJ // 2)]

    def second(p, q, j0, h):
        return [_twiddle(v, j0 * (h + 2 * i)) for i, v in enumerate(_half4(p, q, h))]

    def spectrum(rows, h, cost, done=0):
        z = [(zs[0, 8 * h + j, rows], zs[1, 8 * h + j, rows]) for j in range(8)]
        paced = (0, 3, 4) if done else (0, 1, 2, 3)
        pz = pace([c for i in paced for c in z[i]], cost)
        for n, i in enumerate(paced):
            z[i] = tuple(pz[2 * n:2 * n + 2])
        a = [(z[j0], z[j0 + 4]) if j0 < done else second(z[j0], z[j0 + 4], j0, h) for j0 in range(4)]
        return [_bfly4([a[j0][i] for j0 in range(4)], False) for i in range(2)]

    def fft(c0, n):
        def run(r0, h):
            rows = pl.ds(r0, 8)
            b = []
            for i, xs_ in enumerate(spectrum(rows, h, 40 + 6 * h, 3)):
                m0 = h + 2 * i
                y = [_cmul(v, (kf[0, 4 * m0 + m1, rows], kf[1, 4 * m0 + m1, rows]))
                     for m1, v in enumerate(xs_)]
                b.append([_twiddle(v, -j0 * m0) for j0, v in enumerate(_bfly4(y, True))])
            for j0 in range(4):
                (ar, ai), (br, bi) = b[0][j0], b[1][j0]
                lo = (ar + br, ai + bi)
                hi = (bi - ai, ar - br) if h else (ar - br, ai - bi)
                for c in range(2):
                    zs[c, 8 * h + j0, rows] = lo[c]
                    zs[c, 8 * h + j0 + 4, rows] = hi[c]
        return [(40 + 6 * h, lambda r0=r0, h=h: run(r0, h))
                for r0 in range(c0, c0 + n, 8) for h in range(2)]

    def inv(c0, n, js):
        def run(j):
            rows = pl.ds(c0, n)
            a, b = (jnp.concatenate([zs[0, i, rows], zs[1, i, rows]], axis=1) for i in (j, j + 8))
            ys = [_dot(z.astype(BF16), _bf(fm[i]), NT) for i, z in ((j, a + b), (j + 8, a - b))]
            for i, y in zip((j, j + 8), ys):
                xr[i, rows] = xr[i, rows] + y
            mark(ys[0])
        return [(n, lambda j=j: run(j)) for j in js]

    def cat(lists):
        return [t for l in lists for t in l]

    k_steps, tab = [], [k_tables(g) for g in range(64)] + [[], [], []]
    for g in range(-2, 64):
        mm, post = k_matmul(g) if g >= 0 else ([], [])
        k_steps.append(mm + tab[g + 1][1:2] + tab[g + 2][:1] + post + tab[g + 1][2:])

    order = [j0 + d for j0 in (0, 2, 1, 3) for d in (0, 8, 4, 12)]

    def lane_dft(n):
        return [dft(xn, fm, c, 128, True)[order[2 * n]] for c in range(0, D, 128)]

    def attention(pre, extra):
        steps = [pre[0] + pre[1] + ln(order[0])]
        for i in range(8):
            steps.append(overlap(kv(order[i]) + pre[i + 2], ln(order[i + 1]), extra[i]))
        steps.append(qproj(order[0]))
        for i in range(NJ + 4):
            wo_, ln2 = ([order[n] for n in (2 * k - 1, 2 * k) if 0 <= n < NJ] for k in (i - 8, i - 9))
            m = pre[i + 10] if i < 6 else []
            m = m + _merge(kv(order[8 + i]) if i < 8 else [],
                           qproj(order[i + 1]) if i + 1 < NJ else [], cat(wout(j) for j in wo_))
            if i >= 12:
                m = _merge(m, [t for c, t in enumerate(lane_dft(i - 12)) if (i - 12, c) not in LATE])
            v = (ln(order[8 + i + 1]) if i < 7 else []) + cat(ln(j) for j in ln2)
            c = core(order[i]) if i < NJ else []
            if i >= NJ - 1:
                c, v = (t + [(0.25 * sum(x for x, _ in t), lambda: None)] for t in (c, v))
            steps.append(overlap(m, c, v))
        return steps

    def ssm(last):
        prog = [(0, barrier)]
        for c in range(0, D, G):
            out = cat(x_out(c // 128 - 1, j2) for j2 in range(8)) if last and c > 128 and c % 128 else []
            prog += overlap(inv(c - G, G, range(NJ // 2)) if c else [lane_dft(n)[b] for n, b in LATE],
                            fft(c, G), out)
            if out and c > 256:
                prog += [(0, barrier)]
        return prog

    def wait(*cps):
        def run():
            for c in cps:
                c.wait()
            marks[:], used[:] = [], []
        return [(0, run)]

    def start(*cps):
        return [(0, lambda: [c.start() for c in cps])]

    kd = [dft(kt, fk, c, 128) for c in range(0, D, 128)]
    a1 = attention([[]] * NJ, [cat(k_fft(g) for g in range(8 * i, 8 * i + 8)) for i in range(8)])
    head = wait(*cp_p[0]) + [(1, step_size)] + cat(k_steps[:P0 // 8]) + wait(*cp_p[1]) + start(cp_wqkv, *cp_x, cp_fk)
    head += cat(k_steps[P0 // 8:]) + wait(cp_wqkv, *cp_x, cp_fk) + start(cp_wo, cp_f) + [(1, d_skip)]
    head += _merge(_merge(cat(kd), cat(w_qkv(b) for b in range(12))),
                   x_in(0) + a1[0] + cat(x_in(j2) for j2 in range(1, 8)))
    head += [(0, barrier)]
    prog = head + cat(a1[1:9]) + wait(cp_wo, cp_f) + cat(w_out(b) for b in range(4))
    prog += cat(a1[9:]) + ssm(False)
    a2 = attention([inv(D - G, G, [j]) if j < 8 else [] for j in order], [[]] * 8)
    prog += cat(a2)
    prog += ssm(True)
    prog += inv(D - G, G, range(NJ // 2))
    prog += cat(x_out(3, j2) for j2 in (0, 4, 1, 5, 2, 6, 3, 7))
    for _, fn in prog:
        fn()
    for c in cp_o:
        c.wait()


@jax.jit
def pallas_interleave_layers__sliding_local_dilated__ssm_conv_s4__prompt_kernel(
    A_x: jax.Array,
    A_wqkv: jax.Array,
    A_wo: jax.Array,
    B_u: jax.Array,
    B_A_re: jax.Array,
    B_A_im: jax.Array,
    B_B_re: jax.Array,
    B_B_im: jax.Array,
    B_C_re: jax.Array,
    B_C_im: jax.Array,
    B_log_dt: jax.Array,
    B_Dskip: jax.Array,
):
    del B_u
    hbm = pl.BlockSpec(memory_space=pl.ANY)
    out = pl.pallas_call(
        _kernel,
        in_specs=[hbm] * 14,
        out_specs=hbm,
        out_shape=jax.ShapeDtypeStruct((S, D), BF16),
        scratch_shapes=[
            pltpu.VMEM((2, NA, NA), BF16),
            pltpu.VMEM((D,), BF16),
            pltpu.VMEM((D,), BF16),
            pltpu.VMEM((6, D, 128), BF16),
            pltpu.VMEM((4, S // 2, 128), U32),
            pltpu.VMEM((D, 3 * D), BF16),
            pltpu.VMEM((D, D), BF16),
            pltpu.VMEM((NJ, NA // 2, 256), U32),
            pltpu.VMEM((NJ, NA // 2, 256), U32),
            pltpu.VMEM((D, 128), F32),
            pltpu.VMEM((D, 128), F32),
            pltpu.VMEM((NJ, D // 2, NA), U32),
            pltpu.VMEM((3 * D // 2, D), U32),
            pltpu.VMEM((D // 2, D), U32),
            pltpu.VMEM((NJ, D // 2, NA), U32),
            pltpu.VMEM((NJ, D // 2, NA), U32),
            pltpu.VMEM((NJ, D, NA), F32),
            pltpu.VMEM((NJ, D, NA), F32),
            pltpu.VMEM((2, NJ - 1, D, NA), F32),
            pltpu.VMEM((2, NJ - 1, D, NA), F32),
            pltpu.VMEM((2, NJ, D, NA), F32),
            pltpu.VMEM((2, NJ, D, NA), F32),
            pltpu.VMEM((24, NA), U32),
            pltpu.SemaphoreType.DMA((8,)),
            pltpu.SemaphoreType.DMA((4,)),
            pltpu.SemaphoreType.DMA((15,)),
            pltpu.SemaphoreType.REGULAR,
        ],
        compiler_params=pltpu.CompilerParams(vmem_limit_bytes=100 << 20),
    )(A_x.reshape(S, D), A_wqkv, A_wo, _F, _FK,
      B_A_re, B_A_im, B_B_re, B_B_im, B_C_re, B_C_im,
      _PM, B_log_dt, B_Dskip)
    return out.reshape(1, S, D)
```

```python
import math

import jax
import jax.numpy as jnp
import ml_dtypes
import numpy as np
import jax.experimental.pallas as pl
import jax.experimental.pallas.tpu as pltpu

S, D, H, DH, WIN = 2048, 512, 32, 16, 8
NJ, NA = 16, 128
EPS = 1e-5
F32, BF16, U32, I32 = jnp.float32, jnp.bfloat16, jnp.uint32, jnp.int32
LG, G = 24, 64
LATE = ((7, 2), (6, 3), (7, 3))
P0 = 80
NT = (((1,), (1,)), ((), ()))


def _dft_consts():
    a = np.arange(NA)[None, :, None]
    j = np.arange(NJ)[:, None, None]
    k = np.arange(NA)[None, None, :]
    th = np.pi * (((NJ * a + j) * (2 * k + 1)) % (4 * S)) / (2 * S)
    f = np.concatenate([np.cos(th), -np.sin(th)], axis=-1)
    lane = np.arange(NA)
    ln = (lane - 3) % NA
    fk = f[:, 32 * (ln % 4) + ln // 4, :]
    perm = np.zeros((NA, NA), np.float32)
    perm[lane, (lane % 8) * DH + lane // 8] = 1.0
    pm = np.stack([perm * DH ** -0.5, perm])
    bf = ml_dtypes.bfloat16
    return f.astype(bf), fk.astype(bf), pm.astype(bf)


_F, _FK, _PM = _dft_consts()


def _round_l(l):
    return int(np.float32(l).astype(ml_dtypes.bfloat16).astype(np.float32))


_R = [[_round_l(256 * q + j) - 256 * q for j in range(NJ)] for q in range(8)]
assert all(_round_l(256 * q + 16 * b + j) == 256 * q + 16 * b + _R[q][j]
           for q in range(8) for b in range(16) for j in range(NJ))
assert _R[2] == _R[3] and _R[4] == _R[5] == _R[6] == _R[7]
_PAIRS = ([((0, r), (0, r + 8)) for r in range(8)]
          + [((1, 0), (1, 4)), ((1, 8), (1, 12)), ((0, 16), (1, 16))]
          + [((2, r), (3, r)) for r in (0, 8, 16)])


def _cmul(x, y):
    return x[0] * y[0] - x[1] * y[1], x[0] * y[1] + x[1] * y[0]


def _csq(x):
    return x[0] * x[0] - x[1] * x[1], (x[0] + x[0]) * x[1]


def _bfly4(x, inv):
    (ar, ai), (br, bi), (cr, ci), (dr, di) = x
    sr, si, tr, ti = ar + cr, ai + ci, ar - cr, ai - ci
    ur, ui, vr, vi = br + dr, bi + di, br - dr, bi - di
    y1, y3 = (tr + vi, ti - vr), (tr - vi, ti + vr)
    if inv:
        y1, y3 = y3, y1
    return [(sr + ur, si + ui), y1, (sr - ur, si - ui), y3]


def _twiddle(x, e):
    e %= 16
    xr, xi = x
    if e == 0:
        return x
    if e == 4:
        return xi, -xr
    if e == 12:
        return -xi, xr
    c, s = math.cos(math.pi * e / 8), -math.sin(math.pi * e / 8)
    if e % 2 == 0:
        if c * s > 0:
            return (xr - xi) * c, (xr + xi) * c
        return (xr + xi) * c, (xi - xr) * c
    return xr * c - xi * s, xr * s + xi * c


def _half4(p, q, h):
    (pr, pi), (qr, qi) = p, q
    if h:
        return (pr + qi, pi - qr), (pr - qi, pi + qr)
    return (pr + qr, pi + qi), (pr - qr, pi - qi)


def _pk(x):
    return pltpu.bitcast(x.astype(BF16), U32)


def _pk4(u):
    return _pk(jnp.concatenate([jnp.concatenate(v, axis=0) for v in (u[:2], u[2:])], axis=1))


def _rows(ref, j, r0, n):
    return _bf(jnp.concatenate([ref[j, pl.ds(8 * (b // 2), 8), pl.ds(128 * (b % 2), 128)]
                                for b in range(r0 // 16, (r0 + n) // 16)], axis=0))


def _bf(x):
    return pltpu.bitcast(x, BF16)


def _dot(a, b, dims=(((1,), (0,)), ((), ()))):
    return jax.lax.dot_general(a, b, dims, preferred_element_type=F32)


def _merge(*streams):
    keyed = []
    for n, st in enumerate(streams):
        tot, acc = sum(c for c, _ in st) or 1, 0
        for t in st:
            keyed.append(((acc + 0.5 * t[0]) / tot, n, len(keyed), t))
            acc += t[0]
    return [k[-1] for k in sorted(keyed, key=lambda k: k[:3])]


def _flip8(x, sub):
    r = [pltpu.roll(x, k, 0) for k in (7, 5, 3, 1)]
    s4 = sub & 3
    return jnp.where(s4 == 3, r[0], jnp.where(s4 == 2, r[1], jnp.where(s4 == 1, r[2], r[3])))


def _kernel(x_hbm, wqkv_hbm, wo_hbm, f_hbm, fk_hbm,
            are_hbm, aim_hbm, bre_hbm, bim_hbm, cre_hbm, cim_hbm, pm_hbm, ldt_hbm, dsk_hbm,
            out_hbm,
            pm_ref, ldt_ref, dsk_ref, par_ref, xu, wqkv, wo, fm, fk, dtc, dsc, kt, wt, wot, xn, os_, xr, qs, ke, ve, kf, zs, zero,
            sem_in, sem_out, sem_p, sem_b):
    xb = xu.bitcast(BF16)
    cp_x = [pltpu.make_async_copy(x_hbm.at[:, pl.ds(128 * c, 128)], xb.at[c], sem_in.at[c])
            for c in range(4)]
    cp_wqkv = pltpu.make_async_copy(wqkv_hbm, wqkv, sem_in.at[4])
    cp_wo = pltpu.make_async_copy(wo_hbm, wo, sem_in.at[5])
    cp_fk = pltpu.make_async_copy(fk_hbm, fk.bitcast(BF16), sem_in.at[6])
    cp_f = pltpu.make_async_copy(f_hbm, fm.bitcast(BF16), sem_in.at[7])
    cp_o = [pltpu.make_async_copy(xb.at[c], out_hbm.at[:, pl.ds(128 * c, 128)], sem_out.at[c])
            for c in range(4)]
    cp_p = [[pltpu.make_async_copy(r.at[rows], par_ref.at[i, rows], sem_p.at[6 * h + i])
             for i, r in enumerate((are_hbm, aim_hbm, bre_hbm, bim_hbm, cre_hbm, cim_hbm))]
            for h, rows in enumerate((pl.ds(0, P0), pl.ds(P0, D - P0)))]
    cp_s = [pltpu.make_async_copy(a, b, sem_p.at[12 + i])
            for i, (a, b) in enumerate(((ldt_hbm, ldt_ref), (dsk_hbm, dsk_ref), (pm_hbm, pm_ref)))]
    cp_p = [cp_s[:1] + cp_p[0], cp_p[1] + cp_s[1:]]
    for c in cp_p[0] + cp_p[1]:
        c.start()

    for ref in (dtc, dsc, kt, wt, wot, xn, os_, xr, qs, ke, ve, kf, zs):
        ref[(0,) * (len(ref.shape) - 2) + (pl.ds(1, 8), pl.ds(0, 128))] = jnp.zeros((8, 128), ref.dtype)

    zero[pl.ds(1, 16)] = jnp.zeros((16, 128), U32)
    marks, used, rate = [], [], [1.0]

    def mark(x):
        marks.extend(x[r:r + 8, :128] for r in range(0, x.shape[0], 16) for _ in range(x.shape[1] // 128))

    def pace(vals, cost):
        if not marks:
            return list(vals)
        i = min(max(used + [0, len(marks) - LG]), len(marks) - 1)
        used[:] = [i + cost * rate[0] / 16]
        t = pltpu.bitcast(marks[int(i)], U32) & zero[8:16]
        return [pltpu.bitcast(pltpu.bitcast(v, U32) | t, F32) for v in vals]

    def overlap(m, *vs):
        r = sum(c for c, _ in m) / max(1, sum(c for v in vs for c, _ in v))
        return [(1, lambda: rate.__setitem__(0, r))] + _merge(m, *vs)

    def barrier():
        pl.semaphore_signal(sem_b, 1)
        pl.semaphore_wait(sem_b, 1)
        marks[:], used[:] = [], []

    def iota(axis):
        return jax.lax.broadcasted_iota(I32, (8, 128), axis)

    def step_size():
        dt_row = jnp.exp(ldt_ref[...].astype(F32).reshape(1, D)).astype(BF16).astype(F32)
        dtc[...] = jnp.broadcast_to(dt_row, (128, D)).T

    def d_skip():
        dsc[...] = jnp.broadcast_to(dsk_ref[...].astype(F32).reshape(1, D), (128, D)).T

    def k_tables(g):
        st = {}

        def par(i):
            return par_ref[i, 16 * (g // 2):16 * (g // 2) + 16].astype(F32)[8 * (g % 2):8 * (g % 2) + 8]

        def mix(u, v):
            lo = iota(0) < 4
            rv = [pltpu.roll(c, 4, 0) for c in v]
            return (tuple(jnp.where(lo, a, b) for a, b in zip(u, rv)),
                    tuple(jnp.where(lo, b, a) for a, b in zip(u, rv)))

        def put(name, t, two):
            kreg.setdefault((name, g, t), []).append(jnp.concatenate(
                [jnp.concatenate([two[0][c], two[1][c]], axis=0) for c in range(2)], axis=1))

        def base():
            dt, = pace([dtc[8 * g:8 * g + 8]], 100)
            zr, zi = dt * par(0), dt * par(1)
            mag = jnp.exp(zr)
            st[1] = (mag * jnp.cos(zi), mag * jnp.sin(zi))
            st[0] = _cmul((par(4), par(5)), (dt * par(2), dt * par(3)))

        def left():
            lam = {1: st[1]}
            for p in range(1, 10):
                lam[2 ** p] = _csq(lam[2 ** (p - 1)])
            st[16] = lam[16]
            e = {(0, 0): st[0]}
            for a1 in (1, 2, 3):
                e[a1, 0] = _cmul(e[a1 - 1, 0], lam[512])
            for a1, r in ((0, 8), (1, 4), (0, 16), (1, 16)):
                e[a1, r] = _cmul(e[a1, 0], lam[r])
            d1, d8 = mix(lam[1], lam[1]), mix(lam[8], lam[8])
            prev, done = None, []
            for i, (u, v) in enumerate(_PAIRS):
                if u in e:
                    cur = mix(e[u], e[v])
                else:
                    m = d1 if i < 8 else d8
                    cur = (_cmul(prev[0], m[0]), _cmul(prev[1], m[1]))
                prev = cur
                done.append(cur)
                if i % 2:
                    for t in range(2):
                        put("l", t, (done[i - 1][t], done[i][t]))

        def right(t):
            lo = iota(0) < 4
            if t == 0:
                f = (_flip8(st[16][0], iota(0)), -_flip8(st[16][1], iota(0)))
                st["d"] = mix(f, f)[::-1]
            d = st["d"][t]
            d2 = _csq(d)
            one = (1.0, 0.0)
            cur = tuple(jnp.where(lo, a, b) for a, b in (zip(one, d), zip(d, d2))[t])
            for v in range(0, 16, 2):
                if v:
                    cur = _cmul(cur, d2)
                nxt = _cmul(cur, d2)
                if t and v == 14:
                    nxt = tuple(jnp.where(lo, a, b) for a, b in zip(nxt, one))
                put("r", t, (cur, nxt))
                cur = nxt

        return [(45, base), (70, left), (35, lambda: right(0)), (30, lambda: right(1))]

    kreg = {}

    def k_matmul(g):
        def mm():
            kreg[g] = [_dot(*(jnp.concatenate(kreg.pop((n, g, t)), axis=0).astype(BF16)
                              for n in "lr"), NT) for t in range(2)]

        def post():
            o0, o1 = kreg.pop(g)
            mark(o0); mark(o1)
            lo = iota(0) < 4
            ln = (iota(1) + (NA - 3)) & (NA - 1)
            piece = {}
            for i, (u, v) in enumerate(_PAIRS):
                a, b = o0[8 * i:8 * i + 8], o1[8 * i:8 * i + 8]
                for e, x in ((u, jnp.where(lo, a, b)), (v, pltpu.roll(jnp.where(lo, b, a), 4, 0))):
                    piece[e] = pltpu.roll(x, e[0], 1, stride=1, stride_axis=0)
            memo, res = {}, []
            for j in range(NJ):
                r2, r4, r8 = _R[1][j], _R[2][j], _R[4][j]
                if r8 not in memo:
                    memo[r8] = jnp.where((ln & 3) == 2, piece[2, r8], piece[3, r8])
                if (r4, r8) not in memo:
                    memo[r4, r8] = jnp.where((ln & 3) == 1, piece[1, r4], memo[r8])
                x = piece[0, j] if r2 == j else jnp.where(ln < 64, piece[0, j], piece[0, r2])
                res.append(jnp.where((ln & 3) == 0, x, memo[r4, r8]))
            if g % 2 == 0:
                kreg["even"] = res
            else:
                ev = kreg.pop("even")
                for j in range(0, NJ, 2):
                    kt.at[j // 2][4 * g - 4:4 * g + 4] = _pk4([ev[j], res[j], ev[j + 1], res[j + 1]])

        return [(5, mm)], [(30, post)]

    def k_fft(g):
        def run(h):
            rows = pl.ds(8 * g, 8)
            dsk = dsc[rows]
            for i, xs_ in enumerate(spectrum(rows, h, 20 + 6 * h)):
                for m1, (yr, yi) in enumerate(xs_):
                    kf[0, 4 * (h + 2 * i) + m1, rows] = (yr + dsk) * (1.0 / S)
                    kf[1, 4 * (h + 2 * i) + m1, rows] = yi * (1.0 / S)
        return [(20 + 6 * h, lambda h=h: run(h)) for h in range(2)]

    def w_qkv(b):
        def run():
            cols = pl.ds(128 * b, 128)
            w = _dot(pm_ref[0 if b < 4 else 1], wqkv[:, cols], NT)
            mark(w)
            wt[64 * b:64 * b + 64] = _pk(w)
        return [(128, run)]

    def w_out(b):
        def run():
            wot[:, 256 * b:256 * b + 256] = _pk(jnp.concatenate(
                [_dot(pm_ref[1], wo[r:r + 128]).T for r in (256 * b, 256 * b + 128)], axis=1))
        return [(256, run)]

    def x_in(j2):
        def run(c):
            v = xu[c, pl.ds(j2, NA, stride=NJ // 2), :].T
            xr[2 * j2, 128 * c:128 * c + 128] = pltpu.bitcast(v << 16, F32)
            xr[2 * j2 + 1, 128 * c:128 * c + 128] = pltpu.bitcast(v & np.uint32(0xFFFF0000), F32)
        return [(40, lambda c=c: run(c)) for c in range(4)]

    def x_out(c, j2):
        def run():
            u = jnp.concatenate([xr[j, 128 * c:128 * c + 128] for j in (2 * j2, 2 * j2 + 1)], axis=1)
            u = pltpu.bitcast(u.astype(BF16).astype(F32), U32)
            v = (u[:, :128] >> 16) | u[:, 128:]
            xu[c, pl.ds(j2, NA, stride=NJ // 2), :] = v.T
            if j2 == NJ // 2 - 1:
                cp_o[c].start()
        return [(25, run)]

    def tree(acc, xs_):
        acc = list(acc)
        for i, x in enumerate(xs_):
            acc[i % 4] = acc[i % 4] + x
        return acc

    def total(acc):
        return jnp.broadcast_to(
            jnp.sum((acc[0] + acc[1]) + (acc[2] + acc[3]), axis=0, keepdims=True), (8, 128))

    def ln(j):
        st = {}

        def mean():
            v = [xr[j, r:r + 8] for r in range(0, D, 8)]
            st["m"] = total(tree(pace(v[:4], 18), v[4:])) * (1.0 / D)

        def var(r0):
            m, = pace([st["m"]], 25)
            c = [xr[j, r:r + 8] - m for r in range(r0, r0 + D // 2, 8)]
            c = [v * v for v in c]
            if r0:
                st["s"] = jax.lax.rsqrt(total(tree(st["v"], c)) * (1.0 / D) + EPS)
            else:
                st["v"] = tree(c[:4], c[4:])

        def norm():
            for r in range(0, D, 32):
                if r % 128 == 0:
                    m, s_ = pace([st["m"], st["s"]], 10)
                u = [(xr[j, r + h:r + h + 8] - m) * s_ for h in range(0, 32, 8)]
                xn.at[j][r // 4:r // 4 + 8] = _pk4(u)

        return [(18, mean), (25, lambda: var(0)), (25, lambda: var(D // 2)), (40, norm)]

    def kv(j):
        p, jj = j & 1, j >> 1

        def run(dst, b):
            k = _dot(_bf(wt[64 * b:64 * b + 64]), _rows(xn, j, 0, D))
            mark(k)
            r = pl.ds(128 * (b % 4), 128)
            dst[p, 7 + jj, r] = k
            if jj:
                dst[p, jj - 1, r] = pltpu.roll(k, 1, 1)

        return [(128, lambda b=b: run(ke if b < 8 else ve, b)) for b in range(4, 12)]

    def qproj(j):
        def run(b):
            q = _dot(_bf(wt[64 * b:64 * b + 64]), _rows(xn, j, 0, D))
            mark(q)
            qs[j, 128 * b:128 * b + 128] = q
        return [(128, lambda b=b: run(b)) for b in range(4)]

    def core(j):
        p, jj = j & 1, j >> 1
        st = {}

        def probs(hg, d0):
            s = st.pop(hg) if d0 else [None] * WIN
            rows = [pl.ds(128 * hg + 8 * d, 8) for d in range(d0, d0 + DH // 2)]
            qv = [qs[j, r] for r in rows]
            for r, q in zip(rows, pace(qv[:4], 16) + pace(qv[4:], 29 if d0 else 17)):
                for w in range(WIN):
                    t = q * ke[p, 7 + jj - w, r]
                    s[w] = t if s[w] is None else s[w] + t
            if not d0:
                st[hg] = s
                return
            for w in range(jj + 1, WIN):
                s[w] = jnp.where(iota(1) >= 1, s[w], -1e9)
            m = s[0]
            for w in range(1, WIN):
                m = jnp.maximum(m, s[w])
            e = [jnp.exp(a - m) for a in s]
            tot = e[0]
            for w in range(1, WIN):
                tot = tot + e[w]
            inv = 1.0 / tot
            st[hg] = [a * inv for a in e]

        def apply(hg, d0):
            e = pace(st.pop(hg) if d0 else st[hg], 32)
            for d in range(d0, d0 + DH // 2, 4):
                o = []
                for r in (pl.ds(128 * hg + 8 * (d + n), 8) for n in range(4)):
                    acc = e[0] * ve[p, 7 + jj, r]
                    for w in range(1, WIN):
                        acc = acc + e[w] * ve[p, 7 + jj - w, r]
                    o.append(acc)
                os_.at[j][pl.ds(32 * hg + 2 * d, 8)] = _pk4(o)

        return [(c, lambda f=f, hg=hg, d0=d0: f(hg, d0)) for hg in range(4)
                for c, f, d0 in ((33, probs, 0), (45, probs, 8), (32, apply, 0), (32, apply, 8))]

    def wout(j):
        def run(b):
            r = pl.ds(128 * b, 128)
            y = _dot(_bf(wot[64 * b:64 * b + 64]), _rows(os_, j, 0, D))
            mark(y)
            xr[j, r] = xr[j, r] + y
        return [(128, lambda b=b: run(b)) for b in range(4)]

    def dft(src, mat, c0, n, more=False):
        def run(j):
            rows = pl.ds(c0, n)
            a, b = (_dot(src(i, c0, n), _bf(mat[i])) for i in (j, j + 8))
            for h, z in enumerate((a + b, a - b)):
                i = 8 * h + j
                res = {i: (z[:, :128], z[:, 128:])}
                if more and 4 <= j < 7:
                    res[i - 4], res[i] = second((zs[0, i - 4, rows], zs[1, i - 4, rows]), res[i], j - 4, h)
                for k, v in res.items():
                    zs[0, k, rows], zs[1, k, rows] = v
            mark(z)
        return [(n, lambda j=j: run(j)) for j in range(NJ // 2)]

    def second(p, q, j0, h):
        return [_twiddle(v, j0 * (h + 2 * i)) for i, v in enumerate(_half4(p, q, h))]

    def spectrum(rows, h, cost, done=0):
        z = [(zs[0, 8 * h + j, rows], zs[1, 8 * h + j, rows]) for j in range(8)]
        paced = (0, 3, 4) if done else (0, 1, 2, 3)
        pz = pace([c for i in paced for c in z[i]], cost)
        for n, i in enumerate(paced):
            z[i] = tuple(pz[2 * n:2 * n + 2])
        a = [(z[j0], z[j0 + 4]) if j0 < done else second(z[j0], z[j0 + 4], j0, h) for j0 in range(4)]
        return [_bfly4([a[j0][i] for j0 in range(4)], False) for i in range(2)]

    def fft(c0, n):
        def run(r0, h):
            rows = pl.ds(r0, 8)
            b = []
            for i, xs_ in enumerate(spectrum(rows, h, 40 + 6 * h, 3)):
                m0 = h + 2 * i
                y = [_cmul(v, (kf[0, 4 * m0 + m1, rows], kf[1, 4 * m0 + m1, rows]))
                     for m1, v in enumerate(xs_)]
                b.append([_twiddle(v, -j0 * m0) for j0, v in enumerate(_bfly4(y, True))])
            for j0 in range(4):
                (ar, ai), (br, bi) = b[0][j0], b[1][j0]
                lo = (ar + br, ai + bi)
                hi = (bi - ai, ar - br) if h else (ar - br, ai - bi)
                for c in range(2):
                    zs[c, 8 * h + j0, rows] = lo[c]
                    zs[c, 8 * h + j0 + 4, rows] = hi[c]
        return [(40 + 6 * h, lambda r0=r0, h=h: run(r0, h))
                for r0 in range(c0, c0 + n, 8) for h in range(2)]

    def inv(c0, n, js):
        def run(j):
            rows = pl.ds(c0, n)
            a, b = (jnp.concatenate([zs[0, i, rows], zs[1, i, rows]], axis=1) for i in (j, j + 8))
            ys = [_dot(z.astype(BF16), _bf(fm[i]), NT) for i, z in ((j, a + b), (j + 8, a - b))]
            for i, y in zip((j, j + 8), ys):
                xr[i, rows] = xr[i, rows] + y
            mark(ys[0])
        return [(n, lambda j=j: run(j)) for j in js]

    def cat(lists):
        return [t for l in lists for t in l]

    k_steps, tab = [], [k_tables(g) for g in range(64)] + [[], [], []]
    for g in range(-2, 64):
        mm, post = k_matmul(g) if g >= 0 else ([], [])
        k_steps.append(mm + tab[g + 1][1:2] + tab[g + 2][:1] + post + tab[g + 1][2:])

    order = [j0 + d for j0 in (0, 2, 1, 3) for d in (0, 8, 4, 12)]

    def lane_dft(n):
        return [dft(lambda *a: _rows(xn, *a), fm, c, 128, True)[order[2 * n]] for c in range(0, D, 128)]

    def attention(pre, extra):
        steps = [pre[0] + pre[1] + ln(order[0])]
        for i in range(8):
            steps.append(overlap(kv(order[i]) + pre[i + 2], ln(order[i + 1]), extra[i]))
        steps.append(qproj(order[0]))
        for i in range(NJ + 4):
            wo_, ln2 = ([order[n] for n in (2 * k - 1, 2 * k) if 0 <= n < NJ] for k in (i - 8, i - 9))
            m = pre[i + 10] if i < 6 else []
            m = m + _merge(kv(order[8 + i]) if i < 8 else [],
                           qproj(order[i + 1]) if i + 1 < NJ else [], cat(wout(j) for j in wo_))
            if i >= 12:
                m = _merge(m, [t for c, t in enumerate(lane_dft(i - 12)) if (i - 12, c) not in LATE])
            v = (ln(order[8 + i + 1]) if i < 7 else []) + cat(ln(j) for j in ln2)
            c = core(order[i]) if i < NJ else []
            if i >= NJ - 1:
                c, v = (t + [(0.25 * sum(x for x, _ in t), lambda: None)] for t in (c, v))
            steps.append(overlap(m, c, v))
        return steps

    def ssm(last):
        prog = [(0, barrier)]
        for c in range(0, D, G):
            out = cat(x_out(c // 128 - 1, j2) for j2 in range(8)) if last and c > 128 and c % 128 else []
            prog += overlap(inv(c - G, G, range(NJ // 2)) if c else [lane_dft(n)[b] for n, b in LATE],
                            fft(c, G), out)
            if out and c > 256:
                prog += [(0, barrier)]
        return prog

    def wait(*cps):
        def run():
            for c in cps:
                c.wait()
            marks[:], used[:] = [], []
        return [(0, run)]

    def start(*cps):
        return [(0, lambda: [c.start() for c in cps])]

    kd = [dft(lambda j, c0, n: _bf(kt[j // 2, pl.ds(c0 // 2, n // 2), pl.ds(128 * (j % 2), 128)]),
              fk, c, 128) for c in range(0, D, 128)]
    a1 = attention([[]] * NJ, [cat(k_fft(g) for g in range(8 * i, 8 * i + 8)) for i in range(8)])
    head = wait(*cp_p[0]) + [(1, step_size)] + cat(k_steps[:P0 // 8]) + wait(*cp_p[1]) + start(cp_wqkv, *cp_x, cp_fk)
    head += cat(k_steps[P0 // 8:]) + wait(cp_wqkv, *cp_x, cp_fk) + start(cp_wo, cp_f) + [(1, d_skip)]
    head += _merge(_merge(cat(kd), cat(w_qkv(b) for b in range(12))),
                   x_in(0) + a1[0] + cat(x_in(j2) for j2 in range(1, 8)))
    head += [(0, barrier)]
    prog = head + cat(a1[1:9]) + wait(cp_wo, cp_f) + w_out(0) + w_out(1)
    prog += cat(a1[9:]) + ssm(False)
    a2 = attention([inv(D - G, G, [j]) if j < 8 else [] for j in order], [[]] * 8)
    prog += cat(a2)
    prog += ssm(True)
    prog += inv(D - G, G, range(NJ // 2))
    prog += cat(x_out(3, j2) for j2 in (0, 4, 1, 5, 2, 6, 3, 7))
    for _, fn in prog:
        fn()
    for c in cp_o:
        c.wait()


@jax.jit
def pallas_interleave_layers__sliding_local_dilated__ssm_conv_s4__prompt_kernel(
    A_x: jax.Array,
    A_wqkv: jax.Array,
    A_wo: jax.Array,
    B_u: jax.Array,
    B_A_re: jax.Array,
    B_A_im: jax.Array,
    B_B_re: jax.Array,
    B_B_im: jax.Array,
    B_C_re: jax.Array,
    B_C_im: jax.Array,
    B_log_dt: jax.Array,
    B_Dskip: jax.Array,
):
    del B_u
    hbm = pl.BlockSpec(memory_space=pl.ANY)
    out = pl.pallas_call(
        _kernel,
        in_specs=[hbm] * 14,
        out_specs=hbm,
        out_shape=jax.ShapeDtypeStruct((S, D), BF16),
        scratch_shapes=[
            pltpu.VMEM((2, NA, NA), BF16),
            pltpu.VMEM((D,), BF16),
            pltpu.VMEM((D,), BF16),
            pltpu.VMEM((6, D, 128), BF16),
            pltpu.VMEM((4, S // 2, 128), U32),
            pltpu.VMEM((D, 3 * D), BF16),
            pltpu.VMEM((D, D), BF16),
            pltpu.VMEM((NJ, NA // 2, 256), U32),
            pltpu.VMEM((NJ, NA // 2, 256), U32),
            pltpu.VMEM((D, 128), F32),
            pltpu.VMEM((D, 128), F32),
            pltpu.VMEM((NJ // 2, D // 2, 256), U32),
            pltpu.VMEM((3 * D // 2, D), U32),
            pltpu.VMEM((D // 2, D), U32),
            pltpu.VMEM((NJ, D // 4, 256), U32),
            pltpu.VMEM((NJ, D // 4, 256), U32),
            pltpu.VMEM((NJ, D, NA), F32),
            pltpu.VMEM((NJ, D, NA), F32),
            pltpu.VMEM((2, NJ - 1, D, NA), F32),
            pltpu.VMEM((2, NJ - 1, D, NA), F32),
            pltpu.VMEM((2, NJ, D, NA), F32),
            pltpu.VMEM((2, NJ, D, NA), F32),
            pltpu.VMEM((24, NA), U32),
            pltpu.SemaphoreType.DMA((8,)),
            pltpu.SemaphoreType.DMA((4,)),
            pltpu.SemaphoreType.DMA((15,)),
            pltpu.SemaphoreType.REGULAR,
        ],
        compiler_params=pltpu.CompilerParams(vmem_limit_bytes=100 << 20),
    )(A_x.reshape(S, D), A_wqkv, A_wo, _F, _FK,
      B_A_re, B_A_im, B_B_re, B_B_im, B_C_re, B_C_im,
      _PM, B_log_dt, B_Dskip)
    return out.reshape(1, S, D)
```

```python
import math

import jax
import jax.numpy as jnp
import ml_dtypes
import numpy as np
import jax.experimental.pallas as pl
import jax.experimental.pallas.tpu as pltpu

S, D, H, DH, WIN = 2048, 512, 32, 16, 8
NJ, NA = 16, 128
EPS = 1e-5
F32, BF16, U32, I32 = jnp.float32, jnp.bfloat16, jnp.uint32, jnp.int32
LG, G = 24, 64
PAIRS_AT = {13: (0,), 14: (2,), 15: (4,), 16: (1,), 17: (3, 5), 18: (6, 7)}
LATE = ((7, 2), (6, 3), (7, 3))
P0 = 80
NT = (((1,), (1,)), ((), ()))


def _dft_consts():
    a = np.arange(NA)[None, :, None]
    j = np.arange(NJ)[:, None, None]
    k = np.arange(NA)[None, None, :]
    th = np.pi * (((NJ * a + j) * (2 * k + 1)) % (4 * S)) / (2 * S)
    f = np.concatenate([np.cos(th), -np.sin(th)], axis=-1)
    lane = np.arange(NA)
    ln = (lane - 3) % NA
    fk = f[:, 32 * (ln % 4) + ln // 4, :]
    perm = np.zeros((NA, NA), np.float32)
    perm[lane, (lane % 8) * DH + lane // 8] = 1.0
    pm = np.stack([perm * DH ** -0.5, perm])
    bf = ml_dtypes.bfloat16
    return f.astype(bf), fk.astype(bf), pm.astype(bf)


_F, _FK, _PM = _dft_consts()


def _round_l(l):
    return int(np.float32(l).astype(ml_dtypes.bfloat16).astype(np.float32))


_R = [[_round_l(256 * q + j) - 256 * q for j in range(NJ)] for q in range(8)]
assert all(_round_l(256 * q + 16 * b + j) == 256 * q + 16 * b + _R[q][j]
           for q in range(8) for b in range(16) for j in range(NJ))
assert _R[2] == _R[3] and _R[4] == _R[5] == _R[6] == _R[7]
_PAIRS = ([((0, r), (0, r + 8)) for r in range(8)]
          + [((1, 0), (1, 4)), ((1, 8), (1, 12)), ((0, 16), (1, 16))]
          + [((2, r), (3, r)) for r in (0, 8, 16)])


def _cmul(x, y):
    return x[0] * y[0] - x[1] * y[1], x[0] * y[1] + x[1] * y[0]


def _csq(x):
    return x[0] * x[0] - x[1] * x[1], (x[0] + x[0]) * x[1]


def _bfly4(x, inv):
    (ar, ai), (br, bi), (cr, ci), (dr, di) = x
    sr, si, tr, ti = ar + cr, ai + ci, ar - cr, ai - ci
    ur, ui, vr, vi = br + dr, bi + di, br - dr, bi - di
    y1, y3 = (tr + vi, ti - vr), (tr - vi, ti + vr)
    if inv:
        y1, y3 = y3, y1
    return [(sr + ur, si + ui), y1, (sr - ur, si - ui), y3]


def _twiddle(x, e):
    e %= 16
    xr, xi = x
    if e == 0:
        return x
    if e == 4:
        return xi, -xr
    if e == 12:
        return -xi, xr
    c, s = math.cos(math.pi * e / 8), -math.sin(math.pi * e / 8)
    if e % 2 == 0:
        if c * s > 0:
            return (xr - xi) * c, (xr + xi) * c
        return (xr + xi) * c, (xi - xr) * c
    return xr * c - xi * s, xr * s + xi * c


def _half4(p, q, h):
    (pr, pi), (qr, qi) = p, q
    if h:
        return (pr + qi, pi - qr), (pr - qi, pi + qr)
    return (pr + qr, pi + qi), (pr - qr, pi - qi)


def _pk(x):
    return pltpu.bitcast(x.astype(BF16), U32)


def _pk4(u):
    return _pk(jnp.concatenate([jnp.concatenate(v, axis=0) for v in (u[:2], u[2:])], axis=1))


def _rows(ref, j, r0, n):
    return _bf(jnp.concatenate([ref[j, pl.ds(8 * (b // 2), 8), pl.ds(128 * (b % 2), 128)]
                                for b in range(r0 // 16, (r0 + n) // 16)], axis=0))


def _bf(x):
    return pltpu.bitcast(x, BF16)


def _dot(a, b, dims=(((1,), (0,)), ((), ()))):
    return jax.lax.dot_general(a, b, dims, preferred_element_type=F32)


def _merge(*streams):
    keyed = []
    for n, st in enumerate(streams):
        tot, acc = sum(c for c, _ in st) or 1, 0
        for t in st:
            keyed.append(((acc + 0.5 * t[0]) / tot, n, len(keyed), t))
            acc += t[0]
    return [k[-1] for k in sorted(keyed, key=lambda k: k[:3])]


def _flip8(x, sub):
    r = [pltpu.roll(x, k, 0) for k in (7, 5, 3, 1)]
    s4 = sub & 3
    return jnp.where(s4 == 3, r[0], jnp.where(s4 == 2, r[1], jnp.where(s4 == 1, r[2], r[3])))


def _kernel(x_hbm, wqkv_hbm, wo_hbm, f_hbm, fk_hbm,
            are_hbm, aim_hbm, bre_hbm, bim_hbm, cre_hbm, cim_hbm, pm_hbm, ldt_hbm, dsk_hbm,
            out_hbm,
            pm_ref, ldt_ref, dsk_ref, par_ref, xu, wqkv, wo, fm, fk, dtc, dsc, kt, wt, wot, xn, os_, xr, qs, ke, ve, kf, zs, zero,
            sem_in, sem_out, sem_p, sem_b):
    xb = xu.bitcast(BF16)
    cp_x = [pltpu.make_async_copy(x_hbm.at[:, pl.ds(128 * c, 128)], xb.at[c], sem_in.at[c])
            for c in range(4)]
    cp_wqkv = pltpu.make_async_copy(wqkv_hbm, wqkv, sem_in.at[4])
    cp_wo = pltpu.make_async_copy(wo_hbm, wo, sem_in.at[5])
    cp_fk = pltpu.make_async_copy(fk_hbm, fk.bitcast(BF16), sem_in.at[6])
    cp_f = pltpu.make_async_copy(f_hbm, fm.bitcast(BF16), sem_in.at[7])
    cp_o = [pltpu.make_async_copy(xb.at[c], out_hbm.at[:, pl.ds(128 * c, 128)], sem_out.at[c])
            for c in range(4)]
    cp_p = [[pltpu.make_async_copy(r.at[rows], par_ref.at[i, rows], sem_p.at[6 * h + i])
             for i, r in enumerate((are_hbm, aim_hbm, bre_hbm, bim_hbm, cre_hbm, cim_hbm))]
            for h, rows in enumerate((pl.ds(0, P0), pl.ds(P0, D - P0)))]
    cp_s = [pltpu.make_async_copy(a, b, sem_p.at[12 + i])
            for i, (a, b) in enumerate(((ldt_hbm, ldt_ref), (dsk_hbm, dsk_ref), (pm_hbm, pm_ref)))]
    cp_p = [cp_s[:1] + cp_p[0], cp_p[1] + cp_s[1:]]
    for c in cp_p[0] + cp_p[1]:
        c.start()

    for ref in (dtc, dsc, kt, wt, wot, xn, os_, xr, qs, ke, ve, kf, zs):
        ref[(0,) * (len(ref.shape) - 2) + (pl.ds(1, 8), pl.ds(0, 128))] = jnp.zeros((8, 128), ref.dtype)

    zero[pl.ds(1, 16)] = jnp.zeros((16, 128), U32)
    marks, used, rate = [], [], [1.0]

    def mark(x):
        marks.extend(x[r:r + 8, :128] for r in range(0, x.shape[0], 16) for _ in range(x.shape[1] // 128))

    def pace(vals, cost):
        if not marks:
            return list(vals)
        i = min(max(used + [0, len(marks) - LG]), len(marks) - 1)
        used[:] = [i + cost * rate[0] / 16]
        t = pltpu.bitcast(marks[int(i)], U32) & zero[8:16]
        return [pltpu.bitcast(pltpu.bitcast(v, U32) | t, F32) for v in vals]

    def overlap(m, *vs):
        r = sum(c for c, _ in m) / max(1, sum(c for v in vs for c, _ in v))
        return [(1, lambda: rate.__setitem__(0, r))] + _merge(m, *vs)

    def barrier():
        pl.semaphore_signal(sem_b, 1)
        pl.semaphore_wait(sem_b, 1)
        marks[:], used[:] = [], []

    def iota(axis):
        return jax.lax.broadcasted_iota(I32, (8, 128), axis)

    def step_size():
        dt_row = jnp.exp(ldt_ref[...].astype(F32).reshape(1, D)).astype(BF16).astype(F32)
        dtc[...] = jnp.broadcast_to(dt_row, (128, D)).T

    def d_skip():
        dsc[...] = jnp.broadcast_to(dsk_ref[...].astype(F32).reshape(1, D), (128, D)).T

    def k_tables(g):
        st = {}

        def par(i):
            return par_ref[i, 16 * (g // 2):16 * (g // 2) + 16].astype(F32)[8 * (g % 2):8 * (g % 2) + 8]

        def mix(u, v):
            lo = iota(0) < 4
            rv = [pltpu.roll(c, 4, 0) for c in v]
            return (tuple(jnp.where(lo, a, b) for a, b in zip(u, rv)),
                    tuple(jnp.where(lo, b, a) for a, b in zip(u, rv)))

        def put(name, t, two):
            kreg.setdefault((name, g, t), []).append(jnp.concatenate(
                [jnp.concatenate([two[0][c], two[1][c]], axis=0) for c in range(2)], axis=1))

        def base():
            dt, = pace([dtc[8 * g:8 * g + 8]], 100)
            zr, zi = dt * par(0), dt * par(1)
            mag = jnp.exp(zr)
            st[1] = (mag * jnp.cos(zi), mag * jnp.sin(zi))
            st[0] = _cmul((par(4), par(5)), (dt * par(2), dt * par(3)))

        def left():
            lam = {1: st[1]}
            for p in range(1, 10):
                lam[2 ** p] = _csq(lam[2 ** (p - 1)])
            st[16] = lam[16]
            e = {(0, 0): st[0]}
            for a1 in (1, 2, 3):
                e[a1, 0] = _cmul(e[a1 - 1, 0], lam[512])
            for a1, r in ((0, 8), (1, 4), (0, 16), (1, 16)):
                e[a1, r] = _cmul(e[a1, 0], lam[r])
            d1, d8 = mix(lam[1], lam[1]), mix(lam[8], lam[8])
            prev, done = None, []
            for i, (u, v) in enumerate(_PAIRS):
                if u in e:
                    cur = mix(e[u], e[v])
                else:
                    m = d1 if i < 8 else d8
                    cur = (_cmul(prev[0], m[0]), _cmul(prev[1], m[1]))
                prev = cur
                done.append(cur)
                if i % 2:
                    for t in range(2):
                        put("l", t, (done[i - 1][t], done[i][t]))

        def right(t):
            lo = iota(0) < 4
            if t == 0:
                f = (_flip8(st[16][0], iota(0)), -_flip8(st[16][1], iota(0)))
                st["d"] = mix(f, f)[::-1]
            d = st["d"][t]
            d2 = _csq(d)
            one = (1.0, 0.0)
            cur = tuple(jnp.where(lo, a, b) for a, b in (zip(one, d), zip(d, d2))[t])
            for v in range(0, 16, 2):
                if v:
                    cur = _cmul(cur, d2)
                nxt = _cmul(cur, d2)
                if t and v == 14:
                    nxt = tuple(jnp.where(lo, a, b) for a, b in zip(nxt, one))
                put("r", t, (cur, nxt))
                cur = nxt

        return [(45, base), (70, left), (35, lambda: right(0)), (30, lambda: right(1))]

    kreg = {}

    def k_matmul(g):
        def mm():
            kreg[g] = [_dot(*(jnp.concatenate(kreg.pop((n, g, t)), axis=0).astype(BF16)
                              for n in "lr"), NT) for t in range(2)]

        def post():
            o0, o1 = kreg.pop(g)
            mark(o0); mark(o1)
            lo = iota(0) < 4
            ln = (iota(1) + (NA - 3)) & (NA - 1)
            piece = {}
            for i, (u, v) in enumerate(_PAIRS):
                a, b = o0[8 * i:8 * i + 8], o1[8 * i:8 * i + 8]
                for e, x in ((u, jnp.where(lo, a, b)), (v, pltpu.roll(jnp.where(lo, b, a), 4, 0))):
                    piece[e] = pltpu.roll(x, e[0], 1, stride=1, stride_axis=0)
            memo, res = {}, []
            for j in range(NJ):
                r2, r4, r8 = _R[1][j], _R[2][j], _R[4][j]
                if r8 not in memo:
                    memo[r8] = jnp.where((ln & 3) == 2, piece[2, r8], piece[3, r8])
                if (r4, r8) not in memo:
                    memo[r4, r8] = jnp.where((ln & 3) == 1, piece[1, r4], memo[r8])
                x = piece[0, j] if r2 == j else jnp.where(ln < 64, piece[0, j], piece[0, r2])
                res.append(jnp.where((ln & 3) == 0, x, memo[r4, r8]))
            if g % 2 == 0:
                kreg["even"] = res
            else:
                ev = kreg.pop("even")
                for j in range(0, NJ, 2):
                    kt.at[j // 2][4 * g - 4:4 * g + 4] = _pk4([ev[j], res[j], ev[j + 1], res[j + 1]])

        return [(5, mm)], [(30, post)]

    def k_fft(g):
        def run(h):
            rows = pl.ds(8 * g, 8)
            dsk = dsc[rows]
            for i, xs_ in enumerate(spectrum(rows, h, 20 + 6 * h)):
                for m1, (yr, yi) in enumerate(xs_):
                    kf[0, 4 * (h + 2 * i) + m1, rows] = (yr + dsk) * (1.0 / S)
                    kf[1, 4 * (h + 2 * i) + m1, rows] = yi * (1.0 / S)
        return [(20 + 6 * h, lambda h=h: run(h)) for h in range(2)]

    def w_qkv(b):
        def run():
            cols = pl.ds(128 * b, 128)
            w = _dot(pm_ref[0 if b < 4 else 1], wqkv[:, cols], NT)
            wt[64 * b:64 * b + 64] = _pk(w)
        return [(128, run)]

    def w_out(b):
        def run():
            wot[:, 256 * b:256 * b + 256] = _pk(jnp.concatenate(
                [_dot(pm_ref[1], wo[r:r + 128]).T for r in (256 * b, 256 * b + 128)], axis=1))
        return [(256, run)]

    def x_in(j2):
        def run(c):
            v = xu[c, pl.ds(j2, NA, stride=NJ // 2), :].T
            xr[2 * j2, 128 * c:128 * c + 128] = pltpu.bitcast(v << 16, F32)
            xr[2 * j2 + 1, 128 * c:128 * c + 128] = pltpu.bitcast(v & np.uint32(0xFFFF0000), F32)
        return [(40, lambda c=c: run(c)) for c in range(4)]

    def x_out(c, j2):
        def run():
            u = jnp.concatenate([xr[j, 128 * c:128 * c + 128] for j in (2 * j2, 2 * j2 + 1)], axis=1)
            u = pltpu.bitcast(u.astype(BF16).astype(F32), U32)
            v = (u[:, :128] >> 16) | u[:, 128:]
            xu[c, pl.ds(j2, NA, stride=NJ // 2), :] = v.T
            if j2 == NJ // 2 - 1:
                cp_o[c].start()
        return [(25, run)]

    def tree(acc, xs_):
        acc = list(acc)
        for i, x in enumerate(xs_):
            acc[i % 4] = acc[i % 4] + x
        return acc

    def total(acc):
        return jnp.broadcast_to(
            jnp.sum((acc[0] + acc[1]) + (acc[2] + acc[3]), axis=0, keepdims=True), (8, 128))

    def ln(j):
        st = {}

        def mean():
            v = [xr[j, r:r + 8] for r in range(0, D, 8)]
            st["m"] = total(tree(pace(v[:4], 18), v[4:])) * (1.0 / D)

        def var(r0):
            m, = pace([st["m"]], 25)
            c = [xr[j, r:r + 8] - m for r in range(r0, r0 + D // 2, 8)]
            c = [v * v for v in c]
            if r0:
                st["s"] = jax.lax.rsqrt(total(tree(st["v"], c)) * (1.0 / D) + EPS)
            else:
                st["v"] = tree(c[:4], c[4:])

        def norm():
            for r in range(0, D, 32):
                if r % 128 == 0:
                    m, s_ = pace([st["m"], st["s"]], 10)
                u = [(xr[j, r + h:r + h + 8] - m) * s_ for h in range(0, 32, 8)]
                xn.at[j][r // 4:r // 4 + 8] = _pk4(u)

        return [(18, mean), (25, lambda: var(0)), (25, lambda: var(D // 2)), (40, norm)]

    def kv(j):
        p, jj = j & 1, j >> 1

        def run(dst, b):
            k = _dot(_bf(wt[64 * b:64 * b + 64]), _rows(xn, j, 0, D))
            mark(k)
            r = pl.ds(128 * (b % 4), 128)
            dst[p, 7 + jj, r] = k
            if jj:
                dst[p, jj - 1, r] = pltpu.roll(k, 1, 1)

        return [(128, lambda b=b: run(ke if b < 8 else ve, b)) for b in range(4, 12)]

    def qproj(j):
        def run(b):
            q = _dot(_bf(wt[64 * b:64 * b + 64]), _rows(xn, j, 0, D))
            mark(q)
            qs[j, 128 * b:128 * b + 128] = q
        return [(128, lambda b=b: run(b)) for b in range(4)]

    def core(j):
        p, jj = j & 1, j >> 1
        st = {}

        def probs(hg, d0):
            s = st.pop(hg) if d0 else [None] * WIN
            rows = [pl.ds(128 * hg + 8 * d, 8) for d in range(d0, d0 + DH // 2)]
            qv = [qs[j, r] for r in rows]
            for r, q in zip(rows, pace(qv[:4], 16) + pace(qv[4:], 29 if d0 else 17)):
                for w in range(WIN):
                    t = q * ke[p, 7 + jj - w, r]
                    s[w] = t if s[w] is None else s[w] + t
            if not d0:
                st[hg] = s
                return
            for w in range(jj + 1, WIN):
                s[w] = jnp.where(iota(1) >= 1, s[w], -1e9)
            m = s[0]
            for w in range(1, WIN):
                m = jnp.maximum(m, s[w])
            e = [jnp.exp(a - m) for a in s]
            tot = e[0]
            for w in range(1, WIN):
                tot = tot + e[w]
            inv = 1.0 / tot
            st[hg] = [a * inv for a in e]

        def apply(hg, d0):
            e = pace(st.pop(hg) if d0 else st[hg], 32)
            for d in range(d0, d0 + DH // 2, 4):
                o = []
                for r in (pl.ds(128 * hg + 8 * (d + n), 8) for n in range(4)):
                    acc = e[0] * ve[p, 7 + jj, r]
                    for w in range(1, WIN):
                        acc = acc + e[w] * ve[p, 7 + jj - w, r]
                    o.append(acc)
                os_.at[j][pl.ds(32 * hg + 2 * d, 8)] = _pk4(o)

        return [(c, lambda f=f, hg=hg, d0=d0: f(hg, d0)) for hg in range(4)
                for c, f, d0 in ((33, probs, 0), (45, probs, 8), (32, apply, 0), (32, apply, 8))]

    def wout(j):
        def run(b):
            r = pl.ds(128 * b, 128)
            y = _dot(_bf(wot[64 * b:64 * b + 64]), _rows(os_, j, 0, D))
            mark(y)
            xr[j, r] = xr[j, r] + y
        return [(128, lambda b=b: run(b)) for b in range(4)]

    def dft(src, mat, c0, n, more=False):
        def run(j):
            rows = pl.ds(c0, n)
            a, b = (_dot(src(i, c0, n), _bf(mat[i])) for i in (j, j + 8))
            for h, z in enumerate((a + b, a - b)):
                i = 8 * h + j
                res = {i: (z[:, :128], z[:, 128:])}
                if more and 4 <= j < 7:
                    res[i - 4], res[i] = second((zs[0, i - 4, rows], zs[1, i - 4, rows]), res[i], j - 4, h)
                for k, v in res.items():
                    zs[0, k, rows], zs[1, k, rows] = v
            if more:
                mark(z)
        return [(n, lambda j=j: run(j)) for j in range(NJ // 2)]

    def second(p, q, j0, h):
        return [_twiddle(v, j0 * (h + 2 * i)) for i, v in enumerate(_half4(p, q, h))]

    def spectrum(rows, h, cost, done=0):
        z = [(zs[0, 8 * h + j, rows], zs[1, 8 * h + j, rows]) for j in range(8)]
        paced = (0, 3, 4) if done else (0, 1, 2, 3)
        pz = pace([c for i in paced for c in z[i]], cost)
        for n, i in enumerate(paced):
            z[i] = tuple(pz[2 * n:2 * n + 2])
        a = [(z[j0], z[j0 + 4]) if j0 < done else second(z[j0], z[j0 + 4], j0, h) for j0 in range(4)]
        return [_bfly4([a[j0][i] for j0 in range(4)], False) for i in range(2)]

    def fft(c0, n):
        def run(r0, h):
            rows = pl.ds(r0, 8)
            b = []
            for i, xs_ in enumerate(spectrum(rows, h, 40 + 6 * h, 3)):
                m0 = h + 2 * i
                y = [_cmul(v, (kf[0, 4 * m0 + m1, rows], kf[1, 4 * m0 + m1, rows]))
                     for m1, v in enumerate(xs_)]
                b.append([_twiddle(v, -j0 * m0) for j0, v in enumerate(_bfly4(y, True))])
            for j0 in range(4):
                (ar, ai), (br, bi) = b[0][j0], b[1][j0]
                lo = (ar + br, ai + bi)
                hi = (bi - ai, ar - br) if h else (ar - br, ai - bi)
                for c in range(2):
                    zs[c, 8 * h + j0, rows] = lo[c]
                    zs[c, 8 * h + j0 + 4, rows] = hi[c]
        return [(40 + 6 * h, lambda r0=r0, h=h: run(r0, h))
                for r0 in range(c0, c0 + n, 8) for h in range(2)]

    def inv(c0, n, js):
        def run(j):
            rows = pl.ds(c0, n)
            a, b = (jnp.concatenate([zs[0, i, rows], zs[1, i, rows]], axis=1) for i in (j, j + 8))
            ys = [_dot(z.astype(BF16), _bf(fm[i]), NT) for i, z in ((j, a + b), (j + 8, a - b))]
            for i, y in zip((j, j + 8), ys):
                xr[i, rows] = xr[i, rows] + y
            mark(ys[0])
        return [(n, lambda j=j: run(j)) for j in js]

    def cat(lists):
        return [t for l in lists for t in l]

    k_steps, tab = [], [k_tables(g) for g in range(64)] + [[], [], []]
    for g in range(-2, 64):
        mm, post = k_matmul(g) if g >= 0 else ([], [])
        k_steps.append(mm + tab[g + 1][1:2] + tab[g + 2][:1] + post + tab[g + 1][2:])

    order = [j0 + d for j0 in (0, 2, 1, 3) for d in (0, 8, 4, 12)]

    def lane_dft(n):
        return [dft(lambda *a: _rows(xn, *a), fm, c, 128, True)[order[2 * n]] for c in range(0, D, 128)]

    def attention(pre, extra):
        steps = [pre[0] + pre[1] + ln(order[0])]
        for i in range(8):
            steps.append(overlap(kv(order[i]) + pre[i + 2], ln(order[i + 1]), extra[i]))
        steps.append(qproj(order[0]))
        for i in range(NJ + 4):
            wo_, ln2 = ([order[n] for n in (2 * k - 1, 2 * k) if 0 <= n < NJ] for k in (i - 8, i - 9))
            m = pre[i + 10] if i < 6 else []
            m = m + _merge(kv(order[8 + i]) if i < 8 else [],
                           qproj(order[i + 1]) if i + 1 < NJ else [], cat(wout(j) for j in wo_))
            m = _merge(m, [t for n in PAIRS_AT.get(i, ()) for c, t in enumerate(lane_dft(n))
                           if (n, c) not in LATE])
            v = (ln(order[8 + i + 1]) if i < 7 else []) + cat(ln(j) for j in ln2)
            c = core(order[i]) if i < NJ else []
            if i >= NJ - 1:
                c, v = (t + [(0.25 * sum(x for x, _ in t), lambda: None)] for t in (c, v))
            steps.append(overlap(m, c, v))
        return steps

    def ssm(last):
        prog = [(0, barrier)]
        for c in range(0, D, G):
            out = cat(x_out(c // 128 - 1, j2) for j2 in range(8)) if last and c > 128 and c % 128 else []
            prog += overlap(inv(c - G, G, range(NJ // 2)) if c else [lane_dft(n)[b] for n, b in LATE],
                            fft(c, G), out)
            if out and c > 256:
                prog += [(0, barrier)]
        return prog

    def wait(*cps):
        def run():
            for c in cps:
                c.wait()
            marks[:], used[:] = [], []
        return [(0, run)]

    def start(*cps):
        return [(0, lambda: [c.start() for c in cps])]

    kd = [dft(lambda j, c0, n: _bf(kt[j // 2, pl.ds(c0 // 2, n // 2), pl.ds(128 * (j % 2), 128)]),
              fk, c, 128) for c in range(0, D, 128)]
    a1 = attention([[]] * NJ, [cat(k_fft(g) for g in range(8 * i, 8 * i + 8)) for i in range(8)])
    head = wait(*cp_p[0]) + [(1, step_size)] + cat(k_steps[:P0 // 8]) + wait(*cp_p[1])
    head += start(cp_fk, cp_wqkv, *cp_x) + cat(k_steps[P0 // 8:40]) + wait(cp_fk)
    head += _merge(cat(k_steps[40:]), kd[0] + kd[1]) + wait(cp_wqkv, *cp_x) + start(cp_wo, cp_f) + [(1, d_skip)]
    head += _merge(_merge(kd[2] + kd[3], cat(w_qkv(b) for b in range(12))),
                   x_in(0) + a1[0] + cat(x_in(j2) for j2 in range(1, 8)))
    head += [(0, barrier)]
    prog = head + cat(a1[1:9]) + wait(cp_wo, cp_f) + w_out(0) + w_out(1)
    prog += cat(a1[9:]) + ssm(False)
    a2 = attention([inv(D - G, G, [j]) if j < 8 else [] for j in order], [[]] * 8)
    prog += cat(a2)
    prog += ssm(True)
    prog += inv(D - G, G, range(NJ // 2))
    prog += cat(x_out(3, j2) for j2 in (0, 4, 1, 5, 2, 6, 3, 7))
    for _, fn in prog:
        fn()
    for c in cp_o:
        c.wait()


@jax.jit
def pallas_interleave_layers__sliding_local_dilated__ssm_conv_s4__prompt_kernel(
    A_x: jax.Array,
    A_wqkv: jax.Array,
    A_wo: jax.Array,
    B_u: jax.Array,
    B_A_re: jax.Array,
    B_A_im: jax.Array,
    B_B_re: jax.Array,
    B_B_im: jax.Array,
    B_C_re: jax.Array,
    B_C_im: jax.Array,
    B_log_dt: jax.Array,
    B_Dskip: jax.Array,
):
    del B_u
    hbm = pl.BlockSpec(memory_space=pl.ANY)
    out = pl.pallas_call(
        _kernel,
        in_specs=[hbm] * 14,
        out_specs=hbm,
        out_shape=jax.ShapeDtypeStruct((S, D), BF16),
        scratch_shapes=[
            pltpu.VMEM((2, NA, NA), BF16),
            pltpu.VMEM((D,), BF16),
            pltpu.VMEM((D,), BF16),
            pltpu.VMEM((6, D, 128), BF16),
            pltpu.VMEM((4, S // 2, 128), U32),
            pltpu.VMEM((D, 3 * D), BF16),
            pltpu.VMEM((D, D), BF16),
            pltpu.VMEM((NJ, NA // 2, 256), U32),
            pltpu.VMEM((NJ, NA // 2, 256), U32),
            pltpu.VMEM((D, 128), F32),
            pltpu.VMEM((D, 128), F32),
            pltpu.VMEM((NJ // 2, D // 2 + 8, 256), U32),
            pltpu.VMEM((3 * D // 2, D), U32),
            pltpu.VMEM((D // 2, D), U32),
            pltpu.VMEM((NJ, D // 4 + 8, 256), U32),
            pltpu.VMEM((NJ, D // 4 + 8, 256), U32),
            pltpu.VMEM((NJ, D + 24, NA), F32),
            pltpu.VMEM((NJ, D + 24, NA), F32),
            pltpu.VMEM((2, NJ - 1, D + 24, NA), F32),
            pltpu.VMEM((2, NJ - 1, D + 24, NA), F32),
            pltpu.VMEM((2, NJ, D + 24, NA), F32),
            pltpu.VMEM((2, NJ, D + 24, NA), F32),
            pltpu.VMEM((24, NA), U32),
            pltpu.SemaphoreType.DMA((8,)),
            pltpu.SemaphoreType.DMA((4,)),
            pltpu.SemaphoreType.DMA((15,)),
            pltpu.SemaphoreType.REGULAR,
        ],
        compiler_params=pltpu.CompilerParams(vmem_limit_bytes=100 << 20),
    )(A_x.reshape(S, D), A_wqkv, A_wo, _F, _FK,
      B_A_re, B_A_im, B_B_re, B_B_im, B_C_re, B_C_im,
      _PM, B_log_dt, B_Dskip)
    return out.reshape(1, S, D)
```

```python
import math

import jax
import jax.numpy as jnp
import ml_dtypes
import numpy as np
import jax.experimental.pallas as pl
import jax.experimental.pallas.tpu as pltpu

S, D, H, DH, WIN = 2048, 512, 32, 16, 8
NJ, NA = 16, 128
EPS = 1e-5
F32, BF16, U32, I32 = jnp.float32, jnp.bfloat16, jnp.uint32, jnp.int32
LG = 24
G = 64
P0 = 80
PAD = 24
PAIRS_AT = {13: (0,), 14: (2,), 15: (4,), 16: (1,), 17: (3, 5), 18: (6, 7)}
LATE = ((7, 2), (6, 3), (7, 3))
NT = (((1,), (1,)), ((), ()))


def _dft_consts():
    a = np.arange(NA)[None, :, None]
    j = np.arange(NJ)[:, None, None]
    k = np.arange(NA)[None, None, :]
    th = np.pi * (((NJ * a + j) * (2 * k + 1)) % (4 * S)) / (2 * S)
    f = np.concatenate([np.cos(th), -np.sin(th)], axis=-1)
    lane = np.arange(NA)
    ln = (lane - 3) % NA
    fk = f[:, 32 * (ln % 4) + ln // 4, :]
    perm = np.zeros((NA, NA), np.float32)
    perm[lane, (lane % 8) * DH + lane // 8] = 1.0
    pm = np.stack([perm * DH ** -0.5, perm])
    bf = ml_dtypes.bfloat16
    return f.astype(bf), fk.astype(bf), pm.astype(bf)


_F, _FK, _PM = _dft_consts()


def _round_l(l):
    return int(np.float32(l).astype(ml_dtypes.bfloat16).astype(np.float32))


_R = [[_round_l(256 * q + j) - 256 * q for j in range(NJ)] for q in range(8)]
assert all(_round_l(256 * q + 16 * b + j) == 256 * q + 16 * b + _R[q][j]
           for q in range(8) for b in range(16) for j in range(NJ))
assert _R[2] == _R[3] and _R[4] == _R[5] == _R[6] == _R[7]
_PAIRS = ([((0, r), (0, r + 8)) for r in range(8)]
          + [((1, 0), (1, 4)), ((1, 8), (1, 12)), ((0, 16), (1, 16))]
          + [((2, r), (3, r)) for r in (0, 8, 16)])


def _cmul(x, y):
    return x[0] * y[0] - x[1] * y[1], x[0] * y[1] + x[1] * y[0]


def _csq(x):
    return x[0] * x[0] - x[1] * x[1], (x[0] + x[0]) * x[1]


def _bfly4(x, inv):
    (ar, ai), (br, bi), (cr, ci), (dr, di) = x
    sr, si, tr, ti = ar + cr, ai + ci, ar - cr, ai - ci
    ur, ui, vr, vi = br + dr, bi + di, br - dr, bi - di
    y1, y3 = (tr + vi, ti - vr), (tr - vi, ti + vr)
    if inv:
        y1, y3 = y3, y1
    return [(sr + ur, si + ui), y1, (sr - ur, si - ui), y3]


def _twiddle(x, e):
    e %= 16
    xr, xi = x
    if e == 0:
        return x
    if e == 4:
        return xi, -xr
    if e == 12:
        return -xi, xr
    c, s = math.cos(math.pi * e / 8), -math.sin(math.pi * e / 8)
    if e % 2 == 0:
        if c * s > 0:
            return (xr - xi) * c, (xr + xi) * c
        return (xr + xi) * c, (xi - xr) * c
    return xr * c - xi * s, xr * s + xi * c


def _half4(p, q, h):
    (pr, pi), (qr, qi) = p, q
    if h:
        return (pr + qi, pi - qr), (pr - qi, pi + qr)
    return (pr + qr, pi + qi), (pr - qr, pi - qi)


def _pk(x):
    return pltpu.bitcast(x.astype(BF16), U32)


def _pk4(u):
    return _pk(jnp.concatenate([jnp.concatenate(v, axis=0) for v in (u[:2], u[2:])], axis=1))


def _rows(ref, j, r0, n):
    return _bf(jnp.concatenate([ref[j, pl.ds(8 * (b // 2), 8), pl.ds(128 * (b % 2), 128)]
                                for b in range(r0 // 16, (r0 + n) // 16)], axis=0))


def _bf(x):
    return pltpu.bitcast(x, BF16)


def _dot(a, b, dims=(((1,), (0,)), ((), ()))):
    return jax.lax.dot_general(a, b, dims, preferred_element_type=F32)


def _merge(*streams):
    keyed = []
    for n, st in enumerate(streams):
        tot, acc = sum(c for c, _ in st) or 1, 0
        for t in st:
            keyed.append(((acc + 0.5 * t[0]) / tot, n, len(keyed), t))
            acc += t[0]
    return [k[-1] for k in sorted(keyed, key=lambda k: k[:3])]


def _flip8(x, sub):
    r = [pltpu.roll(x, k, 0) for k in (7, 5, 3, 1)]
    s4 = sub & 3
    return jnp.where(s4 == 3, r[0], jnp.where(s4 == 2, r[1], jnp.where(s4 == 1, r[2], r[3])))


def _kernel(x_hbm, wqkv_hbm, wo_hbm, f_hbm, fk_hbm,
            are_hbm, aim_hbm, bre_hbm, bim_hbm, cre_hbm, cim_hbm, pm_hbm, ldt_hbm, dsk_hbm,
            out_hbm,
            pm_ref, ldt_ref, dsk_ref, par_ref, xu, wqkv, wo, fm, fk, dtc, dsc, kt, wt, wot,
            xn, os_, xr, qs, ke, ve, kf, zs, zero,
            sem_in, sem_out, sem_p, sem_b):
    xb = xu.bitcast(BF16)
    cp_x = [pltpu.make_async_copy(x_hbm.at[:, pl.ds(128 * c, 128)], xb.at[c], sem_in.at[c])
            for c in range(4)]
    cp_wqkv = pltpu.make_async_copy(wqkv_hbm, wqkv, sem_in.at[4])
    cp_wo = pltpu.make_async_copy(wo_hbm, wo, sem_in.at[5])
    cp_fk = pltpu.make_async_copy(fk_hbm, fk.bitcast(BF16), sem_in.at[6])
    cp_f = pltpu.make_async_copy(f_hbm, fm.bitcast(BF16), sem_in.at[7])
    cp_o = [pltpu.make_async_copy(xb.at[c], out_hbm.at[:, pl.ds(128 * c, 128)], sem_out.at[c])
            for c in range(4)]
    cp_p = [[pltpu.make_async_copy(r.at[rows], par_ref.at[i, rows], sem_p.at[6 * h + i])
             for i, r in enumerate((are_hbm, aim_hbm, bre_hbm, bim_hbm, cre_hbm, cim_hbm))]
            for h, rows in enumerate((pl.ds(0, P0), pl.ds(P0, D - P0)))]
    cp_s = [pltpu.make_async_copy(a, b, sem_p.at[12 + i])
            for i, (a, b) in enumerate(((ldt_hbm, ldt_ref), (dsk_hbm, dsk_ref), (pm_hbm, pm_ref)))]
    cp_p = [cp_s[:1] + cp_p[0], cp_p[1] + cp_s[1:]]
    for c in cp_p[0] + cp_p[1]:
        c.start()

    for ref in (dtc, dsc, kt, wt, wot, xn, os_, xr, qs, ke, ve, kf, zs):
        ref[(0,) * (len(ref.shape) - 2) + (pl.ds(1, 8), pl.ds(0, 128))] = jnp.zeros((8, 128), ref.dtype)

    zero[pl.ds(1, 16)] = jnp.zeros((16, 128), U32)
    marks, used, rate = [], [], [1.0]

    def mark(x):
        marks.extend(x[r:r + 8, :128] for r in range(0, x.shape[0], 16) for _ in range(x.shape[1] // 128))

    def pace(vals, cost):
        if not marks:
            return list(vals)
        i = min(max(used + [0, len(marks) - LG]), len(marks) - 1)
        used[:] = [i + cost * rate[0] / 16]
        t = pltpu.bitcast(marks[int(i)], U32) & zero[8:16]
        return [pltpu.bitcast(pltpu.bitcast(v, U32) | t, F32) for v in vals]

    def overlap(m, *vs):
        r = sum(c for c, _ in m) / max(1, sum(c for v in vs for c, _ in v))
        return [(1, lambda: rate.__setitem__(0, r))] + _merge(m, *vs)

    def barrier():
        pl.semaphore_signal(sem_b, 1)
        pl.semaphore_wait(sem_b, 1)
        marks[:], used[:] = [], []

    def iota(axis):
        return jax.lax.broadcasted_iota(I32, (8, 128), axis)

    def step_size():
        dt_row = jnp.exp(ldt_ref[...].astype(F32).reshape(1, D)).astype(BF16).astype(F32)
        dtc[...] = jnp.broadcast_to(dt_row, (128, D)).T

    def d_skip():
        dsc[...] = jnp.broadcast_to(dsk_ref[...].astype(F32).reshape(1, D), (128, D)).T

    def k_tables(g):
        st = {}

        def par(i):
            return par_ref[i, 16 * (g // 2):16 * (g // 2) + 16].astype(F32)[8 * (g % 2):8 * (g % 2) + 8]

        def mix(u, v):
            lo = iota(0) < 4
            rv = [pltpu.roll(c, 4, 0) for c in v]
            return (tuple(jnp.where(lo, a, b) for a, b in zip(u, rv)),
                    tuple(jnp.where(lo, b, a) for a, b in zip(u, rv)))

        def put(name, t, two):
            kreg.setdefault((name, g, t), []).append(jnp.concatenate(
                [jnp.concatenate([two[0][c], two[1][c]], axis=0) for c in range(2)], axis=1))

        def base():
            dt, = pace([dtc[8 * g:8 * g + 8]], 100)
            zr, zi = dt * par(0), dt * par(1)
            mag = jnp.exp(zr)
            st[1] = (mag * jnp.cos(zi), mag * jnp.sin(zi))
            st[0] = _cmul((par(4), par(5)), (dt * par(2), dt * par(3)))

        def left():
            lam = {1: st[1]}
            for p in range(1, 10):
                lam[2 ** p] = _csq(lam[2 ** (p - 1)])
            st[16] = lam[16]
            e = {(0, 0): st[0]}
            for a1 in (1, 2, 3):
                e[a1, 0] = _cmul(e[a1 - 1, 0], lam[512])
            for a1, r in ((0, 8), (1, 4), (0, 16), (1, 16)):
                e[a1, r] = _cmul(e[a1, 0], lam[r])
            d1, d8 = mix(lam[1], lam[1]), mix(lam[8], lam[8])
            prev, done = None, []
            for i, (u, v) in enumerate(_PAIRS):
                if u in e:
                    cur = mix(e[u], e[v])
                else:
                    m = d1 if i < 8 else d8
                    cur = (_cmul(prev[0], m[0]), _cmul(prev[1], m[1]))
                prev = cur
                done.append(cur)
                if i % 2:
                    for t in range(2):
                        put("l", t, (done[i - 1][t], done[i][t]))

        def right(t):
            lo = iota(0) < 4
            if t == 0:
                f = (_flip8(st[16][0], iota(0)), -_flip8(st[16][1], iota(0)))
                st["d"] = mix(f, f)[::-1]
            d = st["d"][t]
            d2 = _csq(d)
            one = (1.0, 0.0)
            cur = tuple(jnp.where(lo, a, b) for a, b in (zip(one, d), zip(d, d2))[t])
            for v in range(0, 16, 2):
                if v:
                    cur = _cmul(cur, d2)
                nxt = _cmul(cur, d2)
                if t and v == 14:
                    nxt = tuple(jnp.where(lo, a, b) for a, b in zip(nxt, one))
                put("r", t, (cur, nxt))
                cur = nxt

        return [(45, base), (70, left), (35, lambda: right(0)), (30, lambda: right(1))]

    kreg = {}

    def k_matmul(g):
        def mm():
            kreg[g] = [_dot(*(jnp.concatenate(kreg.pop((n, g, t)), axis=0).astype(BF16)
                              for n in "lr"), NT) for t in range(2)]

        def post():
            o0, o1 = kreg.pop(g)
            mark(o0); mark(o1)
            lo = iota(0) < 4
            ln = (iota(1) + (NA - 3)) & (NA - 1)
            piece = {}
            for i, (u, v) in enumerate(_PAIRS):
                a, b = o0[8 * i:8 * i + 8], o1[8 * i:8 * i + 8]
                for e, x in ((u, jnp.where(lo, a, b)), (v, pltpu.roll(jnp.where(lo, b, a), 4, 0))):
                    piece[e] = pltpu.roll(x, e[0], 1, stride=1, stride_axis=0)
            memo, res = {}, []
            for j in range(NJ):
                r2, r4, r8 = _R[1][j], _R[2][j], _R[4][j]
                if r8 not in memo:
                    memo[r8] = jnp.where((ln & 3) == 2, piece[2, r8], piece[3, r8])
                if (r4, r8) not in memo:
                    memo[r4, r8] = jnp.where((ln & 3) == 1, piece[1, r4], memo[r8])
                x = piece[0, j] if r2 == j else jnp.where(ln < 64, piece[0, j], piece[0, r2])
                res.append(jnp.where((ln & 3) == 0, x, memo[r4, r8]))
            if g % 2 == 0:
                kreg["even"] = res
            else:
                ev = kreg.pop("even")
                for j in range(0, NJ, 2):
                    kt.at[j // 2][4 * g - 4:4 * g + 4] = _pk4([ev[j], res[j], ev[j + 1], res[j + 1]])

        return [(5, mm)], [(30, post)]

    def k_fft(g):
        def run(h):
            rows = pl.ds(8 * g, 8)
            dsk = dsc[rows]
            for i, xs_ in enumerate(spectrum(rows, h, 20 + 6 * h)):
                for m1, (yr, yi) in enumerate(xs_):
                    kf[0, 4 * (h + 2 * i) + m1, rows] = (yr + dsk) * (1.0 / S)
                    kf[1, 4 * (h + 2 * i) + m1, rows] = yi * (1.0 / S)
        return [(20 + 6 * h, lambda h=h: run(h)) for h in range(2)]

    def w_qkv(b):
        def run():
            cols = pl.ds(128 * b, 128)
            w = _dot(pm_ref[0 if b < 4 else 1], wqkv[:, cols], NT)
            wt[64 * b:64 * b + 64] = _pk(w)
        return [(128, run)]

    def w_out(b):
        def run():
            wot[:, 256 * b:256 * b + 256] = _pk(jnp.concatenate(
                [_dot(pm_ref[1], wo[r:r + 128]).T for r in (256 * b, 256 * b + 128)], axis=1))
        return [(256, run)]

    def x_in(j2):
        def run(c):
            v = xu[c, pl.ds(j2, NA, stride=NJ // 2), :].T
            xr[2 * j2, 128 * c:128 * c + 128] = pltpu.bitcast(v << 16, F32)
            xr[2 * j2 + 1, 128 * c:128 * c + 128] = pltpu.bitcast(v & np.uint32(0xFFFF0000), F32)
        return [(40, lambda c=c: run(c)) for c in range(4)]

    def x_out(c, j2):
        def run():
            u = jnp.concatenate([xr[j, 128 * c:128 * c + 128] for j in (2 * j2, 2 * j2 + 1)], axis=1)
            u = pltpu.bitcast(u.astype(BF16).astype(F32), U32)
            v = (u[:, :128] >> 16) | u[:, 128:]
            xu[c, pl.ds(j2, NA, stride=NJ // 2), :] = v.T
            if j2 == NJ // 2 - 1:
                cp_o[c].start()
        return [(25, run)]

    def tree(acc, xs_):
        acc = list(acc)
        for i, x in enumerate(xs_):
            acc[i % 4] = acc[i % 4] + x
        return acc

    def total(acc):
        return jnp.broadcast_to(
            jnp.sum((acc[0] + acc[1]) + (acc[2] + acc[3]), axis=0, keepdims=True), (8, 128))

    def ln(j):
        st = {}

        def mean():
            v = [xr[j, r:r + 8] for r in range(0, D, 8)]
            st["m"] = total(tree(pace(v[:4], 18), v[4:])) * (1.0 / D)

        def var(r0):
            m, = pace([st["m"]], 25)
            c = [xr[j, r:r + 8] - m for r in range(r0, r0 + D // 2, 8)]
            c = [v * v for v in c]
            if r0:
                st["s"] = jax.lax.rsqrt(total(tree(st["v"], c)) * (1.0 / D) + EPS)
            else:
                st["v"] = tree(c[:4], c[4:])

        def norm():
            for r in range(0, D, 32):
                if r % 128 == 0:
                    m, s_ = pace([st["m"], st["s"]], 10)
                u = [(xr[j, r + h:r + h + 8] - m) * s_ for h in range(0, 32, 8)]
                xn.at[j][r // 4:r // 4 + 8] = _pk4(u)

        return [(18, mean), (25, lambda: var(0)), (25, lambda: var(D // 2)), (40, norm)]

    def kv(j):
        p, jj = j & 1, j >> 1

        def run(dst, b):
            k = _dot(_bf(wt[64 * b:64 * b + 64]), _rows(xn, j, 0, D))
            mark(k)
            r = pl.ds(128 * (b % 4), 128)
            dst[p, 7 + jj, r] = k
            if jj:
                dst[p, jj - 1, r] = pltpu.roll(k, 1, 1)

        return [(128, lambda b=b: run(ke if b < 8 else ve, b)) for b in range(4, 12)]

    def qproj(j):
        def run(b):
            q = _dot(_bf(wt[64 * b:64 * b + 64]), _rows(xn, j, 0, D))
            mark(q)
            qs[j, 128 * b:128 * b + 128] = q
        return [(128, lambda b=b: run(b)) for b in range(4)]

    def core(j):
        p, jj = j & 1, j >> 1
        st = {}

        def probs(hg, d0):
            s = st.pop(hg) if d0 else [None] * WIN
            rows = [pl.ds(128 * hg + 8 * d, 8) for d in range(d0, d0 + DH // 2)]
            qv = [qs[j, r] for r in rows]
            for r, q in zip(rows, pace(qv[:4], 16) + pace(qv[4:], 29 if d0 else 17)):
                for w in range(WIN):
                    t = q * ke[p, 7 + jj - w, r]
                    s[w] = t if s[w] is None else s[w] + t
            if not d0:
                st[hg] = s
                return
            for w in range(jj + 1, WIN):
                s[w] = jnp.where(iota(1) >= 1, s[w], -1e9)
            m = s[0]
            for w in range(1, WIN):
                m = jnp.maximum(m, s[w])
            e = [jnp.exp(a - m) for a in s]
            tot = e[0]
            for w in range(1, WIN):
                tot = tot + e[w]
            inv = 1.0 / tot
            st[hg] = [a * inv for a in e]

        def apply(hg, d0):
            e = pace(st.pop(hg) if d0 else st[hg], 32)
            for d in range(d0, d0 + DH // 2, 4):
                o = []
                for r in (pl.ds(128 * hg + 8 * (d + n), 8) for n in range(4)):
                    acc = e[0] * ve[p, 7 + jj, r]
                    for w in range(1, WIN):
                        acc = acc + e[w] * ve[p, 7 + jj - w, r]
                    o.append(acc)
                os_.at[j][pl.ds(32 * hg + 2 * d, 8)] = _pk4(o)

        return [(c, lambda f=f, hg=hg, d0=d0: f(hg, d0)) for hg in range(4)
                for c, f, d0 in ((33, probs, 0), (45, probs, 8), (32, apply, 0), (32, apply, 8))]

    def wout(j):
        def run(b):
            r = pl.ds(128 * b, 128)
            y = _dot(_bf(wot[64 * b:64 * b + 64]), _rows(os_, j, 0, D))
            mark(y)
            xr[j, r] = xr[j, r] + y
        return [(128, lambda b=b: run(b)) for b in range(4)]

    def dft(src, mat, c0, n, more=False):
        def run(j):
            rows = pl.ds(c0, n)
            a, b = (_dot(src(i, c0, n), _bf(mat[i])) for i in (j, j + 8))
            for h, z in enumerate((a + b, a - b)):
                i = 8 * h + j
                res = {i: (z[:, :128], z[:, 128:])}
                if more and 4 <= j < 7:
                    res[i - 4], res[i] = second((zs[0, i - 4, rows], zs[1, i - 4, rows]), res[i], j - 4, h)
                for k, v in res.items():
                    zs[0, k, rows], zs[1, k, rows] = v
            if more:
                mark(z)
        return [(n, lambda j=j: run(j)) for j in range(NJ // 2)]

    def second(p, q, j0, h):
        return [_twiddle(v, j0 * (h + 2 * i)) for i, v in enumerate(_half4(p, q, h))]

    def spectrum(rows, h, cost, done=0):
        z = [(zs[0, 8 * h + j, rows], zs[1, 8 * h + j, rows]) for j in range(8)]
        paced = (0, 3, 4) if done else (0, 1, 2, 3)
        pz = pace([c for i in paced for c in z[i]], cost)
        for n, i in enumerate(paced):
            z[i] = tuple(pz[2 * n:2 * n + 2])
        a = [(z[j0], z[j0 + 4]) if j0 < done else second(z[j0], z[j0 + 4], j0, h) for j0 in range(4)]
        return [_bfly4([a[j0][i] for j0 in range(4)], False) for i in range(2)]

    def fft(c0, n):
        def run(r0, h):
            rows = pl.ds(r0, 8)
            b = []
            for i, xs_ in enumerate(spectrum(rows, h, 40 + 6 * h, 3)):
                m0 = h + 2 * i
                y = [_cmul(v, (kf[0, 4 * m0 + m1, rows], kf[1, 4 * m0 + m1, rows]))
                     for m1, v in enumerate(xs_)]
                b.append([_twiddle(v, -j0 * m0) for j0, v in enumerate(_bfly4(y, True))])
            for j0 in range(4):
                (ar, ai), (br, bi) = b[0][j0], b[1][j0]
                lo = (ar + br, ai + bi)
                hi = (bi - ai, ar - br) if h else (ar - br, ai - bi)
                for c in range(2):
                    zs[c, 8 * h + j0, rows] = lo[c]
                    zs[c, 8 * h + j0 + 4, rows] = hi[c]
        return [(40 + 6 * h, lambda r0=r0, h=h: run(r0, h))
                for r0 in range(c0, c0 + n, 8) for h in range(2)]

    def inv(c0, n, js):
        def run(j):
            rows = pl.ds(c0, n)
            a, b = (jnp.concatenate([zs[0, i, rows], zs[1, i, rows]], axis=1) for i in (j, j + 8))
            ys = [_dot(z.astype(BF16), _bf(fm[i]), NT) for i, z in ((j, a + b), (j + 8, a - b))]
            for i, y in zip((j, j + 8), ys):
                xr[i, rows] = xr[i, rows] + y
            mark(ys[0])
        return [(n, lambda j=j: run(j)) for j in js]

    def cat(lists):
        return [t for l in lists for t in l]

    k_steps, tab = [], [k_tables(g) for g in range(64)] + [[], [], []]
    for g in range(-2, 64):
        mm, post = k_matmul(g) if g >= 0 else ([], [])
        k_steps.append(mm + tab[g + 1][1:2] + tab[g + 2][:1] + post + tab[g + 1][2:])

    order = [j0 + d for j0 in (0, 2, 1, 3) for d in (0, 8, 4, 12)]

    def lane_dft(n):
        return [dft(lambda *a: _rows(xn, *a), fm, c, 128, True)[order[2 * n]] for c in range(0, D, 128)]

    def attention(pre, extra):
        steps = [pre[0] + pre[1] + ln(order[0])]
        for i in range(8):
            steps.append(overlap(kv(order[i]) + pre[i + 2], ln(order[i + 1]), extra[i]))
        steps.append(qproj(order[0]))
        for i in range(NJ + 4):
            wo_, ln2 = ([order[n] for n in (2 * k - 1, 2 * k) if 0 <= n < NJ] for k in (i - 8, i - 9))
            m = pre[i + 10] if i < 6 else []
            m = m + _merge(kv(order[8 + i]) if i < 8 else [],
                           qproj(order[i + 1]) if i + 1 < NJ else [], cat(wout(j) for j in wo_))
            m = _merge(m, [t for n in PAIRS_AT.get(i, ()) for c, t in enumerate(lane_dft(n))
                           if (n, c) not in LATE])
            v = (ln(order[8 + i + 1]) if i < 7 else []) + cat(ln(j) for j in ln2)
            c = core(order[i]) if i < NJ else []
            if i >= NJ - 1:
                c, v = (t + [(0.25 * sum(x for x, _ in t), lambda: None)] for t in (c, v))
            steps.append(overlap(m, c, v))
        return steps

    def ssm(last):
        prog = [(0, barrier)]
        for c in range(0, D, G):
            out = cat(x_out(c // 128 - 1, j2) for j2 in range(8)) if last and c > 128 and c % 128 else []
            prog += overlap(inv(c - G, G, range(NJ // 2)) if c else [lane_dft(n)[b] for n, b in LATE],
                            fft(c, G), out)
            if out and c > 256:
                prog += [(0, barrier)]
        return prog

    def wait(*cps):
        def run():
            for c in cps:
                c.wait()
            marks[:], used[:] = [], []
        return [(0, run)]

    def start(*cps):
        return [(0, lambda: [c.start() for c in cps])]

    kd = [dft(lambda j, c0, n: _bf(kt[j // 2, pl.ds(c0 // 2, n // 2), pl.ds(128 * (j % 2), 128)]),
              fk, c, 128) for c in range(0, D, 128)]
    a1 = attention([[]] * NJ, [cat(k_fft(g) for g in range(8 * i, 8 * i + 8)) for i in range(8)])
    head = wait(*cp_p[0]) + [(1, step_size)] + cat(k_steps[:P0 // 8]) + wait(*cp_p[1])
    head += start(cp_fk, cp_wqkv, *cp_x) + cat(k_steps[P0 // 8:40]) + wait(cp_fk)
    head += _merge(cat(k_steps[40:]), kd[0] + kd[1]) + wait(cp_wqkv, *cp_x) + start(cp_wo, cp_f) + [(1, d_skip)]
    head += _merge(_merge(kd[2] + kd[3], cat(w_qkv(b) for b in range(12))),
                   x_in(0) + a1[0] + cat(x_in(j2) for j2 in range(1, 8)))
    head += [(0, barrier)]
    prog = head + cat(a1[1:9]) + wait(cp_wo, cp_f) + w_out(0) + w_out(1)
    prog += cat(a1[9:]) + ssm(False)
    a2 = attention([inv(D - G, G, [j]) if j < 8 else [] for j in order], [[]] * 8)
    prog += cat(a2)
    prog += ssm(True)
    prog += inv(D - G, G, range(NJ // 2))
    prog += cat(x_out(3, j2) for j2 in (0, 4, 1, 5, 2, 6, 3, 7))
    for _, fn in prog:
        fn()
    for c in cp_o:
        c.wait()


@jax.jit
def pallas_interleave_layers__sliding_local_dilated__ssm_conv_s4__prompt_kernel(
    A_x: jax.Array,
    A_wqkv: jax.Array,
    A_wo: jax.Array,
    B_u: jax.Array,
    B_A_re: jax.Array,
    B_A_im: jax.Array,
    B_B_re: jax.Array,
    B_B_im: jax.Array,
    B_C_re: jax.Array,
    B_C_im: jax.Array,
    B_log_dt: jax.Array,
    B_Dskip: jax.Array,
):
    del B_u
    hbm = pl.BlockSpec(memory_space=pl.ANY)
    out = pl.pallas_call(
        _kernel,
        in_specs=[hbm] * 14,
        out_specs=hbm,
        out_shape=jax.ShapeDtypeStruct((S, D), BF16),
        scratch_shapes=[
            pltpu.VMEM((2, NA, NA), BF16),
            pltpu.VMEM((D,), BF16),
            pltpu.VMEM((D,), BF16),
            pltpu.VMEM((6, D, 128), BF16),
            pltpu.VMEM((4, S // 2, 128), U32),
            pltpu.VMEM((D, 3 * D), BF16),
            pltpu.VMEM((D, D), BF16),
            pltpu.VMEM((NJ, NA // 2, 256), U32),
            pltpu.VMEM((NJ, NA // 2, 256), U32),
            pltpu.VMEM((D, 128), F32),
            pltpu.VMEM((D, 128), F32),
            pltpu.VMEM((NJ // 2, D // 2 + 8, 256), U32),
            pltpu.VMEM((3 * D // 2, D), U32),
            pltpu.VMEM((D // 2, D), U32),
            pltpu.VMEM((NJ, D // 4 + 8, 256), U32),
            pltpu.VMEM((NJ, D // 4 + 8, 256), U32),
            pltpu.VMEM((NJ, D + PAD, NA), F32),
            pltpu.VMEM((NJ, D + PAD, NA), F32),
            pltpu.VMEM((2, NJ - 1, D + PAD, NA), F32),
            pltpu.VMEM((2, NJ - 1, D + PAD, NA), F32),
            pltpu.VMEM((2, NJ, D + PAD, NA), F32),
            pltpu.VMEM((2, NJ, D + PAD, NA), F32),
            pltpu.VMEM((24, NA), U32),
            pltpu.SemaphoreType.DMA((8,)),
            pltpu.SemaphoreType.DMA((4,)),
            pltpu.SemaphoreType.DMA((15,)),
            pltpu.SemaphoreType.REGULAR,
        ],
        compiler_params=pltpu.CompilerParams(vmem_limit_bytes=100 << 20),
    )(A_x.reshape(S, D), A_wqkv, A_wo, _F, _FK,
      B_A_re, B_A_im, B_B_re, B_B_im, B_C_re, B_C_im,
      _PM, B_log_dt, B_Dskip)
    return out.reshape(1, S, D)
```
